```python
import os as _os
_os.environ.setdefault("JAX_PLATFORMS", "cpu")
import jax
import jax.numpy as jnp

def _softmax(x, axis=-1):
    return jax.nn.softmax(x, axis=axis)
def _gelu(x):
    return jax.nn.gelu(x, approximate=True)
def _silu(x):
    return jax.nn.silu(x)
def _sigmoid(x):
    return jax.nn.sigmoid(x)
def _layernorm(x, axis=-1, eps=1e-5):
    m = jnp.mean(x, axis=axis, keepdims=True)
    v = jnp.var(x, axis=axis, keepdims=True)
    return (x - m) / jnp.sqrt(v + eps)
def _scatter_add(tgt, idx, src, axis=0):
    return tgt.at[idx].add(src)
def _segment_sum(src, seg, n):
    return jax.ops.segment_sum(src, seg, n)
class _Rng:
    def __init__(self, key):
        self._k = key
    def _next(self):
        self._k, sub = jax.random.split(self._k)
        return sub
    def normal(self, shape):
        return jax.random.normal(self._next(), shape, dtype=jnp.bfloat16)
    def randint(self, lo, hi, shape):
        return jax.random.randint(self._next(), shape, lo, hi, dtype=jnp.int32)
    def uniform(self, shape, lo=0.0, hi=1.0):
        return jax.random.uniform(self._next(), shape, jnp.bfloat16, lo, hi)
    def permutation(self, n):
        return jax.random.permutation(self._next(), n)


kernel_name = 'gated_mix__spectral_gfnet__dense_activation_silu__prompt'

def setup_inputs():
    _rng = _Rng(jax.random.key(int.from_bytes(__import__("os").urandom(4), "little")))
    _w = (lambda a: (lambda t: t.astype(jnp.bfloat16) if jnp.issubdtype(t.dtype, jnp.floating) else t)(jnp.asarray(a)))
    def _A_setup():
        B, S, D = 1, 2048, 512
        Df = D // 2 + 1
        return {
            "x": _w((lambda *s: _rng.normal(s) * 0.05)(B, S, D)),
            "w_r": _w((lambda *s: _rng.normal(s) * 0.05)(S, Df) * 0.02),
            "w_i": _w((lambda *s: _rng.normal(s) * 0.05)(S, Df) * 0.02),
        }
    _A_in = _A_setup()

    def _B_setup():
        B, S, D, F = 1, 2048, 512, 1376
        return {
            "x": _w((lambda *s: _rng.normal(s) * 0.05)(B, S, D)),
            "w1": _w((lambda *s: _rng.normal(s) * 0.05)(D, F) * (D ** -0.5)),
            "w2": _w((lambda *s: _rng.normal(s) * 0.05)(F, D) * (F ** -0.5)),
        }
    _B_in = _B_setup()

    return {
        "A_x": _A_in["x"],
        "A_w_r": _A_in["w_r"],
        "A_w_i": _A_in["w_i"],
        "B_x": _B_in["x"],
        "B_w1": _B_in["w1"],
        "B_w2": _B_in["w2"],
        "gate_w": _w((lambda *s: _rng.normal(s) * 0.05)(512) * 16.0),
    }

def reference(A_x, A_w_r, A_w_i, B_x, B_w1, B_w2, gate_w):
    def _A_ref(x, w_r, w_i):
        B, S, D = x.shape
        X = (lambda x, axes=(-2,-1): jnp.fft.rfft2(x.astype(jnp.float32), axes=axes))(x, axes=(-2, -1))
        W = w_r + 1j * w_i
        X = X * W
        y = (lambda x, s, axes=(-2,-1): jnp.fft.irfft2(x, s=s, axes=axes).astype(jnp.bfloat16))(X, (S, D), axes=(-2, -1))
        return y

    def _B_ref(x, w1, w2):
        h = jnp.einsum("bsd,df->bsf", x, w1)
        h = _silu(h)
        out = jnp.einsum("bsf,fd->bsd", h, w2)
        return out

    x = A_x
    g = _sigmoid((x * gate_w).sum(-1, keepdims=True))
    a = _A_ref(x, A_w_r, A_w_i)
    b = _B_ref(x, B_w1, B_w2)
    return g * a + (1 - g) * b
```

```python
import functools
import numpy as np
import jax
import jax.numpy as jnp
import jax.experimental.pallas as pl
import jax.experimental.pallas.tpu as pltpu

S, D, F = 2048, 512, 1376
FP = 1408
RES = (0, 4, 2, 6, 1, 7, 5, 3)
BF = jnp.bfloat16
F32 = jnp.float32
U32 = jnp.uint32
C8 = float(np.sqrt(0.5))
NT = (((1,), (1,)), ((), ()))


def _kd_of_row(rho):
    return 8 * (rho % 32) + RES[rho // 32]


@functools.lru_cache(maxsize=None)
def _consts():
    l = np.arange(128)
    A = np.zeros((4, 128, 128))
    for t in range(4):
        for i in range(64):
            rho = 64 * t + i
            kd = _kd_of_row(rho)
            if t < 2:
                ang = 2 * np.pi * ((l * kd) % 512) / 512
                A[t, i] = np.cos(ang)
                A[t, 64 + i] = -np.sin(ang)
                if rho == 0:
                    A[t, 64] = np.where(l % 2 == 0, 1.0, -1.0)
            else:
                f = t - 2
                lp = np.arange(64)
                k, cj = (kd, 1.0) if kd % 8 == 1 + 4 * f else (512 - kd, -1.0)
                ang = 2 * np.pi * ((lp * k) % 512) / 512
                c, s = np.cos(ang), -np.sin(ang)
                sg = 1.0 if f == 0 else -1.0
                A[t, i, :64] = c
                A[t, i, 64:] = -s * sg
                A[t, 64 + i, :64] = cj * s
                A[t, 64 + i, 64:] = cj * c * sg
    Ai = np.zeros((4, 128, 128))
    for t in range(4):
        sc = np.full(128, 2.0 / (S * D))
        if t == 0:
            sc[0] = sc[64] = 1.0 / (S * D)
        M = A[t] * sc[:, None]
        Ai[t] = M if t % 2 == 0 else np.concatenate([M[64:], M[:64]], 0)
    Ms = np.zeros((16, 2, 128, 128))
    n1 = np.arange(64)[:, None]
    k1 = np.arange(64)[None, :]
    for e in range(2):
        for n2 in range(16):
            ang = 2 * np.pi * (((16 * n1 + n2) * (e + 2 * k1)) % 2048) / 2048
            c, s = np.cos(ang), -np.sin(ang)
            re_cols = 2 * np.arange(64) + e
            im_cols = (2 * np.arange(64) + 1 + e) % 128
            M = np.zeros((128, 128))
            rr = slice(0, 64) if e == 0 else slice(64, 128)
            ir = slice(64, 128) if e == 0 else slice(0, 64)
            M[rr, re_cols] = c
            M[ir, re_cols] = -s
            M[rr, im_cols] = s
            M[ir, im_cols] = c
            Ms[n2, e] = M
    J = np.zeros((1, 128, 128))
    J[0, l, (128 - l) % 128] = 1.0
    allc = np.concatenate([A, Ai, J, Ms.reshape(32, 128, 128)], 0)
    return allc.astype(np.float32)


CA, CAI, CJ, CM = 0, 4, 8, 9
NCONST = 41


def _add(a, b):
    (x, sx), (y, sy) = a, b
    if sx == sy:
        return (x + y, sx)
    return (x - y, 1) if sx > 0 else (y - x, 1)


def _neg(a):
    return (a[0], -a[1])


def _sub(a, b):
    return _add(a, _neg(b))


def _scale(a, c):
    return (a[0] * (c * a[1]), 1) if True else None


def _cadd(a, b):
    return (_add(a[0], b[0]), _add(a[1], b[1]))


def _csub(a, b):
    return (_sub(a[0], b[0]), _sub(a[1], b[1]))


def _mul_mi(a, sgn):
    re, im = a
    return (im, _neg(re)) if sgn > 0 else (_neg(im), re)


def _twiddle(a, j, sgn):
    j = j % 16
    if j % 4 == 0:
        for _ in range(j // 4):
            a = _mul_mi(a, sgn)
        return a
    re, im = a
    if j % 2 == 0:
        q = j // 4
        if sgn > 0:
            r = _scale(_add(re, im), C8)
            i = _scale(_sub(im, re), C8)
        else:
            r = _scale(_sub(re, im), C8)
            i = _scale(_add(im, re), C8)
        a = (r, i)
        for _ in range(q):
            a = _mul_mi(a, sgn)
        return a
    c = float(np.cos(2 * np.pi * j / 16))
    s = float(-sgn * np.sin(2 * np.pi * j / 16))
    r = _sub(_scale(re, c), _scale(im, s))
    i = _add(_scale(re, s), _scale(im, c))
    return (r, i)


def _dft4(v, sgn):
    a, b, c, d = v
    t0, t1 = _cadd(a, c), _csub(a, c)
    t2, t3 = _cadd(b, d), _mul_mi(_csub(b, d), sgn)
    return [_cadd(t0, t2), _cadd(t1, t3), _csub(t0, t2), _csub(t1, t3)]


def _dft16(v, sgn):
    y = [[None] * 4 for _ in range(4)]
    for b in range(4):
        o = _dft4([v[4 * a + b] for a in range(4)], sgn)
        for kap in range(4):
            y[kap][b] = _twiddle(o[kap], b * kap, sgn)
    out = [None] * 16
    for kap in range(4):
        o = _dft4(y[kap], sgn)
        for io in range(4):
            out[kap + 4 * io] = o[io]
    return out


def _force(a):
    return a[0] if a[1] > 0 else -a[0]


def _lo_f32(w):
    return pltpu.bitcast(w << 16, F32)


def _hi_f32(w):
    return pltpu.bitcast(w & jnp.uint32(0xFFFF0000), F32)


def _kernel(x_hbm, wr_hbm, wi_hbm, w1_hbm, w2_hbm, gw_ref, c_hbm, o_hbm,
            x_b, x_u, w1_v, w2_v, wr_u, wi_u, wl_v, c_v, xr_v, xi_v, a_u, bb_v, g_v, o_v,
            s_x, s_xu, s_w1, s_w2, s_w, s_wl, s_c, s_o):
    TM = 256
    NCH = S // TM
    cp_x = [pltpu.make_async_copy(x_hbm.at[0, :, pl.ds(128 * c, 128)], x_b.at[c], s_x.at[c]) for c in range(4)]
    xu_b = x_u.bitcast(BF)
    cp_xu = [pltpu.make_async_copy(x_hbm.at[0, :, pl.ds(128 * c, 128)], xu_b.at[c], s_xu.at[c]) for c in range(4)]
    cp_w1 = [pltpu.make_async_copy(w1_hbm.at[:, pl.ds(128 * c, 128)], w1_v.at[c, pl.ds(0, F)], s_w1.at[c]) for c in range(4)]
    cp_w2 = [pltpu.make_async_copy(w2_hbm.at[:, pl.ds(128 * c, 128)], w2_v.at[c, pl.ds(0, F)], s_w2.at[c]) for c in range(4)]
    wr_b = wr_u.bitcast(BF)
    wi_b = wi_u.bitcast(BF)
    cp_w = []
    for k in range(16):
        cp_w.append(pltpu.make_async_copy(wr_hbm.at[pl.ds(0, 256), pl.ds(128 * k, 128)], wr_b.at[k], s_w.at[k]))
        cp_w.append(pltpu.make_async_copy(wi_hbm.at[pl.ds(0, 256), pl.ds(128 * k, 128)], wi_b.at[k], s_w.at[16 + k]))
    cp_wl = [pltpu.make_async_copy(wr_hbm.at[pl.ds(256, 1), :], wl_v.at[0], s_wl.at[0]),
             pltpu.make_async_copy(wi_hbm.at[pl.ds(256, 1), :], wl_v.at[1], s_wl.at[1])]
    cp_c = [pltpu.make_async_copy(c_hbm, c_v, s_c.at[0])]
    for cp in cp_x + cp_xu + cp_c + cp_w1 + cp_w2 + cp_w + cp_wl:
        cp.start()
    for c in range(4):
        w1_v[c, pl.ds(F, FP - F), :] = jnp.broadcast_to(gw_ref[c:c + 1, :].astype(F32), (FP - F, 128)).astype(BF)
        w2_v[c, pl.ds(F, FP - F), :] = jnp.zeros((FP - F, 128), BF)
    for cp in cp_x + cp_xu + cp_c + cp_w1 + cp_w2 + cp_w + cp_wl:
        cp.wait()

    lane = jax.lax.broadcasted_iota(jnp.int32, (128, 128), 1)
    lo = lane < 64
    lane2 = jax.lax.broadcasted_iota(jnp.int32, (256, 128), 1)
    even2 = (lane2 % 2) == 0
    even = (lane % 2) == 0
    lo64 = jax.lax.broadcasted_iota(jnp.int32, (64, 128), 1) < 64

    def p1_one(xs, n2):
        U = [jnp.concatenate([t[:64] + t[64:], t[:64] - t[64:]], 0) for t in xs]
        p0, p1, m0, m1 = U[0] + U[2], U[1] + U[3], U[0] - U[2], U[1] - U[3]
        v0, v2 = p0 + p1, p0 - p1
        P = jnp.where(lo, m0, (m0 + m1) * (-C8))
        Q = pltpu.roll(jnp.where(lo, -m1, (m0 - m1) * C8), 64, 1)
        T = [v0, v2, P + Q, P - Q]
        Z = [jax.lax.dot_general(c_v[CA + t], T[t].astype(BF), NT, preferred_element_type=F32) for t in range(4)]
        ZR = jnp.concatenate([z[:64] for z in Z], 0).astype(BF)
        ZI = jnp.concatenate([z[64:] for z in Z], 0).astype(BF)
        ZRu = pltpu.bitcast(ZR, U32)
        RIu = pltpu.roll(pltpu.bitcast(ZI, U32), 64, 1)
        T0 = pltpu.bitcast(jnp.where(lo, ZRu, RIu), BF)
        T1 = pltpu.bitcast(jnp.where(lo, RIu, ZRu), BF)
        O0 = jnp.dot(T0, c_v[CM + 2 * n2], preferred_element_type=F32)
        O1 = jnp.dot(T1, c_v[CM + 2 * n2 + 1], preferred_element_type=F32)
        xr_v[n2] = jnp.where(even2, O0, O1)
        xi_v[n2] = pltpu.roll(jnp.where(even2, O1, O0), 127, 1)

    def p1(r0, _):
        ws = [x_u[c, pl.ds(r0, 128, stride=8), :] for c in range(4)]
        p1_one([_lo_f32(w) for w in ws], 2 * r0)
        p1_one([_hi_f32(w) for w in ws], 2 * r0 + 1)
        return 0

    jax.lax.fori_loop(0, 8, p1, 0)

    def p2_group(cls, ig, special):
        row = pl.ds(pl.multiple_of(32 * cls + 8 * ig, 8), 8)
        wrow = pl.ds(32 * ig + RES[cls] // 2, 8, stride=4)
        unp = _hi_f32 if RES[cls] % 2 else _lo_f32
        v = [((xr_v[k, row, :], 1), (xi_v[k, row, :], 1)) for k in range(16)]
        X = _dft16(v, +1)
        Y = []
        for k in range(16):
            wr = unp(wr_u[k, wrow, :])
            wi = unp(wi_u[k, wrow, :])
            (xr, sr), (xi, si) = X[k]
            yr = _sub((xr * wr, sr), (xi * wi, si))
            yi = _add((xr * wi, sr), (xi * wr, si))
            Y.append((yr, yi))
        if special:
            sub = jax.lax.broadcasted_iota(jnp.int32, (8, 128), 0)
            ln = jax.lax.broadcasted_iota(jnp.int32, (8, 128), 1)
            ar, ai, br, bi, stack = [], [], [], [], []
            for k in range(16):
                w0r = unp(wr_u[k, wrow, :])[0:1]
                w0i = unp(wi_u[k, wrow, :])[0:1]
                wlr = wl_v[0, :, 128 * k:128 * k + 128].astype(F32)
                wli = wl_v[1, :, 128 * k:128 * k + 128].astype(F32)
                pr = _force(X[k][0])[0:1]
                pi = _force(X[k][1])[0:1]
                rows = [pr, pi, w0r, w0i, wlr, wli]
                blk = jnp.zeros((8, 128), F32)
                for j, r in enumerate(rows):
                    blk = jnp.where(sub == j, jnp.broadcast_to(r, (8, 128)), blk)
                stack.append(blk)
            full = jnp.concatenate(stack, 0)
            hi_ = full.astype(BF)
            lo_ = (full - hi_.astype(F32)).astype(BF)
            fl = (jnp.dot(hi_, c_v[CJ], preferred_element_type=F32)
                  + jnp.dot(lo_, c_v[CJ], preferred_element_type=F32))
            for k in range(16):
                fa = fl[8 * (15 - k):8 * (15 - k) + 8]
                fb = fl[8 * ((16 - k) % 16):8 * ((16 - k) % 16) + 8]
                f = jnp.where(ln == 0, fb, fa)
                o = stack[k]
                pr, pi, w0r, w0i, wlr, wli = [o[j:j + 1] for j in range(6)]
                fpr, fpi, f0r, f0i, flr, fli = [f[j:j + 1] for j in range(6)]
                s0r, s0i = w0r + f0r, w0i - f0i
                slr, sli = wlr + flr, wli - fli
                Ar, Ai_ = (s0r + slr) * 0.25, (s0i + sli) * 0.25
                Br, Bi = (s0r - slr) * 0.25, (s0i - sli) * 0.25
                yr0 = pr * Ar - pi * Ai_ + fpr * Br + fpi * Bi
                yi0 = pr * Ai_ + pi * Ar + fpr * Bi - fpi * Br
                yr = jnp.where(sub == 0, jnp.broadcast_to(yr0, (8, 128)), _force(Y[k][0]))
                yi = jnp.where(sub == 0, jnp.broadcast_to(yi0, (8, 128)), _force(Y[k][1]))
                Y[k] = ((yr, 1), (yi, 1))
        Y1 = _dft16(Y, -1)
        for k in range(16):
            xr_v[k, row, :] = _force(Y1[k][0])
            xi_v[k, row, :] = _force(Y1[k][1])

    p2_group(0, 0, True)
    for cls in range(8):
        def body(ig, _, cls=cls):
            p2_group(cls, ig, False)
            return 0
        jax.lax.fori_loop(1 if cls == 0 else 0, 4, body, 0)

    def p3_one(n2):
        Ru = pltpu.bitcast(xr_v[n2].astype(BF), U32)
        Ou = pltpu.roll(pltpu.bitcast(xi_v[n2].astype(BF), U32), 1, 1)
        B0 = pltpu.bitcast(jnp.where(even, Ru, Ou), BF)
        B1 = pltpu.bitcast(jnp.where(even, Ou, Ru), BF)
        V0 = jax.lax.dot_general(c_v[CM + 2 * n2], B0, NT, preferred_element_type=F32)
        V1 = jax.lax.dot_general(c_v[CM + 2 * n2 + 1], B1, NT, preferred_element_type=F32)
        V0r, V0i = V0[:64], V0[64:]
        V1i, V1r = V1[:64], V1[64:]
        VR = jnp.concatenate([V0r + V1r, V0r - V1r], 0).astype(BF)
        VI = jnp.concatenate([V0i + V1i, V0i - V1i], 0).astype(BF)
        G = []
        for h in range(2):
            r = pltpu.bitcast(VR[:, 128 * h:128 * h + 128], U32)
            ri = pltpu.roll(pltpu.bitcast(VI[:, 128 * h:128 * h + 128], U32), 64, 1)
            G += [pltpu.bitcast(jnp.where(lo64, r, ri), BF), pltpu.bitcast(jnp.where(lo64, ri, r), BF)]
        v0, v2, T1, T3 = [jnp.dot(G[t], c_v[CAI + t], preferred_element_type=F32) for t in range(4)]
        Pp = T1 + T3
        Qp = pltpu.roll(T1 - T3, 64, 1)
        m0 = jnp.where(lo, Pp, (Qp - Pp) * C8)
        m1n = jnp.where(lo, Qp, (Pp + Qp) * C8)
        p0, p1 = v0 + v2, v0 - v2
        return [p0 + m0, p1 - m1n, p0 - m0, p1 + m1n]

    def p3(r0, _):
        ya = p3_one(2 * r0)
        yb = p3_one(2 * r0 + 1)
        for c in range(4):
            a_u[c, pl.ds(r0, 128, stride=8), :] = pltpu.pack_elementwise([ya[c], yb[c]], packed_dtype=BF)
        return 0

    jax.lax.fori_loop(0, 8, p3, 0)

    def ffn(i, _):
        r = pl.multiple_of(i * TM, TM)
        xc = jnp.concatenate([x_b[c, pl.ds(r, TM), :] for c in range(4)], 1)
        w1 = jnp.concatenate([w1_v[c] for c in range(4)], 1)
        h = jax.lax.dot_general(xc, w1, NT, preferred_element_type=F32)
        t = 0.5 * h
        th = jnp.tanh(t)
        g = jnp.broadcast_to(0.5 + 0.5 * th[:, FP - 1:FP], (TM, 128))
        hs = (t + t * th).astype(BF)
        r2 = pl.multiple_of(i * (TM // 2), TM // 2)
        for c in range(4):
            b = jnp.dot(hs, w2_v[c], preferred_element_type=F32)
            a = pltpu.bitcast(a_u[c, pl.ds(r2, TM // 2), :], BF).astype(F32)
            o_v[pl.ds(r, TM), 128 * c:128 * c + 128] = (b + g * (a - b)).astype(BF)
        pltpu.make_async_copy(o_v.at[pl.ds(r, TM)], o_hbm.at[0, pl.ds(r, TM)], s_o.at[i]).start()
        return 0

    jax.lax.fori_loop(0, NCH, ffn, 0)
    for i in range(NCH):
        pltpu.make_async_copy(o_v.at[pl.ds(i * TM, TM)], o_hbm.at[0, pl.ds(i * TM, TM)], s_o.at[i]).wait()


@jax.jit
def pallas_gated_mix__spectral_gfnet__dense_activation_silu__prompt_kernel(A_x, A_w_r, A_w_i, B_x, B_w1, B_w2, gate_w):
    consts = jnp.asarray(_consts(), dtype=BF)
    hbm = pl.BlockSpec(memory_space=pltpu.HBM)
    vmem = pl.BlockSpec(memory_space=pltpu.VMEM)
    dma = pltpu.SemaphoreType.DMA
    return pl.pallas_call(
        _kernel,
        in_specs=[hbm, hbm, hbm, hbm, hbm, vmem, hbm],
        out_specs=hbm,
        out_shape=jax.ShapeDtypeStruct((1, S, D), BF),
        scratch_shapes=[
            pltpu.VMEM((4, S, 128), BF),
            pltpu.VMEM((4, S // 2, 128), U32),
            pltpu.VMEM((4, FP, 128), BF),
            pltpu.VMEM((4, FP, 128), BF),
            pltpu.VMEM((16, 128, 128), U32),
            pltpu.VMEM((16, 128, 128), U32),
            pltpu.VMEM((2, 1, S), BF),
            pltpu.VMEM((NCONST, 128, 128), BF),
            pltpu.VMEM((16, 256, 128), F32),
            pltpu.VMEM((16, 256, 128), F32),
            pltpu.VMEM((4, S // 2, 128), U32),
            pltpu.VMEM((8, 128), F32),
            pltpu.VMEM((8, 128), F32),
            pltpu.VMEM((S, D), BF),
            dma((4,)), dma((4,)), dma((4,)), dma((4,)), dma((32,)), dma((2,)), dma((1,)), dma((8,)),
        ],
        compiler_params=pltpu.CompilerParams(vmem_limit_bytes=100 << 20),
    )(A_x, A_w_r.T, A_w_i.T, B_w1.T, B_w2, gate_w.reshape(4, 128), consts)
```

```python
import functools
import numpy as np
import jax
import jax.numpy as jnp
import jax.experimental.pallas as pl
import jax.experimental.pallas.tpu as pltpu

S, D, F = 2048, 512, 1376
FP = 1408
RES = (0, 4, 2, 6, 1, 7, 5, 3)
JR = (0, 2, 1, 3)
BF = jnp.bfloat16
F32 = jnp.float32
U32 = jnp.uint32
C8 = float(np.sqrt(0.5))
NT = (((1,), (1,)), ((), ()))


def _kd_of_row(rho):
    return 8 * (rho % 32) + RES[rho // 32]


def _n1_of_pos(p):
    return 8 * (2 * (p // 16) + p % 2) + (p % 16) // 2


_POS_OF_N1 = {_n1_of_pos(p): p for p in range(64)}


@functools.lru_cache(maxsize=None)
def _consts():
    l = np.arange(128)
    A = np.zeros((4, 128, 128))
    where = {}
    for t in range(4):
        for i in range(64):
            rho = 64 * t + i
            kd = _kd_of_row(rho)
            where[kd] = (t, i)
            if t < 2:
                ang = 2 * np.pi * ((l * kd) % 512) / 512
                A[t, i] = np.cos(ang)
                A[t, 64 + i] = -np.sin(ang)
                if rho == 0:
                    A[t, 64] = np.where(l % 2 == 0, 1.0, -1.0)
            else:
                f = t - 2
                lp = np.arange(64)
                k, cj = (kd, 1.0) if kd % 8 == 1 + 4 * f else (512 - kd, -1.0)
                ang = 2 * np.pi * ((lp * k) % 512) / 512
                c, s = np.cos(ang), -np.sin(ang)
                sg = 1.0 if f == 0 else -1.0
                A[t, i, :64] = c
                A[t, i, 64:] = -s * sg
                A[t, 64 + i, :64] = cj * s
                A[t, 64 + i, 64:] = cj * c * sg
    Ai = np.zeros((4, 128, 128))
    for half in range(2):
        sh = 1 + half
        for lam in range(128):
            kd = 2 * lam + half
            t, i = where[kd]
            sc = (1.0 if kd == 0 else 2.0) / (S * D)
            Ai[t, lam] = A[t, i] * sc
            Ai[t, (lam + sh) % 128] = A[t, 64 + i] * sc
    Ms = np.zeros((16, 2, 128, 128))
    n1 = np.array([_n1_of_pos(p) for p in range(64)])[:, None]
    k1 = np.arange(64)[None, :]
    for e in range(2):
        for n2 in range(16):
            ang = 2 * np.pi * (((16 * n1 + n2) * (e + 2 * k1)) % 2048) / 2048
            c, s = np.cos(ang), -np.sin(ang)
            re_cols = 2 * np.arange(64) + e
            im_cols = (2 * np.arange(64) + 1 + e) % 128
            M = np.zeros((128, 128))
            rr = slice(0, 64) if e == 0 else slice(64, 128)
            ir = slice(64, 128) if e == 0 else slice(0, 64)
            M[rr, re_cols] = c
            M[ir, re_cols] = -s
            M[rr, im_cols] = s
            M[ir, im_cols] = c
            Ms[n2, e] = M
    J = np.zeros((1, 128, 128))
    J[0, l, (128 - l) % 128] = 1.0
    allc = np.concatenate([A, Ai, J, Ms.reshape(32, 128, 128)], 0)
    return allc.astype(np.float32)


CA, CAI, CJ, CM = 0, 4, 8, 9
NCONST = 41


def _add(a, b):
    (x, sx), (y, sy) = a, b
    if sx == sy:
        return (x + y, sx)
    return (x - y, 1) if sx > 0 else (y - x, 1)


def _neg(a):
    return (a[0], -a[1])


def _sub(a, b):
    return _add(a, _neg(b))


def _scale(a, c):
    return (a[0] * (c * a[1]), 1)


def _cadd(a, b):
    return (_add(a[0], b[0]), _add(a[1], b[1]))


def _csub(a, b):
    return (_sub(a[0], b[0]), _sub(a[1], b[1]))


def _mul_mi(a, sgn):
    re, im = a
    return (im, _neg(re)) if sgn > 0 else (_neg(im), re)


def _twiddle(a, j, sgn):
    j = j % 16
    if j % 4 == 0:
        for _ in range(j // 4):
            a = _mul_mi(a, sgn)
        return a
    re, im = a
    if j % 2 == 0:
        if sgn > 0:
            r = _scale(_add(re, im), C8)
            i = _scale(_sub(im, re), C8)
        else:
            r = _scale(_sub(re, im), C8)
            i = _scale(_add(im, re), C8)
        a = (r, i)
        for _ in range(j // 4):
            a = _mul_mi(a, sgn)
        return a
    c = float(np.cos(2 * np.pi * j / 16))
    s = float(-sgn * np.sin(2 * np.pi * j / 16))
    r = _sub(_scale(re, c), _scale(im, s))
    i = _add(_scale(re, s), _scale(im, c))
    return (r, i)


def _dft4(v, sgn):
    a, b, c, d = v
    t0, t1 = _cadd(a, c), _csub(a, c)
    t2, t3 = _cadd(b, d), _mul_mi(_csub(b, d), sgn)
    return [_cadd(t0, t2), _cadd(t1, t3), _csub(t0, t2), _csub(t1, t3)]


def _dft16(v, sgn):
    y = [[None] * 4 for _ in range(4)]
    for b in range(4):
        o = _dft4([v[4 * a + b] for a in range(4)], sgn)
        for kap in range(4):
            y[kap][b] = _twiddle(o[kap], b * kap, sgn)
    out = [None] * 16
    for kap in range(4):
        o = _dft4(y[kap], sgn)
        for io in range(4):
            out[kap + 4 * io] = o[io]
    return out


def _force(a):
    return a[0] if a[1] > 0 else -a[0]


def _lo_f32(w):
    return pltpu.bitcast(w << 16, F32)


def _hi_f32(w):
    return pltpu.bitcast(w & jnp.uint32(0xFFFF0000), F32)


def _pk(a, b):
    return pltpu.pack_elementwise([a, b], packed_dtype=BF)


def _bf(u):
    return pltpu.bitcast(u, BF)


def _lane(shape):
    return jax.lax.broadcasted_iota(jnp.int32, shape, 1)


TM = 256
NCH = S // TM
H = TM // 2
RATE = 2.0
MGAP = 200
L_PRE = 400
L_DS = 500
L_SD = 450
L_POST = 450
AHEAD1 = 2
AHEAD3 = 1
PER3 = 700
MBURST = 256
TDL = 230
XDL = 100
RATE1 = 1.0
PSKIP = 0
DLAT = 260
PDL = 300
DLQ2 = 48
WAVE = [(1, 3), (2, 4), (3, 7), (8, 11)]
HDL = 1
M2AFTER = 88
WWAIT = 61
NSEM = len(WAVE) + 1
PART = "all"
PFFN = "m2"
PN = 30


def _kernel(z_hbm, x_hbm, wr_hbm, wi_hbm, w1_hbm, w2_hbm, gw_hbm, c_hbm, o_hbm,
            x_u, w1_u, w2_u, wr_u, wi_u, wl_v, c_u, xr_v, xi_v, yr_v, yi_v, a_u, bb_v, g_v, o_u,
            z_ref, gw_ref, sems, s_o, *h_u):
    P = functools.partial
    xb, w1b, w2b = x_u.bitcast(BF), w1_u.bitcast(BF), w2_u.bitcast(BF)
    groups = []

    def xrows(r0, n):
        return [(x_hbm.at[0, pl.ds(r0, n), pl.ds(128 * c, 128)], xb.at[c, pl.ds(r0, n)]) for c in range(4)]

    def w1rows(r0, r1):
        r1 = min(r1, F)
        return [(w1_hbm.at[pl.ds(r0, r1 - r0), pl.ds(128 * c, 128)], w1b.at[c, pl.ds(r0, r1 - r0)]) for c in range(4)]

    pa, pb = 0, 0
    for a, b in WAVE:
        pairs = []
        if a > pa:
            pairs += xrows(TM * pa, TM * (a - pa))
        if b > pb:
            pairs += w1rows(128 * pb, 128 * b)
        pa, pb = a, b
        groups.append(pairs)
    groups[0] += [(z_hbm, z_ref), (gw_hbm, gw_ref)]
    rest = [(c_hbm, c_u.bitcast(BF))]
    rest += [(w2_hbm.at[:, pl.ds(128 * c, 128)], w2b.at[c, pl.ds(0, F)]) for c in range(4)]
    for k in range(16):
        rest.append((wr_hbm.at[pl.ds(0, 256), pl.ds(128 * k, 128)], wr_u.bitcast(BF).at[k]))
        rest.append((wi_hbm.at[pl.ds(0, 256), pl.ds(128 * k, 128)], wi_u.bitcast(BF).at[k]))
    rest.append((wr_hbm.at[pl.ds(256, 1), :], wl_v.at[0]))
    rest.append((wi_hbm.at[pl.ds(256, 1), :], wl_v.at[1]))
    groups.append(rest)
    copies = [[pltpu.make_async_copy(s_, d_, sems.at[gi]) for s_, d_ in g] for gi, g in enumerate(groups)]
    for g in copies:
        for cp in g:
            cp.start()
    for c in range(4):
        w2_u[c, pl.ds(F // 2, (FP - F) // 2), :] = jnp.zeros(((FP - F) // 2, 128), U32)

    def wait(gi):
        for cp in copies[gi]:
            cp.wait()
        if gi == 0:
            for c in range(4):
                gwc = jnp.broadcast_to(gw_ref[c:c + 1, :].astype(F32), ((FP - F) // 2, 128))
                w1_u[c, pl.ds(F // 2, (FP - F) // 2), :] = _pk(gwc, gwc)

    fmask_box = {}
    dlq = []

    def gate(v, tok):
        if v.dtype != tok.dtype:
            tok = pltpu.bitcast(tok, v.dtype)
        return jnp.where(fmask_box['m'], tok, v)

    def new_mask():
        dlq.clear()
        z = z_ref[0]
        fmask_box['z'] = z
        fmask_box['m'] = jnp.full((8, 128), z, jnp.int32) != 0

    def oq(k):
        return k + fmask_box['z']

    def gatec(v, tok):
        out = list(v)
        for i in (0, 1):
            (r, sr), (im, si) = v[i]
            out[i] = ((gate(r, tok), sr), (gate(im, tok), si))
        return out

    def cmat(i):
        return _bf(c_u[i])

    def rows8(a, step):
        return [(a[8 * q:8 * q + 8, 0:128], step * q) for q in range(a.shape[0] // 8)]

    state = dict(t=0, nxt=0)

    def push_dl(a, t0, step):
        for v, dt in rows8(a, step):
            dlq.append((v, t0 + dt))

    def lhs(u, dt):
        tok = None
        dlq.sort(key=lambda e: e[1])
        for _ in range(2 if len(dlq) > DLQ2 else 1):
            if dlq and dlq[0][1] <= state['t'] + dt:
                v = pltpu.bitcast(dlq.pop(0)[0], U32)
                tok = v if tok is None else tok | v
        return u if tok is None else gate(u, tok)

    def lhs_par(ops):
        n = ops[0].shape[0] // 8
        g = [[lhs(u[8 * q:8 * q + 8], 16 * q) for u in ops] for q in range(n)]
        return [_bf(jnp.concatenate([g[q][k] for q in range(n)], 0)) for k in range(len(ops))]

    T1s = {}
    Zs = {}

    def p1_pre(n2, gam, tok):
        unp = _hi_f32 if n2 % 2 else _lo_f32
        lo = _lane((8, 128)) < 64
        r0 = n2 // 2 + 64 * gam
        a = [unp(gate(x_u[c, pl.ds(r0, 8, stride=8), :], tok)) for c in range(4)]
        b = [unp(x_u[c, pl.ds(r0 + 512, 8, stride=8), :]) for c in range(4)]
        for e in range(2):
            U = [a[c] + b[c] if e == 0 else a[c] - b[c] for c in range(4)]
            p0, p1_, m0, m1 = U[0] + U[2], U[1] + U[3], U[0] - U[2], U[1] - U[3]
            Pv = jnp.where(lo, m0, (m0 + m1) * (-C8))
            Qn = pltpu.roll(jnp.where(lo, m1, (m1 - m0) * C8), 64, 1)
            for t, val in enumerate([p0 + p1_, p0 - p1_, Pv - Qn, Pv + Qn]):
                if gam % 2 == 0:
                    T1s[n2, t, e, 'a'] = val
                else:
                    pk = _pk(T1s.pop((n2, t, e, 'a')), val)
                    T1s[n2, t, 4 * e + gam // 2] = pk
                    if t >= 2:
                        dlq.append((pk, state['now'] + PDL))

    def p1_d(n2):
        Z = []
        As = lhs_par([c_u[CA + t] for t in range(4)])
        for t in range(4):
            T = _bf(jnp.concatenate([T1s.pop((n2, t, q)) for q in range(8)], 0))
            Z.append(jax.lax.dot_general(As[t], T, NT, preferred_element_type=F32))
        lo = _lane((128, 128)) < 64

        def packed(o):
            return jnp.concatenate([
                _pk(Z[0][o:o + 32], Z[0][o + 32:o + 64]),
                _pk(Z[1][o:o + 32], Z[1][o + 32:o + 64]),
                _pk(Z[2][o:o + 32], Z[3][o:o + 32]),
                _pk(Z[3][o + 32:o + 64], Z[2][o + 32:o + 64])], 0)
        ZRu = packed(0)
        RIu = pltpu.roll(packed(64), 64, 1)
        T0 = jnp.where(lo, ZRu, RIu)
        T1 = jnp.where(lo, RIu, ZRu)
        Zs[n2] = (T0, T1)
        push_dl(T0, state['t'] + DLAT + TDL, 8)
        push_dl(T1, state['t'] + DLAT + TDL, 8)
        return rows8(Z[3], 8), 128

    def p1_s(n2):
        T0, T1 = Zs.pop(n2)
        even = (_lane((128, 128)) % 2) == 0
        xi = []
        Ls = lhs_par([T0[:64], T1[:64], T0[64:], T1[64:]])
        for hf in range(2):
            O0 = jnp.dot(Ls[2 * hf], cmat(CM + 2 * n2), preferred_element_type=F32)
            O1 = jnp.dot(Ls[2 * hf + 1], cmat(CM + 2 * n2 + 1), preferred_element_type=F32)
            xr_v[n2, 128 * hf:128 * hf + 128, :] = jnp.where(even, O0, O1)
            xi.append(pltpu.roll(jnp.where(even, O1, O0), 127, 1))
            xi_v[n2, 128 * hf:128 * hf + 128, :] = xi[-1]
        for q in range(16):
            for hf in range(2):
                dlq.append((xi[hf][8 * q:8 * q + 8], state['t'] + DLAT + XDL + 8 * q))
        return rows8(O1, 8), 128

    def p2_items(grp):
        j, g8 = grp // 8, grp % 8
        jr = JR[j]
        row = pl.ds(8 * grp, 8)
        wrow = pl.ds(16 * g8 + jr // 2, 8, stride=2)
        unp = _hi_f32 if jr % 2 else _lo_f32
        y = [[None] * 4 for _ in range(4)]
        z = [[None] * 4 for _ in range(4)]
        X = [None] * 16
        Y = [None] * 16
        st = {}

        def f1(b, tok):
            v = [((xr_v[oq(4 * a + b), row, :], 1), (xi_v[oq(4 * a + b), row, :], 1)) for a in range(4)]
            o = _dft4(gatec(v, tok), +1)
            for kap in range(4):
                y[kap][b] = _twiddle(o[kap], b * kap, +1)

        def mid_a(kap, tok):
            o = _dft4(gatec(y[kap], tok), +1)
            for io in range(4):
                k = kap + 4 * io
                wr = unp(wr_u[k, wrow, :])
                wi = unp(wi_u[k, wrow, :])
                X[k] = o[io]
                (xr, sr), (xi, si) = o[io]
                Y[k] = (_sub((xr * wr, sr), (xi * wi, si)), _add((xr * wi, sr), (xi * wr, si)))

        def mid_b(kap):
            o2 = _dft4([Y[kap + 4 * io] for io in range(4)], -1)
            for b2 in range(4):
                z[b2][kap] = _twiddle(o2[b2], kap * b2, -1)

        def mid(kap, tok):
            mid_a(kap, tok)
            mid_b(kap)

        def i2(b2, tok):
            o = _dft4(gatec(z[b2], tok), -1)
            for io in range(4):
                yr_v[b2 + 4 * io, row, :] = _force(o[io][0])
                yi_v[b2 + 4 * io, row, :] = _force(o[io][1])

        def sp_stack(k, tok):
            sub = jax.lax.broadcasted_iota(jnp.int32, (8, 128), 0)
            w0r = unp(wr_u[k, wrow, :])[0:1]
            w0i = unp(wi_u[k, wrow, :])[0:1]
            wlr = wl_v[0, :, 128 * k:128 * k + 128].astype(F32)
            wli = wl_v[1, :, 128 * k:128 * k + 128].astype(F32)
            pr = gate(_force(X[k][0]), tok)[0:1]
            pi = _force(X[k][1])[0:1]
            blk = jnp.zeros((8, 128), F32)
            for jj, r in enumerate([pr, pi, w0r, w0i, wlr, wli]):
                blk = jnp.where(sub == jj, jnp.broadcast_to(r, (8, 128)), blk)
            st[k] = blk

        def sp_flip():
            full = jnp.concatenate([st[k] for k in range(16)], 0)
            fl = []
            for hf in range(2):
                part = full[64 * hf:64 * hf + 64]
                hi_ = part.astype(BF)
                lo_ = (part - hi_.astype(F32)).astype(BF)
                fh = jnp.dot(hi_, cmat(CJ), preferred_element_type=F32)
                fl.append(jnp.dot(lo_, cmat(CJ), preferred_element_type=F32) + fh)
            fl = jnp.concatenate(fl, 0)
            st['fl'] = fl
            return rows8(fl, 4), 64

        def sp_fix(k, tok):
            sub = jax.lax.broadcasted_iota(jnp.int32, (8, 128), 0)
            fl = st['fl']
            fa = fl[8 * (15 - k):8 * (15 - k) + 8]
            fb = fl[8 * ((16 - k) % 16):8 * ((16 - k) % 16) + 8]
            f = gate(jnp.where(_lane((8, 128)) == 0, fb, fa), tok)
            o = st[k]
            pr, pi, w0r, w0i, wlr, wli = [o[jj:jj + 1] for jj in range(6)]
            fpr, fpi, f0r, f0i, flr, fli = [f[jj:jj + 1] for jj in range(6)]
            s0r, s0i = w0r + f0r, w0i - f0i
            slr, sli = wlr + flr, wli - fli
            Ar, Ai_ = (s0r + slr) * 0.25, (s0i + sli) * 0.25
            Br, Bi = (s0r - slr) * 0.25, (s0i - sli) * 0.25
            yr0 = pr * Ar - pi * Ai_ + fpr * Br + fpi * Bi
            yi0 = pr * Ai_ + pi * Ar + fpr * Bi - fpi * Br
            yr = jnp.where(sub == 0, jnp.broadcast_to(yr0, (8, 128)), _force(Y[k][0]))
            yi = jnp.where(sub == 0, jnp.broadcast_to(yi0, (8, 128)), _force(Y[k][1]))
            Y[k] = ((yr, 1), (yi, 1))
            dlq.append((yr, state['t'] + 400))
            dlq.append((yi, state['t'] + 400))
            if k >= 12:
                mid_b(k - 12)

        first = [('v', P(f1, b), 30) for b in range(4)]
        last = [('v', P(i2, b), 20) for b in range(4)]
        if grp != 0:
            return first + [('v', P(mid, k), 78) for k in range(4)] + last, []
        a = (first + [('v', P(mid_a, k), 52) for k in range(4)] + [('v', P(sp_stack, k), 24) for k in range(16)]
             + [('m', sp_flip, 64)])
        b = [('v', P(sp_fix, k), 50 + (26 if k >= 12 else 0)) for k in range(16)] + last
        return a, b

    B3 = {}
    V3 = {}

    def p3_pre(n2, q, tok):
        hf, o = q // 2, 32 * (q % 2)
        even = (_lane((32, 128)) % 2) == 0

        def packed(ref):
            a = ref[oq(n2), 128 * hf + o:128 * hf + o + 32, :]
            b = ref[oq(n2), 128 * hf + 64 + o:128 * hf + 64 + o + 32, :]
            a = jnp.concatenate([gate(a[8 * i:8 * i + 8], tok) for i in range(4)], 0)
            return _pk(a, b)
        Ru = packed(yr_v)
        Ou = pltpu.roll(packed(yi_v), 1, 1)
        B3[n2, 0, q] = jnp.where(even, Ru, Ou)
        B3[n2, 1, q] = jnp.where(even, Ou, Ru)
        push_dl(B3[n2, 0, q], state['now'] + PDL, 4)

    def p3_s(n2):
        V = []
        Ms_ = lhs_par([c_u[CM + 2 * n2 + e] for e in range(2)])
        for e in range(2):
            B = _bf(jnp.concatenate([B3.pop((n2, e, q)) for q in range(4)], 0))
            V.append(jax.lax.dot_general(Ms_[e], B, NT, preferred_element_type=F32))
        l64 = _lane((64, 128))
        masks = [(l64 % 2) == 0, ((l64 + 1) % 4) < 2]
        V0, V1 = V
        V0r, V0i = V0[:64], V0[64:]
        V1i, V1r = V1[:64], V1[64:]
        VR = _pk(V0r + V1r, V0r - V1r)
        VI = _pk(V0i + V1i, V0i - V1i)
        G = []
        for h in range(2):
            r = VR[:, 128 * h:128 * h + 128]
            ri = pltpu.roll(VI[:, 128 * h:128 * h + 128], 1 + h, 1)
            G += [jnp.where(masks[h], r, ri), jnp.where(masks[h], ri, r)]
        for g in G:
            push_dl(g, state['t'] + DLAT + 64, 8)
        V3[n2] = G
        return rows8(V[1], 8), 128

    def p3_d(r0):
        Gs = [V3.pop(2 * r0), V3.pop(2 * r0 + 1)]
        Gl = lhs_par([jnp.concatenate([Gs[s][t][8 * q:8 * q + 8] for q in range(8) for s in range(2)], 0)
                      for t in range(4)])
        o = [jnp.dot(Gl[t], cmat(CAI + t), preferred_element_type=F32) for t in range(4)]
        v0, v2, T1, T3 = o
        lo = _lane((256, 128)) < 64
        Pp = T1 + T3
        Qp = pltpu.roll(T1 - T3, 64, 1)
        m0 = jnp.where(lo, Pp, (Qp - Pp) * C8)
        m1n = jnp.where(lo, Qp, (Pp + Qp) * C8)
        p0, p1_ = v0 + v2, v0 - v2
        y = [p0 + m0, p1_ - m1n, p0 - m0, p1_ + m1n]
        for q in range(8):
            for c in range(4):
                pk = _pk(y[c][32 * q:32 * q + 16], y[c][32 * q + 16:32 * q + 32])
                a_u[c, pl.ds(r0 + 128 * q, 16, stride=8), :] = pk
                dlq.append((pk[0:8], state['t'] + DLAT + 32 * q + 32))
                dlq.append((pk[8:16], state['t'] + DLAT + 32 * q + 32))
        return [], 256

    def m1(i, j):
        r, r2 = i * TM, i * H
        xs = [[lhs(x_u[c, pl.ds(r2 + 8 * q, 8), :], 16 * q) for c in range(4)] for q in range(H // 8)]
        xc = jnp.concatenate([_bf(jnp.concatenate([xq[c] for xq in xs], 0)) for c in range(4)], 1)
        w1 = jnp.concatenate([_bf(w1_u[c, pl.ds(64 * j, 64), :]) for c in range(4)], 1)
        t = 0.5 * jax.lax.dot_general(xc, w1, NT, preferred_element_type=F32)
        th = jnp.tanh(t)
        if j == 10:
            g = 0.5 + jnp.broadcast_to(0.5 * th[:, 127:128], (TM, 128))
            g_v[pl.ds(r, TM), :] = g
            push_dl(g, state['t'] + DLAT + 64, 8)
        hs = t + t * th
        hp = _pk(hs[:H], hs[H:])
        h_u[i][j] = hp
        if HDL:
            push_dl(hp, state['t'] + DLAT + H, 8)
        return rows8(t, 8), TM

    accs = {}

    def m2(i, g):
        cj = [divmod(f, 11) for f in range(4 * g, 4 * g + 4)]
        hq = [[lhs(h_u[i][oq(j), pl.ds(8 * q, 8), :], 16 * q) for _, j in cj] for q in range(H // 8)]
        fin = []
        for c in sorted(set(c for c, _ in cj)):
            ks = [k for k in range(4) if cj[k][0] == c]
            j0 = cj[ks[0]][1]
            hs = jnp.concatenate([_bf(jnp.concatenate([hq_[k] for hq_ in hq], 0)) for k in ks], 1)
            o = jnp.dot(hs, _bf(w2_u[c, pl.ds(64 * j0, 64 * len(ks)), :]), preferred_element_type=F32)
            acc = o if j0 == 0 else o + accs.pop((i, c))
            if j0 + len(ks) < 11:
                accs[i, c] = acc
            else:
                bb_v[c, pl.ds(i * TM, TM), :] = acc
                fin.append(c)
        return rows8(acc, 8), TM, fin

    def out_copy(i, c):
        return pltpu.make_async_copy(o_u.bitcast(BF).at[c, pl.ds(128 * i, 128)],
                                     o_hbm.at[0, pl.ds(128 * i, 128), pl.ds(128 * c, 128)], s_o.at[0])

    def combine(i, c, tok):
        h, n0 = i // 8, 8 * (i % 8)
        base = (128 * i // TM) * TM
        outs = []
        for n in range(8):
            s0 = 128 * i + 16 * n
            q0 = s0 - base
            b0 = base + (2 * q0 if q0 < H else 2 * (q0 - H) + 1)
            au = a_u[c, pl.ds(16 * _POS_OF_N1[n0 + n] + 8 * h, 8), :]
            if tok is not None:
                au = gate(au, tok)
            ge = g_v[pl.ds(s0, 8, stride=2), :]
            go = g_v[pl.ds(s0 + 1, 8, stride=2), :]
            be = bb_v[c, pl.ds(b0, 8, stride=4), :]
            bo = bb_v[c, pl.ds(b0 + 2, 8, stride=4), :]
            outs.append(_pk(be + ge * (_lo_f32(au) - be), bo + go * (_hi_f32(au) - bo)))
        o_u[c, pl.ds(64 * i, 64), :] = jnp.concatenate(outs, 0)
        out_copy(i, c).start()

    VQ, MQ = [], []
    if PART in ('all', 'p1'):
        for r0 in range(8):
            for n2 in (2 * r0, 2 * r0 + 1):
                for gam in range(8):
                    deps = [('rest', 0)] + ([(('d1', 2 * (r0 - AHEAD1)), 0)] if r0 >= AHEAD1 else [])
                    VQ.append((('pre1', n2, gam), P(p1_pre, n2, gam), 58 * RATE / RATE1, deps))
        for r0 in range(9):
            if r0 < 8:
                for n2 in (2 * r0, 2 * r0 + 1):
                    MQ.append((('d1', n2), P(p1_d, n2), [(('pre1', n2, 7), L_PRE)]))
            if r0 > 0:
                for n2 in (2 * r0 - 2, 2 * r0 - 1):
                    MQ.append((('s1', n2), P(p1_s, n2), [(('d1', n2), L_DS)]))
    if PART in ('all', 'p2'):
        kp = [0]

        def add2(items, extra=()):
            for it in items:
                kp[0] += 1
                deps = [('rest', 0)] + list(extra) + ([(('s1', 15), L_POST)] if PART == 'all' else [])
                if it[0] == 'v':
                    VQ.append((('p2', kp[0]), it[1], it[2], deps))
                else:
                    MQ.append(('flip', it[1], [(('p2', kp[0] - 1), L_PRE)]))
        a0, b0 = p2_items(0)
        add2(a0)
        for g in range(1, 4):
            add2(p2_items(g)[0])
        add2(b0, [('flip', 250)])
        for g in range(4, 32):
            add2(p2_items(g)[0])
    if PART in ('all', 'p3'):
        last2 = [(VQ[-1][0], 100)] if PART == 'all' else []
        for r0 in range(8):
            for n2 in (2 * r0, 2 * r0 + 1):
                for q in range(4):
                    deps = [('rest', 0)] + last2 + ([(('s3', 2 * (r0 - AHEAD3)), 0)] if r0 >= AHEAD3 else [])
                    VQ.append((('pre3', n2, q), P(p3_pre, n2, q), 40, deps))
        for r0 in range(9):
            if r0 < 8:
                for n2 in (2 * r0, 2 * r0 + 1):
                    deps = [(('pre3', n2, 3), L_PRE)] + ([(('s3', n2 - 2), PER3)] if r0 > 0 else [])
                    MQ.append((('s3', n2), P(p3_s, n2), deps))
            if r0 > 0:
                MQ.append((('d3', r0 - 1), P(p3_d, r0 - 1), [(('s3', 2 * r0 - 1), L_SD)]))
    if PART == 'all':
        for i in range(NCH):
            for c in range(4):
                for ii in range(TM // 128):
                    VQ.append((('cmb', i, c, ii), P(combine, (TM // 128) * i + ii, c), 80,
                               [(('d3', 7), L_POST + 256), (('m2', i, c), 0)]))

    m1s = []
    seen = set()
    for wv, (a, b) in enumerate(WAVE):
        for i in range(a):
            for j in range(b):
                if (i, j) not in seen:
                    seen.add((i, j))
                    m1s.append((wv, i, j))
    m2s = [(i, g) for i in range(NCH) for g in range(11)]
    pieces = []
    done1 = set()
    k1 = k2 = 0
    while k1 < len(m1s) or k2 < len(m2s):
        ready2 = k2 < len(m2s) and all((m2s[k2][0], j) in done1 for j in range(11)) and k1 >= M2AFTER
        if ready2 or k1 >= len(m1s):
            pieces.append(('m2',) + m2s[k2])
            k2 += 1
        else:
            pieces.append(('m1',) + m1s[k1])
            done1.add(m1s[k1][1:])
            k1 += 1

    done = set()
    if PART != 'all':
        pieces = [p_ for p_ in pieces if p_[0] == PFFN][PSKIP:PSKIP + PN]
        for gi in range(len(WAVE) + 1):
            wait(gi)
        new_mask()
        done.add('rest')
        state['nxt'] = 0

    when = {}
    if PART != 'all':
        when['rest'] = 0

    def ok(deps, now):
        return all(d in when and when[d] + dl <= now for d, dl in deps)

    def issue(toks, cost):
        for tok, dt in toks:
            now = state['t'] + dt
            if VQ and now >= state['nxt'] and ok(VQ[0][3], now):
                name, fn, ops, _ = VQ.pop(0)
                state['now'] = now
                fn(tok)
                when[name] = now
                state['nxt'] = max(state['nxt'], now - 8) + ops / RATE
        state['t'] += cost

    def try_mxu():
        t0 = state['t']
        while MQ and ok(MQ[0][2], state['t']) and state['t'] - t0 < MBURST:
            name, fn, _ = MQ.pop(0)
            when[name] = state['t']
            issue(*fn())

    wv_done = -1 if PART == 'all' else 99
    log = []
    for n, pc in enumerate(pieces):
        if pc[0] == 'm1' and pc[1] > wv_done:
            wv_done = pc[1]
            wait(wv_done)
            new_mask()
            log.append(('wait', wv_done, state['t']))
        if 'rest' not in done and (n >= WWAIT or pc[0] == 'm2'):
            wait(len(WAVE))
            new_mask()
            done.add('rest')
            when['rest'] = state['t']
            log.append(('wait rest', state['t']))
        try_mxu()
        if pc[0] == 'm1':
            issue(*m1(pc[2], pc[3]))
        else:
            toks, cost, fin = m2(pc[1], pc[2])
            issue(toks, cost)
            for c in fin:
                when['m2', pc[1], c] = state['t']
    assert not MQ
    for it in VQ:
        assert it[0][0] == 'cmb', it[0]
        it[1](None)
    if PART != 'all':
        z = pl.multiple_of(z_ref[0] * 8, 8)
        acc = a_u[z, pl.ds(z, 8), :]
        for r in (bb_v, xr_v, xi_v, yr_v, yi_v) + tuple(h_u):
            acc = acc | pltpu.bitcast(r[z, pl.ds(z, 8), :], U32)
        acc = acc | pltpu.bitcast(g_v[pl.ds(z, 8), :], U32)
        o_u[0, 0:8, :] = acc
        out_copy(0, 0).start()
        out_copy(0, 0).wait()
        return
    for i in range(16):
        for c in range(4):
            out_copy(i, c).wait()


@jax.jit
def pallas_gated_mix__spectral_gfnet__dense_activation_silu__prompt_kernel(A_x, A_w_r, A_w_i, B_x, B_w1, B_w2, gate_w):
    consts = jnp.asarray(_consts(), dtype=BF)
    zero = jnp.zeros((1,), jnp.int32)
    hbm = pl.BlockSpec(memory_space=pltpu.HBM)
    vmem = pl.BlockSpec(memory_space=pltpu.VMEM)
    smem = pl.BlockSpec(memory_space=pltpu.SMEM)
    dma = pltpu.SemaphoreType.DMA
    return pl.pallas_call(
        _kernel,
        in_specs=[hbm] * 8,
        out_specs=hbm,
        out_shape=jax.ShapeDtypeStruct((1, S, D), BF),
        scratch_shapes=[
            pltpu.VMEM((4, S // 2, 128), U32),
            pltpu.VMEM((4, FP // 2, 128), U32),
            pltpu.VMEM((4, FP // 2, 128), U32),
            pltpu.VMEM((16, 128, 128), U32),
            pltpu.VMEM((16, 128, 128), U32),
            pltpu.VMEM((2, 1, S), BF),
            pltpu.VMEM((NCONST, 64, 128), U32),
            pltpu.VMEM((16, 256, 128), F32),
            pltpu.VMEM((16, 256, 128), F32),
            pltpu.VMEM((16, 256, 128), F32),
            pltpu.VMEM((16, 256, 128), F32),
            pltpu.VMEM((4, S // 2, 128), U32),
            pltpu.VMEM((4, S, 128), F32),
            pltpu.VMEM((S, 128), F32),
            pltpu.VMEM((4, S // 2, 128), U32),
            pltpu.SMEM((1,), jnp.int32),
            pltpu.VMEM((4, 128), BF),
            dma((NSEM,)), dma((1,)),
        ] + [pltpu.VMEM((11, H, 128), U32) for _ in range(NCH)],
        compiler_params=pltpu.CompilerParams(vmem_limit_bytes=100 << 20),
    )(zero, A_x, A_w_r.T, A_w_i.T, B_w1.T, B_w2, gate_w.reshape(4, 128), consts)
```

```python
import functools
import numpy as np
import jax
import jax.numpy as jnp
import jax.experimental.pallas as pl
import jax.experimental.pallas.tpu as pltpu

S, D, F = 2048, 512, 1376
FP = 1408
RES = (0, 4, 2, 6, 1, 7, 5, 3)
JR = (0, 2, 1, 3)
BF = jnp.bfloat16
F32 = jnp.float32
U32 = jnp.uint32
C8 = float(np.sqrt(0.5))
NT = (((1,), (1,)), ((), ()))


def _kd_of_row(rho):
    return 8 * (rho % 32) + RES[rho // 32]


def _n1_of_pos(p):
    return 8 * (2 * (p // 16) + p % 2) + (p % 16) // 2


_POS_OF_N1 = {_n1_of_pos(p): p for p in range(64)}


@functools.lru_cache(maxsize=None)
def _consts():
    l = np.arange(128)
    A = np.zeros((4, 128, 128))
    where = {}
    for t in range(4):
        for i in range(64):
            rho = 64 * t + i
            kd = _kd_of_row(rho)
            where[kd] = (t, i)
            if t < 2:
                ang = 2 * np.pi * ((l * kd) % 512) / 512
                A[t, i] = np.cos(ang)
                A[t, 64 + i] = -np.sin(ang)
                if rho == 0:
                    A[t, 64] = np.where(l % 2 == 0, 1.0, -1.0)
            else:
                f = t - 2
                lp = np.arange(64)
                k, cj = (kd, 1.0) if kd % 8 == 1 + 4 * f else (512 - kd, -1.0)
                ang = 2 * np.pi * ((lp * k) % 512) / 512
                c, s = np.cos(ang), -np.sin(ang)
                sg = 1.0 if f == 0 else -1.0
                A[t, i, :64] = c
                A[t, i, 64:] = -s * sg
                A[t, 64 + i, :64] = cj * s
                A[t, 64 + i, 64:] = cj * c * sg
    Ai = np.zeros((4, 128, 128))
    for half in range(2):
        sh = 1 + half
        for lam in range(128):
            kd = 2 * lam + half
            t, i = where[kd]
            sc = (1.0 if kd == 0 else 2.0) / (S * D)
            Ai[t, lam] = A[t, i] * sc
            Ai[t, (lam + sh) % 128] = A[t, 64 + i] * sc
    Ms = np.zeros((16, 2, 128, 128))
    n1 = np.array([_n1_of_pos(p) for p in range(64)])[:, None]
    k1 = np.arange(64)[None, :]
    for e in range(2):
        for n2 in range(16):
            ang = 2 * np.pi * (((16 * n1 + n2) * (e + 2 * k1)) % 2048) / 2048
            c, s = np.cos(ang), -np.sin(ang)
            re_cols = 2 * np.arange(64) + e
            im_cols = (2 * np.arange(64) + 1 + e) % 128
            M = np.zeros((128, 128))
            rr = slice(0, 64) if e == 0 else slice(64, 128)
            ir = slice(64, 128) if e == 0 else slice(0, 64)
            M[rr, re_cols] = c
            M[ir, re_cols] = -s
            M[rr, im_cols] = s
            M[ir, im_cols] = c
            Ms[n2, e] = M
    J = np.zeros((1, 128, 128))
    J[0, l, (128 - l) % 128] = 1.0
    allc = np.concatenate([A, Ai, J, Ms.reshape(32, 128, 128)], 0)
    return allc.astype(np.float32)


CA, CAI, CJ, CM = 0, 4, 8, 9
NCONST = 41


def _add(a, b):
    (x, sx), (y, sy) = a, b
    if sx == sy:
        return (x + y, sx)
    return (x - y, 1) if sx > 0 else (y - x, 1)


def _neg(a):
    return (a[0], -a[1])


def _sub(a, b):
    return _add(a, _neg(b))


def _scale(a, c):
    return (a[0] * (c * a[1]), 1)


def _cadd(a, b):
    return (_add(a[0], b[0]), _add(a[1], b[1]))


def _csub(a, b):
    return (_sub(a[0], b[0]), _sub(a[1], b[1]))


def _mul_mi(a, sgn):
    re, im = a
    return (im, _neg(re)) if sgn > 0 else (_neg(im), re)


def _twiddle(a, j, sgn):
    j = j % 16
    if j % 4 == 0:
        for _ in range(j // 4):
            a = _mul_mi(a, sgn)
        return a
    re, im = a
    if j % 2 == 0:
        if sgn > 0:
            r = _scale(_add(re, im), C8)
            i = _scale(_sub(im, re), C8)
        else:
            r = _scale(_sub(re, im), C8)
            i = _scale(_add(im, re), C8)
        a = (r, i)
        for _ in range(j // 4):
            a = _mul_mi(a, sgn)
        return a
    c = float(np.cos(2 * np.pi * j / 16))
    s = float(-sgn * np.sin(2 * np.pi * j / 16))
    r = _sub(_scale(re, c), _scale(im, s))
    i = _add(_scale(re, s), _scale(im, c))
    return (r, i)


def _dft4(v, sgn):
    a, b, c, d = v
    t0, t1 = _cadd(a, c), _csub(a, c)
    t2, t3 = _cadd(b, d), _mul_mi(_csub(b, d), sgn)
    return [_cadd(t0, t2), _cadd(t1, t3), _csub(t0, t2), _csub(t1, t3)]


def _dft16(v, sgn):
    y = [[None] * 4 for _ in range(4)]
    for b in range(4):
        o = _dft4([v[4 * a + b] for a in range(4)], sgn)
        for kap in range(4):
            y[kap][b] = _twiddle(o[kap], b * kap, sgn)
    out = [None] * 16
    for kap in range(4):
        o = _dft4(y[kap], sgn)
        for io in range(4):
            out[kap + 4 * io] = o[io]
    return out


def _force(a):
    return a[0] if a[1] > 0 else -a[0]


def _lo_f32(w):
    return pltpu.bitcast(w << 16, F32)


def _hi_f32(w):
    return pltpu.bitcast(w & jnp.uint32(0xFFFF0000), F32)


def _pk(a, b):
    half = jnp.uint32(0x8000)
    lo = (pltpu.bitcast(a, U32) + half) >> 16
    hi = (pltpu.bitcast(b, U32) + half) & jnp.uint32(0xFFFF0000)
    return lo | hi


def _bf(u):
    return pltpu.bitcast(u, BF)


def _lane(shape):
    return jax.lax.broadcasted_iota(jnp.int32, shape, 1)


TM = 256
NCH = S // TM
H = TM // 2
RATE = 2.0
L_PRE = 400
L_DS = 500
L_SD = 450
L_POST = 450
AHEAD1 = 2
AHEAD3 = 1
PER3 = 700
PRE3D = 200
C3 = 72
MBURST = 256
TDL = 230
XDL = 100
RATE1 = 1.0
DLAT = 260
PDL = 300
DLQ2 = 48
KA, KB = (4, 8)
KWAVE = [(0,), (1, 2), (3,)]
KMIX = 4
WAVE = KWAVE
WWAIT = 63
NSEM = len(WAVE) + 1
AP = 136
CCOST = 160


def _kernel(z_hbm, x_hbm, wr_hbm, wi_hbm, w1_hbm, w2_hbm, gw_hbm, c_hbm, o_hbm,
            x_u, w1_u, w2_u, wr_u, wi_u, wl_v, c_u, xr_v, xi_v, yr_v, yi_v, a_v, bb_v, g_v, o_v, p_v,
            z_ref, gw_ref, sems, s_o, *h_u):
    P = functools.partial
    xb, w1b, w2b = x_u.bitcast(BF), w1_u.bitcast(BF), w2_u.bitcast(BF)
    groups = []

    def xrows(r0, r1, cs):
        return [(x_hbm.at[0, pl.ds(r0, r1 - r0), pl.ds(128 * c, 128)], xb.at[c, pl.ds(r0, r1 - r0)]) for c in cs]

    def w1rows(r0, r1, cs):
        return [(w1_hbm.at[pl.ds(r0, r1 - r0), pl.ds(128 * c, 128)], w1b.at[c, pl.ds(r0, r1 - r0)]) for c in cs]

    for cs in KWAVE:
        groups.append([p_ for c in cs for p_ in xrows(0, KA * TM, [c]) + w1rows(0, KB * 128, [c])])
    groups[-1] += w1rows(KB * 128, F, range(4)) + xrows(KA * TM, S, range(4))
    groups[0].append((z_hbm, z_ref))
    groups[-1].append((gw_hbm, gw_ref))
    rest = [(c_hbm, c_u.bitcast(BF))]
    rest += [(w2_hbm.at[:, pl.ds(128 * c, 128)], w2b.at[c, pl.ds(0, F)]) for c in range(4)]
    for k in range(16):
        rest.append((wr_hbm.at[pl.ds(0, 256), pl.ds(128 * k, 128)], wr_u.bitcast(BF).at[k]))
        rest.append((wi_hbm.at[pl.ds(0, 256), pl.ds(128 * k, 128)], wi_u.bitcast(BF).at[k]))
    rest.append((wr_hbm.at[pl.ds(256, 1), :], wl_v.at[0]))
    rest.append((wi_hbm.at[pl.ds(256, 1), :], wl_v.at[1]))
    groups.append(rest)
    copies = [[pltpu.make_async_copy(s_, d_, sems.at[gi]) for s_, d_ in g] for gi, g in enumerate(groups)]
    for g in copies:
        for cp in g:
            cp.start()

    def wait(gi):
        for cp in copies[gi]:
            cp.wait()
        if gi == len(WAVE) - 1:
            for c in range(4):
                gwc = jnp.broadcast_to(gw_ref[c:c + 1, :].astype(F32), ((FP - F) // 2, 128))
                w1_u[c, pl.ds(F // 2, (FP - F) // 2), :] = _pk(gwc, gwc)
        if gi == len(WAVE):
            for c in range(4):
                w2_u[c, pl.ds(F // 2, (FP - F) // 2), :] = jnp.zeros(((FP - F) // 2, 128), U32)

    fmask_box = {}
    dlq = []

    def gate(v, tok):
        if v.dtype != tok.dtype:
            tok = pltpu.bitcast(tok, v.dtype)
        return jnp.where(fmask_box['m'], tok, v)

    def new_mask():
        dlq.clear()
        z = z_ref[0]
        fmask_box['z'] = z
        fmask_box['m'] = jnp.full((8, 128), z, jnp.int32) != 0

    def oq(k, n):
        return jnp.clip(k + fmask_box['z'], 0, n - 1)

    def gatec(v, tok):
        out = list(v)
        for i in (0, 1):
            (r, sr), (im, si) = v[i]
            out[i] = ((gate(r, tok), sr), (gate(im, tok), si))
        return out

    def cmat(i):
        return _bf(c_u[i])

    def rows8(a, step):
        return [(a[8 * q:8 * q + 8, 0:128], step * q) for q in range(a.shape[0] // 8)]

    state = dict(t=0, nxt=0)

    def push_dl(a, t0, step):
        for v, dt in rows8(a, step):
            dlq.append((v, t0 + dt))

    def lhs(u, dt):
        tok = None
        dlq.sort(key=lambda e: e[1])
        for _ in range(2 if len(dlq) > DLQ2 else 1):
            if dlq and dlq[0][1] <= state['t'] + dt:
                v = pltpu.bitcast(dlq.pop(0)[0], U32)
                tok = v if tok is None else tok | v
        return u if tok is None else gate(u, tok)

    def lhs_par(ops):
        n = ops[0].shape[0] // 8
        g = [[lhs(u[8 * q:8 * q + 8], 16 * q) for u in ops] for q in range(n)]
        return [_bf(jnp.concatenate([g[q][k] for q in range(n)], 0)) for k in range(len(ops))]

    T1s = {}
    Zs = {}

    def p1_pre(n2, gam, tok):
        unp = _hi_f32 if n2 % 2 else _lo_f32
        lo = _lane((8, 128)) < 64
        r0 = n2 // 2 + 64 * gam
        a = [unp(gate(x_u[c, pl.ds(r0, 8, stride=8), :], tok)) for c in range(4)]
        b = [unp(x_u[c, pl.ds(r0 + 512, 8, stride=8), :]) for c in range(4)]
        for e in range(2):
            U = [a[c] + b[c] if e == 0 else a[c] - b[c] for c in range(4)]
            p0, p1_, m0, m1 = U[0] + U[2], U[1] + U[3], U[0] - U[2], U[1] - U[3]
            Pv = jnp.where(lo, m0, (m0 + m1) * (-C8))
            Qn = pltpu.roll(jnp.where(lo, m1, (m1 - m0) * C8), 64, 1)
            for t, val in enumerate([p0 + p1_, p0 - p1_, Pv - Qn, Pv + Qn]):
                if gam % 2 == 0:
                    T1s[n2, t, e, 'a'] = val
                else:
                    pk = _pk(T1s.pop((n2, t, e, 'a')), val)
                    T1s[n2, t, 4 * e + gam // 2] = pk
                    if t >= 2:
                        dlq.append((pk, state['now'] + PDL))

    def p1_d(n2):
        Z = []
        As = lhs_par([c_u[CA + t] for t in range(4)])
        for t in range(4):
            T = _bf(jnp.concatenate([T1s.pop((n2, t, q)) for q in range(8)], 0))
            Z.append(jax.lax.dot_general(As[t], T, NT, preferred_element_type=F32))
        lo = _lane((128, 128)) < 64

        def packed(o):
            return jnp.concatenate([
                _pk(Z[0][o:o + 32], Z[0][o + 32:o + 64]),
                _pk(Z[1][o:o + 32], Z[1][o + 32:o + 64]),
                _pk(Z[2][o:o + 32], Z[3][o:o + 32]),
                _pk(Z[3][o + 32:o + 64], Z[2][o + 32:o + 64])], 0)
        ZRu = packed(0)
        RIu = pltpu.roll(packed(64), 64, 1)
        T0 = jnp.where(lo, ZRu, RIu)
        T1 = jnp.where(lo, RIu, ZRu)
        Zs[n2] = (T0, T1)
        push_dl(T0, state['t'] + DLAT + TDL, 8)
        push_dl(T1, state['t'] + DLAT + TDL, 8)
        return rows8(Z[3], 8), 128

    def p1_s(n2):
        T0, T1 = Zs.pop(n2)
        even = (_lane((128, 128)) % 2) == 0
        xi = []
        Ls = lhs_par([T0[:64], T1[:64], T0[64:], T1[64:]])
        for hf in range(2):
            O0 = jnp.dot(Ls[2 * hf], cmat(CM + 2 * n2), preferred_element_type=F32)
            O1 = jnp.dot(Ls[2 * hf + 1], cmat(CM + 2 * n2 + 1), preferred_element_type=F32)
            xr_v[n2, 128 * hf:128 * hf + 128, :] = jnp.where(even, O0, O1)
            xi.append(pltpu.roll(jnp.where(even, O1, O0), 127, 1))
            xi_v[n2, 128 * hf:128 * hf + 128, :] = xi[-1]
        for q in range(16):
            for hf in range(2):
                dlq.append((xi[hf][8 * q:8 * q + 8], state['t'] + DLAT + XDL + 8 * q))
        return rows8(O1, 8), 128

    def p2_items(grp):
        j, g8 = grp // 8, grp % 8
        jr = JR[j]
        row = pl.ds(8 * grp, 8)
        wrow = pl.ds(16 * g8 + jr // 2, 8, stride=2)
        unp = _hi_f32 if jr % 2 else _lo_f32
        y = [[None] * 4 for _ in range(4)]
        z = [[None] * 4 for _ in range(4)]
        X = [None] * 16
        Y = [None] * 16
        st = {}

        def f1(b, tok):
            v = [((xr_v[oq(4 * a + b, 16), row, :], 1), (xi_v[oq(4 * a + b, 16), row, :], 1)) for a in range(4)]
            o = _dft4(gatec(v, tok), +1)
            for kap in range(4):
                y[kap][b] = _twiddle(o[kap], b * kap, +1)

        def mid_a(kap, tok):
            o = _dft4(gatec(y[kap], tok), +1)
            for io in range(4):
                k = kap + 4 * io
                wr = unp(wr_u[k, wrow, :])
                wi = unp(wi_u[k, wrow, :])
                X[k] = o[io]
                (xr, sr), (xi, si) = o[io]
                Y[k] = (_sub((xr * wr, sr), (xi * wi, si)), _add((xr * wi, sr), (xi * wr, si)))

        def mid_b(kap):
            o2 = _dft4([Y[kap + 4 * io] for io in range(4)], -1)
            for b2 in range(4):
                z[b2][kap] = _twiddle(o2[b2], kap * b2, -1)

        def mid(kap, tok):
            mid_a(kap, tok)
            mid_b(kap)

        def i2(b2, tok):
            o = _dft4(gatec(z[b2], tok), -1)
            for io in range(4):
                yr_v[b2 + 4 * io, row, :] = _force(o[io][0])
                yi_v[b2 + 4 * io, row, :] = _force(o[io][1])

        def sp_stack(k, tok):
            sub = jax.lax.broadcasted_iota(jnp.int32, (8, 128), 0)
            w0r = unp(wr_u[k, wrow, :])[0:1]
            w0i = unp(wi_u[k, wrow, :])[0:1]
            wlr = wl_v[0, :, 128 * k:128 * k + 128].astype(F32)
            wli = wl_v[1, :, 128 * k:128 * k + 128].astype(F32)
            pr = gate(_force(X[k][0]), tok)[0:1]
            pi = _force(X[k][1])[0:1]
            blk = jnp.zeros((8, 128), F32)
            for jj, r in enumerate([pr, pi, w0r, w0i, wlr, wli]):
                blk = jnp.where(sub == jj, jnp.broadcast_to(r, (8, 128)), blk)
            st[k] = blk

        def sp_flip():
            full = jnp.concatenate([st[k] for k in range(16)], 0)
            fl = []
            for hf in range(2):
                part = full[64 * hf:64 * hf + 64]
                hi_ = part.astype(BF)
                lo_ = (part - hi_.astype(F32)).astype(BF)
                fh = jnp.dot(hi_, cmat(CJ), preferred_element_type=F32)
                fl.append(jnp.dot(lo_, cmat(CJ), preferred_element_type=F32) + fh)
            fl = jnp.concatenate(fl, 0)
            st['fl'] = fl
            return rows8(fl, 4), 64

        def sp_fix(k, tok):
            sub = jax.lax.broadcasted_iota(jnp.int32, (8, 128), 0)
            fl = st['fl']
            fa = fl[8 * (15 - k):8 * (15 - k) + 8]
            fb = fl[8 * ((16 - k) % 16):8 * ((16 - k) % 16) + 8]
            f = gate(jnp.where(_lane((8, 128)) == 0, fb, fa), tok)
            o = st[k]
            pr, pi, w0r, w0i, wlr, wli = [o[jj:jj + 1] for jj in range(6)]
            fpr, fpi, f0r, f0i, flr, fli = [f[jj:jj + 1] for jj in range(6)]
            s0r, s0i = w0r + f0r, w0i - f0i
            slr, sli = wlr + flr, wli - fli
            Ar, Ai_ = (s0r + slr) * 0.25, (s0i + sli) * 0.25
            Br, Bi = (s0r - slr) * 0.25, (s0i - sli) * 0.25
            yr0 = pr * Ar - pi * Ai_ + fpr * Br + fpi * Bi
            yi0 = pr * Ai_ + pi * Ar + fpr * Bi - fpi * Br
            yr = jnp.where(sub == 0, jnp.broadcast_to(yr0, (8, 128)), _force(Y[k][0]))
            yi = jnp.where(sub == 0, jnp.broadcast_to(yi0, (8, 128)), _force(Y[k][1]))
            Y[k] = ((yr, 1), (yi, 1))
            dlq.append((yr, state['t'] + 400))
            dlq.append((yi, state['t'] + 400))
            if k >= 12:
                mid_b(k - 12)

        first = [('v', P(f1, b), 30) for b in range(4)]
        last = [('v', P(i2, b), 20) for b in range(4)]
        if grp != 0:
            return first + [('v', P(mid, k), 78) for k in range(4)] + last, []
        a = (first + [('v', P(mid_a, k), 52) for k in range(4)] + [('v', P(sp_stack, k), 24) for k in range(16)]
             + [('m', sp_flip, 64)])
        b = [('v', P(sp_fix, k), 50 + (26 if k >= 12 else 0)) for k in range(16)] + last
        return a, b

    B3 = {}
    V3 = {}

    def p3_pre(n2, q, tok):
        hf, o = q // 2, 32 * (q % 2)
        even = (_lane((32, 128)) % 2) == 0

        def packed(ref):
            a = ref[oq(n2, 16), 128 * hf + o:128 * hf + o + 32, :]
            b = ref[oq(n2, 16), 128 * hf + 64 + o:128 * hf + 64 + o + 32, :]
            a = jnp.concatenate([gate(a[8 * i:8 * i + 8], tok) for i in range(4)], 0)
            return _pk(a, b)
        Ru = packed(yr_v)
        Ou = pltpu.roll(packed(yi_v), 1, 1)
        B3[n2, 0, q] = jnp.where(even, Ru, Ou)
        B3[n2, 1, q] = jnp.where(even, Ou, Ru)
        push_dl(B3[n2, 0, q], state['now'] + PDL, 4)

    def p3_s(n2):
        V = []
        Ms_ = lhs_par([c_u[CM + 2 * n2 + e] for e in range(2)])
        for e in range(2):
            B = _bf(jnp.concatenate([B3.pop((n2, e, q)) for q in range(4)], 0))
            V.append(jax.lax.dot_general(Ms_[e], B, NT, preferred_element_type=F32))
        l64 = _lane((64, 128))
        masks = [(l64 % 2) == 0, ((l64 + 1) % 4) < 2]
        V0, V1 = V
        V0r, V0i = V0[:64], V0[64:]
        V1i, V1r = V1[:64], V1[64:]
        VR = _pk(V0r + V1r, V0r - V1r)
        VI = _pk(V0i + V1i, V0i - V1i)
        G = []
        for h in range(2):
            r = VR[:, 128 * h:128 * h + 128]
            ri = pltpu.roll(VI[:, 128 * h:128 * h + 128], 1 + h, 1)
            G += [jnp.where(masks[h], r, ri), jnp.where(masks[h], ri, r)]
        for g in G:
            push_dl(g, state['t'] + DLAT + 64, 8)
        V3[n2] = G
        return rows8(V[1], 8), 128

    def p3_d(r0):
        Gs = [V3.pop(2 * r0), V3.pop(2 * r0 + 1)]
        Gl = lhs_par([jnp.concatenate([Gs[s][t][8 * q:8 * q + 8] for q in range(8) for s in range(2)], 0)
                      for t in range(4)])
        o = [jnp.dot(Gl[t], cmat(CAI + t), preferred_element_type=F32) for t in range(4)]
        v0, v2, T1, T3 = o
        lo = _lane((256, 128)) < 64
        Pp = T1 + T3
        Qp = pltpu.roll(T1 - T3, 64, 1)
        m0 = jnp.where(lo, Pp, (Qp - Pp) * C8)
        m1n = jnp.where(lo, Qp, (Pp + Qp) * C8)
        p0, p1_ = v0 + v2, v0 - v2
        y = [p0 + m0, p1_ - m1n, p0 - m0, p1_ + m1n]
        for q in range(8):
            for s_ in range(2):
                r_ = slice(32 * q + 16 * s_, 32 * q + 16 * s_ + 16)
                for c in range(4):
                    a_v[c, pl.ds(AP * (2 * r0 + s_) + 16 * q, 16), :] = y[c][r_]
                push_dl(m0[r_], state['t'] + DLAT + 32 * q + 16 * s_ + 16, 0)
                push_dl(m1n[r_], state['t'] + DLAT + 32 * q + 16 * s_ + 16, 0)
        return rows8(v0, 8), 256

    def m1(i, js, cs, defer):
        r2 = i * H
        xs = [[lhs(x_u[c, pl.ds(r2 + 8 * q, 8), :], 16 * q) for c in cs] for q in range(H // 8)]
        xc = jnp.concatenate([_bf(jnp.concatenate([xq[k] for xq in xs], 0)) for k in range(len(cs))], 1)
        w1 = jnp.concatenate([_bf(w1_u[c, pl.ds(64 * js[0], 64 * len(js)), :]) for c in cs], 1)
        raw = jax.lax.dot_general(xc, w1, NT, preferred_element_type=F32)

        def post(lat):
            for k, j in enumerate(js):
                r = raw[:, 128 * k:128 * k + 128]
                if cs[0] > 0:
                    r = r + p_v[i, j]
                if cs[-1] < 3:
                    p_v[i, j] = r
                    continue
                t = 0.5 * r
                th = jnp.tanh(t)
                t0 = state['t'] + lat + TM * k
                if j == 10:
                    g = 0.5 + jnp.broadcast_to(0.5 * th[:, 127:128], (TM, 128))
                    for ii in range(TM // 128):
                        g_v[(TM // 128) * i + ii] = g[128 * ii:128 * ii + 128]
                    push_dl(g, t0 + 64, 8)
                hs = t + t * th
                hp = pltpu.bitcast(hs.astype(BF), U32)
                h_u[i][j] = hp
                push_dl(hp, t0 + 16, 16)
        if defer:
            pending.append(post)
        else:
            post(DLAT)
        return rows8(raw, 8), TM

    pending = []

    def flush():
        while pending:
            pending.pop()(64)

    accs = {}

    def m2(i, g):
        cj = [divmod(f, 11) for f in range(4 * g, 4 * g + 4)]
        hq = [[lhs(h_u[i][oq(j, 11), pl.ds(8 * q, 8), :], 16 * q) for _, j in cj] for q in range(H // 8)]
        fin = []
        for c in sorted(set(c for c, _ in cj)):
            ks = [k for k in range(4) if cj[k][0] == c]
            j0 = cj[ks[0]][1]
            hs = jnp.concatenate([_bf(jnp.concatenate([hq_[k] for hq_ in hq], 0)) for k in ks], 1)
            o = jnp.dot(hs, _bf(w2_u[c, pl.ds(64 * j0, 64 * len(ks)), :]), preferred_element_type=F32)
            acc = o if j0 == 0 else o + accs.pop((i, c))
            if j0 + len(ks) < 11:
                accs[i, c] = acc
            else:
                bb_v[c, pl.ds(i * TM, TM), :] = acc
                fin.append(c)
        return rows8(acc, 8), TM, fin

    def out_copy(i, c):
        return pltpu.make_async_copy(o_v.at[c, pl.ds(128 * i, 128)],
                                     o_hbm.at[0, pl.ds(128 * i, 128), pl.ds(128 * c, 128)], s_o.at[0])

    def combine(i, c, tok):
        h, n0 = i // 8, 8 * (i % 8)
        av = []
        for n in range(8):
            for hf in range(2):
                a = a_v[c, pl.ds(8 * hf * AP + 2 * _POS_OF_N1[n0 + n] + h, 8, stride=AP), :]
                av.append(a if tok is None else gate(a, tok))
        b = bb_v[c, pl.ds(128 * i, 128), :]
        g = g_v[oq(i, 16)]
        o_v[c, pl.ds(128 * i, 128), :] = (b + g * (jnp.concatenate(av, 0) - b)).astype(BF)
        out_copy(i, c).start()

    VQ, MQ = [], []
    for r0 in range(8):
        for n2 in (2 * r0, 2 * r0 + 1):
            for gam in range(8):
                deps = [('rest', 0)] + ([(('d1', 2 * (r0 - AHEAD1)), 0)] if r0 >= AHEAD1 else [])
                VQ.append((('pre1', n2, gam), P(p1_pre, n2, gam), 58 * RATE / RATE1, deps))
    for r0 in range(9):
        if r0 < 8:
            for n2 in (2 * r0, 2 * r0 + 1):
                MQ.append((('d1', n2), P(p1_d, n2), [(('pre1', n2, 7), L_PRE)]))
        if r0 > 0:
            for n2 in (2 * r0 - 2, 2 * r0 - 1):
                MQ.append((('s1', n2), P(p1_s, n2), [(('d1', n2), L_DS)]))
    kp = [0]

    def add2(items, extra=()):
        for it in items:
            kp[0] += 1
            if it[0] == 'v':
                VQ.append((('p2', kp[0]), it[1], it[2], list(extra) + [(('s1', 15), L_POST)]))
            else:
                MQ.append(('flip', it[1], [(('p2', kp[0] - 1), L_PRE)]))
    a0, b0 = p2_items(0)
    add2(a0)
    for g in range(1, 4):
        add2(p2_items(g)[0])
    add2(b0, [('flip', 250)])
    for g in range(4, 32):
        add2(p2_items(g)[0])
    last2 = [(VQ[-1][0], 100)]
    for r0 in range(8):
        for n2 in (2 * r0, 2 * r0 + 1):
            for q in range(4):
                deps = last2 + ([(('s3', 2 * (r0 - AHEAD3)), PRE3D)] if r0 >= AHEAD3 else [])
                VQ.append((('pre3', n2, q), P(p3_pre, n2, q), C3, deps))
    for r0 in range(9):
        if r0 < 8:
            for n2 in (2 * r0, 2 * r0 + 1):
                deps = [(('pre3', n2, 3), L_PRE)] + ([(('s3', n2 - 2), PER3)] if r0 > 0 else [])
                MQ.append((('s3', n2), P(p3_s, n2), deps))
        if r0 > 0:
            MQ.append((('d3', r0 - 1), P(p3_d, r0 - 1), [(('s3', 2 * r0 - 1), L_SD)]))
    for i in range(NCH):
        for c in range(4):
            for ii in range(TM // 128):
                VQ.append((('cmb', i, c, ii), P(combine, (TM // 128) * i + ii, c), CCOST,
                           [(('d3', 7), L_POST + 256), (('m2', i, c), 0)]))

    pieces = []
    for wv, cs in enumerate(KWAVE):
        nj = 4 // len(cs)
        ks = [('m1', wv, i, tuple(range(j0, j0 + nj)), cs) for i in range(KA) for j0 in range(0, KB, nj)]
        if wv < len(KWAVE) - 1:
            pieces += ks
    full = [('m1', len(KWAVE) - 1, i, (j,), (0, 1, 2, 3))
            for i in range(NCH) for j in range(11) if i >= KA or j >= KB]
    while ks or full:
        pieces += ks[:1] + full[:KMIX]
        ks, full = ks[1:], full[KMIX:]
    pieces += [('m2', i, g) for i in range(NCH) for g in range(11)]

    when = {}

    def ok(deps, now):
        return all(d in when and when[d] + dl <= now for d, dl in deps)

    def issue(toks, cost):
        for tok, dt in toks:
            now = state['t'] + dt
            if VQ and now >= state['nxt'] and ok(VQ[0][3], now):
                name, fn, ops, _ = VQ.pop(0)
                state['now'] = now
                fn(tok)
                when[name] = now
                state['nxt'] = max(state['nxt'], now - 8) + ops / RATE
        state['t'] += cost

    def try_mxu():
        t0 = state['t']
        while MQ and ok(MQ[0][2], state['t']) and state['t'] - t0 < MBURST:
            name, fn, _ = MQ.pop(0)
            when[name] = state['t']
            issue(*fn())

    wv_done = -1
    for n, pc in enumerate(pieces):
        if pc[0] == 'm1' and pc[1] > wv_done:
            wv_done = pc[1]
            wait(wv_done)
            new_mask()
            flush()
        if n == WWAIT:
            wait(len(WAVE))
            new_mask()
            flush()
            when['rest'] = state['t']
        try_mxu()
        if pc[0] == 'm1':
            nxt = pieces[n + 1]
            issue(*m1(pc[2], pc[3], pc[4], len(pc[3]) == 1 and n + 1 == WWAIT))
        else:
            toks, cost, fin = m2(pc[1], pc[2])
            issue(toks, cost)
            for c in fin:
                when['m2', pc[1], c] = state['t']
    assert not MQ
    for it in VQ:
        assert it[0][0] == 'cmb', it[0]
        it[1](None)
    for i in range(16):
        for c in range(4):
            out_copy(i, c).wait()


@jax.jit
def pallas_gated_mix__spectral_gfnet__dense_activation_silu__prompt_kernel(A_x, A_w_r, A_w_i, B_x, B_w1, B_w2, gate_w):
    consts = jnp.asarray(_consts(), dtype=BF)
    zero = jnp.zeros((1,), jnp.int32)
    hbm = pl.BlockSpec(memory_space=pltpu.HBM)
    dma = pltpu.SemaphoreType.DMA
    return pl.pallas_call(
        _kernel,
        in_specs=[hbm] * 8,
        out_specs=hbm,
        out_shape=jax.ShapeDtypeStruct((1, S, D), BF),
        scratch_shapes=[
            pltpu.VMEM((4, S // 2, 128), U32),
            pltpu.VMEM((4, FP // 2, 128), U32),
            pltpu.VMEM((4, FP // 2, 128), U32),
            pltpu.VMEM((16, 128, 128), U32),
            pltpu.VMEM((16, 128, 128), U32),
            pltpu.VMEM((2, 1, S), BF),
            pltpu.VMEM((NCONST, 64, 128), U32),
            pltpu.VMEM((16, 256, 128), F32),
            pltpu.VMEM((16, 256, 128), F32),
            pltpu.VMEM((16, 256, 128), F32),
            pltpu.VMEM((16, 256, 128), F32),
            pltpu.VMEM((4, 16 * AP, 128), F32),
            pltpu.VMEM((4, S, 128), F32),
            pltpu.VMEM((16, 128, 128), F32),
            pltpu.VMEM((4, S, 128), BF),
            pltpu.VMEM((KA, KB, TM, 128), F32),
            pltpu.SMEM((1,), jnp.int32),
            pltpu.VMEM((4, 128), BF),
            dma((NSEM,)), dma((1,)),
        ] + [pltpu.VMEM((11, H, 128), U32) for _ in range(NCH)],
        compiler_params=pltpu.CompilerParams(vmem_limit_bytes=100 << 20),
    )(zero, A_x, A_w_r.T, A_w_i.T, B_w1.T, B_w2, gate_w.reshape(4, 128), consts)
```

```python
import functools
import numpy as np
import jax
import jax.numpy as jnp
import jax.experimental.pallas as pl
import jax.experimental.pallas.tpu as pltpu

S, D, F = 2048, 512, 1376
FP = 1408
ODD = ((1, 7), (5, 3))
BF = jnp.bfloat16
F32 = jnp.float32
U32 = jnp.uint32
C8 = float(np.sqrt(0.5))
NT = (((1,), (1,)), ((), ()))


def _kd_of_row(rho):
    t, i = divmod(rho, 64)
    return 4 * i + 2 * t if t < 2 else 8 * (i % 32) + ODD[t - 2][i // 32]


@functools.lru_cache(maxsize=None)
def _consts():
    l = np.arange(128)
    A = np.zeros((4, 128, 128))
    for t in range(4):
        for i in range(64):
            rho = 64 * t + i
            kd = _kd_of_row(rho)
            if t < 2:
                ang = 2 * np.pi * ((l * kd) % 512) / 512
                A[t, i] = np.cos(ang)
                A[t, 64 + i] = -np.sin(ang)
                if rho == 0:
                    A[t, 64] = np.where(l % 2 == 0, 1.0, -1.0)
            else:
                f = t - 2
                lp = np.arange(64)
                k, cj = (kd, 1.0) if kd % 8 == 1 + 4 * f else (512 - kd, -1.0)
                ang = 2 * np.pi * ((lp * k) % 512) / 512
                c, s = np.cos(ang), -np.sin(ang)
                sg = 1.0 if f == 0 else -1.0
                A[t, i, :64] = c
                A[t, i, 64:] = -s * sg
                A[t, 64 + i, :64] = cj * s
                A[t, 64 + i, 64:] = cj * c * sg
    Ai = np.zeros((4, 128, 128))
    for t in range(4):
        sc = np.full(128, 2.0 / (S * D))
        if t == 0:
            sc[0] = sc[64] = 1.0 / (S * D)
        M = A[t] * sc[:, None]
        Ai[t] = M if t % 2 == 0 else np.concatenate([M[64:], M[:64]], 0)
    Ms = np.zeros((16, 2, 128, 128))
    n1 = np.arange(64)[:, None]
    k1 = np.arange(64)[None, :]
    for e in range(2):
        for n2 in range(16):
            ang = 2 * np.pi * (((16 * n1 + n2) * (e + 2 * k1)) % 2048) / 2048
            c, s = np.cos(ang), -np.sin(ang)
            re_cols = 2 * np.arange(64) + e
            im_cols = (2 * np.arange(64) + 1 + e) % 128
            M = np.zeros((128, 128))
            rr = slice(0, 64) if e == 0 else slice(64, 128)
            ir = slice(64, 128) if e == 0 else slice(0, 64)
            M[rr, re_cols] = c
            M[ir, re_cols] = -s
            M[rr, im_cols] = s
            M[ir, im_cols] = c
            Ms[n2, e] = M
    J = np.zeros((1, 128, 128))
    J[0, l, (128 - l) % 128] = 1.0
    allc = np.concatenate([A, Ai, J, Ms.reshape(32, 128, 128)], 0)
    return allc.astype(np.float32)


CA, CAI, CJ, CM = 0, 4, 8, 9
NCONST = 41


def _add(a, b):
    (x, sx), (y, sy) = a, b
    if sx == sy:
        return (x + y, sx)
    return (x - y, 1) if sx > 0 else (y - x, 1)


def _neg(a):
    return (a[0], -a[1])


def _sub(a, b):
    return _add(a, _neg(b))


def _scale(a, c):
    return (a[0] * (c * a[1]), 1)


def _cadd(a, b):
    return (_add(a[0], b[0]), _add(a[1], b[1]))


def _csub(a, b):
    return (_sub(a[0], b[0]), _sub(a[1], b[1]))


def _mul_mi(a, sgn):
    re, im = a
    return (im, _neg(re)) if sgn > 0 else (_neg(im), re)


def _twiddle(a, j, sgn):
    j = j % 16
    if j % 4 == 0:
        for _ in range(j // 4):
            a = _mul_mi(a, sgn)
        return a
    re, im = a
    if j % 2 == 0:
        if sgn > 0:
            r = _scale(_add(re, im), C8)
            i = _scale(_sub(im, re), C8)
        else:
            r = _scale(_sub(re, im), C8)
            i = _scale(_add(im, re), C8)
        a = (r, i)
        for _ in range(j // 4):
            a = _mul_mi(a, sgn)
        return a
    c = float(np.cos(2 * np.pi * j / 16))
    s = float(-sgn * np.sin(2 * np.pi * j / 16))
    r = _sub(_scale(re, c), _scale(im, s))
    i = _add(_scale(re, s), _scale(im, c))
    return (r, i)


def _dft4(v, sgn):
    a, b, c, d = v
    t0, t1 = _cadd(a, c), _csub(a, c)
    t2, t3 = _cadd(b, d), _mul_mi(_csub(b, d), sgn)
    return [_cadd(t0, t2), _cadd(t1, t3), _csub(t0, t2), _csub(t1, t3)]


def _force(a):
    return a[0] if a[1] > 0 else -a[0]


def _lo_f32(w):
    return pltpu.bitcast(w << 16, F32)


def _hi_f32(w):
    return pltpu.bitcast(w & jnp.uint32(0xFFFF0000), F32)


def _bf(u):
    return pltpu.bitcast(u, BF)


def _lane(shape):
    return jax.lax.broadcasted_iota(jnp.int32, shape, 1)


TM = 256
NCH = S // TM
H = TM // 2
TR = F - 1280
AP = 136
NB = 16
KA, KB = 4, 8
XC = 6
NWAVE = 4
RATE = 1.8
RATE1 = 1.15
C3 = 24
CMID = 24
CG = 110
CCOST = 110
L_PRE = 350
L_LHS = 250
L_MID = 150
L_POST = 450
DLAT = 260
XDL = 100
PDL = 300
GDL = 400
TDL2 = 500
DLQ2 = 48
MBURST = 256
MTPOS = 30


def _kernel(z_hbm, x_hbm, wr_hbm, wi_hbm, w1_hbm, w2_hbm, gw_hbm, c_hbm, o_hbm,
            xb, w1b, w2b, wr_b, wi_b, wl_v, c_b, xr_v, xi_v, yr_b, yi_b, a_v, bb_v, g_v, og_v, o_v, p_v,
            z_ref, gw_ref, gw_f, sems, s_o, *bufs):
    P = functools.partial
    h_b, t_b, z_b, v_b = bufs[:NCH], bufs[NCH:NCH + NB], bufs[NCH + NB:NCH + 2 * NB], bufs[NCH + 2 * NB:]
    x_u, w1_u, w2_u, wr_u, wi_u, c_u, yr_u, yi_u = [
        r.bitcast(U32) for r in (xb, w1b, w2b, wr_b, wi_b, c_b, yr_b, yi_b)]
    h_u, t_u, z_u, v_u = [[r.bitcast(U32) for r in rs] for rs in (h_b, t_b, z_b, v_b)]
    groups = []

    def xrows(r0, r1, cs):
        return [(x_hbm.at[0, pl.ds(r0, r1 - r0), pl.ds(128 * c, 128)], xb.at[c, pl.ds(r0, r1 - r0)]) for c in cs]

    def w1rows(r0, r1, cs):
        return [(w1_hbm.at[pl.ds(r0, r1 - r0), pl.ds(128 * c, 128)], w1b.at[c, pl.ds(r0, r1 - r0)]) for c in cs]

    A4 = range(4)
    groups.append(xrows(0, 2 * TM, [0]) + w1rows(0, 512, [0]))
    groups.append(xrows(2 * TM, 4 * TM, [0]) + w1rows(512, 1024, [0]))
    groups.append(xrows(0, 4 * TM, [1]) + w1rows(0, 1024, [1]) + xrows(0, 4 * TM, [2]) + w1rows(0, 512, [2]))
    groups.append(w1rows(512, 1024, [2]) + xrows(0, 4 * TM, [3]) + w1rows(0, 1024, [3])
                  + w1rows(1024, F, A4) + xrows(4 * TM, XC * TM, A4))
    groups[0].append((z_hbm, z_ref))
    groups[-1].append((gw_hbm, gw_ref))
    rest = xrows(XC * TM, S, A4) + [(c_hbm, c_b)]
    rest += [(w2_hbm.at[:, pl.ds(128 * c, 128)], w2b.at[c, pl.ds(0, F)]) for c in range(4)]
    for k in range(16):
        rest.append((wr_hbm.at[pl.ds(0, 256), pl.ds(128 * k, 128)], wr_b.at[k]))
        rest.append((wi_hbm.at[pl.ds(0, 256), pl.ds(128 * k, 128)], wi_b.at[k]))
    rest.append((wr_hbm.at[pl.ds(256, 1), :], wl_v.at[0]))
    rest.append((wi_hbm.at[pl.ds(256, 1), :], wl_v.at[1]))
    groups.append(rest)
    copies = [[pltpu.make_async_copy(s_, d_, sems.at[gi]) for s_, d_ in g] for gi, g in enumerate(groups)]
    for g in copies:
        for cp in g:
            cp.start()

    def wait(gi):
        for cp in copies[gi]:
            cp.wait()
        if gi == NWAVE - 1:
            for c in range(4):
                gw_f[c] = jnp.broadcast_to(gw_ref[c:c + 1, :].astype(F32), (16, 128))
        if gi == NWAVE:
            for c in range(4):
                w2b[c, pl.ds(F, FP - F), :] = jnp.zeros((FP - F, 128), BF)

    fmask_box = {}
    dlq = []

    def gate(v, tok):
        if v.dtype != tok.dtype:
            tok = pltpu.bitcast(tok, v.dtype)
        return jnp.where(fmask_box['m'], tok, v)

    def new_mask():
        dlq.clear()
        z = z_ref[0]
        fmask_box.clear()
        fmask_box['z'] = z
        fmask_box['m'] = jnp.full((8, 128), z, jnp.int32) != 0

    def oq(k, n):
        if (k, n) not in fmask_box:
            fmask_box[k, n] = jnp.clip(k + fmask_box['z'], 0, n - 1)
        return fmask_box[k, n]

    def gatec(v, tok):
        out = list(v)
        for i in (0, 1):
            (r, sr), (im, si) = v[i]
            out[i] = ((gate(r, tok), sr), (gate(im, tok), si))
        return out

    def cmat(i):
        return _bf(c_u[i])

    def rows8(a, step):
        return [(a[8 * q:8 * q + 8, 0:128], step * q) for q in range(a.shape[0] // 8)]

    state = dict(t=0, nxt=0)

    def push_dl(a, t0, step):
        for v, dt in rows8(a, step):
            dlq.append((v, t0 + dt))

    def lhs(u, dt):
        tok = None
        dlq.sort(key=lambda e: e[1])
        for _ in range(2 if len(dlq) > DLQ2 else 1):
            if dlq and dlq[0][1] <= state['t'] + dt:
                v = pltpu.bitcast(dlq.pop(0)[0], U32)
                tok = v if tok is None else tok | v
        return u if tok is None else gate(u, tok)

    def lhs_par(ops):
        n = ops[0].shape[0] // 8
        g = [[lhs(u[8 * q:8 * q + 8], 16 * q) for u in ops] for q in range(n)]
        return [_bf(jnp.concatenate([g[q][k] for q in range(n)], 0)) for k in range(len(ops))]

    T1s = {}
    Zs = {}

    def p1_pre(n2, gam, tok):
        unp = _hi_f32 if n2 % 2 else _lo_f32
        lo = _lane((8, 128)) < 64
        r0 = n2 // 2 + 64 * gam
        a = [unp(gate(x_u[c, pl.ds(r0, 8, stride=8), :], tok)) for c in range(4)]
        b = [unp(x_u[c, pl.ds(r0 + 512, 8, stride=8), :]) for c in range(4)]
        for e in range(2):
            U = [a[c] + b[c] if e == 0 else a[c] - b[c] for c in range(4)]
            p0, p1_, m0, m1 = U[0] + U[2], U[1] + U[3], U[0] - U[2], U[1] - U[3]
            Pv = jnp.where(lo, m0, (m0 + m1) * (-C8))
            Qn = pltpu.roll(jnp.where(lo, m1, (m1 - m0) * C8), 64, 1)
            for t, val in enumerate([p0 + p1_, p0 - p1_, Pv - Qn, Pv + Qn]):
                if gam % 2 == 0:
                    T1s[n2, t, e] = val
                else:
                    pair = jnp.concatenate([T1s.pop((n2, t, e)), val], 0)
                    t_b[n2][t, pl.ds(64 * e + 8 * (gam - 1), 16), :] = pair.astype(BF)
                if t == 2:
                    dlq.append((val, state['now'] + PDL))

    def p1_d(n2):
        As = lhs_par([c_u[CA + t] for t in range(4)])
        for t in range(4):
            Z = jax.lax.dot_general(As[t], _bf(t_u[n2][oq(t, 4)]), NT, preferred_element_type=F32)
            z_b[n2][t] = Z.astype(BF)
        return rows8(Z, 8), 128

    def p1_mid(n2, t, tok):
        lo = _lane((32, 128)) < 64
        z = z_u[n2][oq(t, 4)]
        ZR = z[:32]
        RI = pltpu.roll(jnp.concatenate([gate(z[32 + 8 * q:40 + 8 * q], tok) for q in range(4)], 0), 64, 1)
        Zs[n2, 0, t] = jnp.where(lo, ZR, RI)
        Zs[n2, 1, t] = jnp.where(lo, RI, ZR)
        push_dl(Zs[n2, 0, t], state['now'] + PDL, 4)

    def p1_s(n2):
        T0, T1 = [jnp.concatenate([Zs.pop((n2, e, t)) for t in range(4)], 0) for e in range(2)]
        even = (_lane((128, 128)) % 2) == 0
        xi = []
        Ls = lhs_par([T0[:64], T1[:64], T0[64:], T1[64:]])
        for hf in range(2):
            O0 = jnp.dot(Ls[2 * hf], cmat(CM + 2 * n2), preferred_element_type=F32)
            O1 = jnp.dot(Ls[2 * hf + 1], cmat(CM + 2 * n2 + 1), preferred_element_type=F32)
            xr_v[n2, 128 * hf:128 * hf + 128, :] = jnp.where(even, O0, O1)
            xi.append(pltpu.roll(jnp.where(even, O1, O0), 127, 1))
            xi_v[n2, 128 * hf:128 * hf + 128, :] = xi[-1]
        for q in range(16):
            for hf in range(2):
                dlq.append((xi[hf][8 * q:8 * q + 8], state['t'] + DLAT + XDL + 8 * q))
        return rows8(O1, 8), 128

    def p2_items(grp):
        row = pl.ds(8 * grp, 8)
        kd0 = _kd_of_row(8 * grp)
        wrow = pl.ds(kd0 // 2, 8, stride=(_kd_of_row(8 * grp + 1) - kd0) // 2)
        unp = _hi_f32 if kd0 % 2 else _lo_f32
        y = [[None] * 4 for _ in range(4)]
        z = [[None] * 4 for _ in range(4)]
        X = [None] * 16
        Y = [None] * 16
        st = {}

        def f1(b, tok):
            v = [((xr_v[oq(4 * a + b, 16), row, :], 1), (xi_v[oq(4 * a + b, 16), row, :], 1)) for a in range(4)]
            o = _dft4(gatec(v, tok), +1)
            for kap in range(4):
                y[kap][b] = _twiddle(o[kap], b * kap, +1)

        def mid_a(kap, tok):
            o = _dft4(gatec(y[kap], tok), +1)
            for io in range(4):
                k = kap + 4 * io
                wr = unp(wr_u[k, wrow, :])
                wi = unp(wi_u[k, wrow, :])
                X[k] = o[io]
                (xr, sr), (xi, si) = o[io]
                Y[k] = (_sub((xr * wr, sr), (xi * wi, si)), _add((xr * wi, sr), (xi * wr, si)))

        def mid_b(kap):
            o2 = _dft4([Y[kap + 4 * io] for io in range(4)], -1)
            for b2 in range(4):
                z[b2][kap] = _twiddle(o2[b2], kap * b2, -1)

        def mid(kap, tok):
            mid_a(kap, tok)
            mid_b(kap)

        def i2(b2, tok):
            o = _dft4(gatec(z[b2], tok), -1)
            for io in range(4):
                yr_b[b2 + 4 * io, row, :] = _force(o[io][0]).astype(BF)
                yi_b[b2 + 4 * io, row, :] = _force(o[io][1]).astype(BF)

        def sp_stack(k, tok):
            sub = jax.lax.broadcasted_iota(jnp.int32, (8, 128), 0)
            w0r = unp(wr_u[k, wrow, :])[0:1]
            w0i = unp(wi_u[k, wrow, :])[0:1]
            wlr = wl_v[0, :, 128 * k:128 * k + 128].astype(F32)
            wli = wl_v[1, :, 128 * k:128 * k + 128].astype(F32)
            pr = gate(_force(X[k][0]), tok)[0:1]
            pi = _force(X[k][1])[0:1]
            blk = jnp.zeros((8, 128), F32)
            for jj, r in enumerate([pr, pi, w0r, w0i, wlr, wli]):
                blk = jnp.where(sub == jj, jnp.broadcast_to(r, (8, 128)), blk)
            st[k] = blk

        def sp_flip():
            full = jnp.concatenate([st[k] for k in range(16)], 0)
            fl = []
            for hf in range(2):
                part = full[64 * hf:64 * hf + 64]
                hi_ = part.astype(BF)
                lo_ = (part - hi_.astype(F32)).astype(BF)
                fh = jnp.dot(hi_, cmat(CJ), preferred_element_type=F32)
                fl.append(jnp.dot(lo_, cmat(CJ), preferred_element_type=F32) + fh)
            fl = jnp.concatenate(fl, 0)
            st['fl'] = fl
            return rows8(fl, 4), 64

        def sp_fix(k, tok):
            sub = jax.lax.broadcasted_iota(jnp.int32, (8, 128), 0)
            fl = st['fl']
            fa = fl[8 * (15 - k):8 * (15 - k) + 8]
            fb = fl[8 * ((16 - k) % 16):8 * ((16 - k) % 16) + 8]
            f = gate(jnp.where(_lane((8, 128)) == 0, fb, fa), tok)
            o = st[k]
            pr, pi, w0r, w0i, wlr, wli = [o[jj:jj + 1] for jj in range(6)]
            fpr, fpi, f0r, f0i, flr, fli = [f[jj:jj + 1] for jj in range(6)]
            s0r, s0i = w0r + f0r, w0i - f0i
            slr, sli = wlr + flr, wli - fli
            Ar, Ai_ = (s0r + slr) * 0.25, (s0i + sli) * 0.25
            Br, Bi = (s0r - slr) * 0.25, (s0i - sli) * 0.25
            yr0 = pr * Ar - pi * Ai_ + fpr * Br + fpi * Bi
            yi0 = pr * Ai_ + pi * Ar + fpr * Bi - fpi * Br
            yr = jnp.where(sub == 0, jnp.broadcast_to(yr0, (8, 128)), _force(Y[k][0]))
            yi = jnp.where(sub == 0, jnp.broadcast_to(yi0, (8, 128)), _force(Y[k][1]))
            Y[k] = ((yr, 1), (yi, 1))
            dlq.append((yr, state['t'] + 400))
            dlq.append((yi, state['t'] + 400))
            if k >= 12:
                mid_b(k - 12)

        first = [('v', P(f1, b), 30) for b in range(4)]
        last = [('v', P(i2, b), 28) for b in range(4)]
        if grp != 0:
            return first + [('v', P(mid, k), 78) for k in range(4)] + last, []
        a = (first + [('v', P(mid_a, k), 52) for k in range(4)] + [('v', P(sp_stack, k), 24) for k in range(16)]
             + [('m', sp_flip, 64)])
        b = [('v', P(sp_fix, k), 50 + (26 if k >= 12 else 0)) for k in range(16)] + last
        return a, b

    B3 = {}
    V3 = {}

    def p3_pre(n2, q, tok):
        even = (_lane((32, 128)) % 2) == 0
        Ru = yr_u[oq(n2, 16), pl.ds(32 * q, 32), :]
        Iu = yi_u[oq(n2, 16), pl.ds(32 * q, 32), :]
        Ou = pltpu.roll(jnp.concatenate([gate(Iu[8 * i:8 * i + 8], tok) for i in range(4)], 0), 1, 1)
        B3[n2, 0, q] = jnp.where(even, Ru, Ou)
        B3[n2, 1, q] = jnp.where(even, Ou, Ru)
        push_dl(B3[n2, 0, q], state['now'] + PDL, 4)

    def p3_s(n2):
        V = []
        Ms_ = lhs_par([c_u[CM + 2 * n2 + e] for e in range(2)])
        for e in range(2):
            B = _bf(jnp.concatenate([B3.pop((n2, e, q)) for q in range(4)], 0))
            V.append(jax.lax.dot_general(Ms_[e], B, NT, preferred_element_type=F32))
        V0, V1 = V
        V0r, V0i = V0[:64], V0[64:]
        V1i, V1r = V1[:64], V1[64:]
        VR = jnp.concatenate([V0r + V1r, V0r - V1r], 0)
        VI = jnp.concatenate([V0i + V1i, V0i - V1i], 0)
        for hf in range(2):
            v_b[n2][hf] = VR[:, 128 * hf:128 * hf + 128].astype(BF)
            v_b[n2][2 + hf] = VI[:, 128 * hf:128 * hf + 128].astype(BF)
        return rows8(V[1], 8), 128

    def p3_mid(n2, q, tok):
        hf, o = q // 2, 32 * (q % 2)
        lo = _lane((32, 128)) < 64
        r = v_u[n2][oq(hf, 4), pl.ds(o, 32), :]
        im = v_u[n2][oq(2 + hf, 4), pl.ds(o, 32), :]
        ri = pltpu.roll(jnp.concatenate([gate(im[8 * i:8 * i + 8], tok) for i in range(4)], 0), 64, 1)
        V3[n2, 2 * hf, q % 2] = jnp.where(lo, r, ri)
        V3[n2, 2 * hf + 1, q % 2] = jnp.where(lo, ri, r)
        push_dl(V3[n2, 2 * hf, q % 2], state['now'] + PDL, 4)

    def p3_d(r0):
        Gl = lhs_par([jnp.concatenate([V3.pop((n2, t, k)) for n2 in (2 * r0, 2 * r0 + 1) for k in range(2)], 0)
                      for t in range(4)])
        o = [jnp.dot(Gl[t], cmat(CAI + t), preferred_element_type=F32) for t in range(4)]
        v0, v2, T1, T3 = o
        lo = _lane((256, 128)) < 64
        Pp = T1 + T3
        Qp = pltpu.roll(T1 - T3, 64, 1)
        m0 = jnp.where(lo, Pp, (Qp - Pp) * C8)
        m1n = jnp.where(lo, Qp, (Pp + Qp) * C8)
        p0, p1_ = v0 + v2, v0 - v2
        y = [p0 + m0, p1_ - m1n, p0 - m0, p1_ + m1n]
        for s_ in range(2):
            for c in range(4):
                a_v[c, pl.ds(AP * (2 * r0 + s_), 128), :] = y[c][128 * s_:128 * s_ + 128]
        push_dl(m0, state['t'] + DLAT + 16, 8)
        push_dl(m1n, state['t'] + DLAT + 16, 8)
        return rows8(v0, 8), 256

    def m1(i, js, cs, defer):
        r2 = i * H
        xs = [[lhs(x_u[c, pl.ds(r2 + 8 * q, 8), :], 16 * q) for c in cs] for q in range(H // 8)]
        xc = jnp.concatenate([_bf(jnp.concatenate([xq[k] for xq in xs], 0)) for k in range(len(cs))], 1)
        w1 = jnp.concatenate([_bf(w1_u[c, pl.ds(64 * js[0], 64 * len(js)), :]) for c in cs], 1)
        raw = jax.lax.dot_general(xc, w1, NT, preferred_element_type=F32)

        def post(lat):
            for k, j in enumerate(js):
                r = raw[:, 128 * k:128 * k + 128]
                if cs[0] > 0:
                    r = r + p_v[i, j]
                if cs[-1] < 3:
                    p_v[i, j] = r
                    continue
                t = 0.5 * r
                th = jnp.tanh(t)
                t0 = state['t'] + lat + TM * k
                hs = t + t * th
                h_b[i][j] = hs.astype(BF)
                for q in range(TM // 16):
                    dlq.append((hs[16 * q + 8:16 * q + 16], t0 + 16 + 16 * q))
        if defer:
            pending.append(post)
        else:
            post(DLAT)
        return rows8(raw, 8), TM

    def gate_pk(b, tok):
        s_ = None
        for c in range(4):
            xv = _bf(gate(x_u[c, pl.ds(8 * b, 8), :], tok)).astype(F32) * gw_f[oq(c, 4)]
            s_ = xv if s_ is None else s_ + xv
        lg = jnp.broadcast_to(jnp.sum(s_, axis=1, keepdims=True), (16, 128))
        tg = 0.5 * jnp.tanh(0.5 * lg)
        g_v[b // 8, pl.ds(16 * (b % 8), 16), :] = 0.5 + tg
        og_v[pl.ds(16 * b, 16), :] = 0.5 - tg
        push_dl(tg, state['now'] + GDL, 0)

    def mt(i):
        toks = []
        for ii in range(TM // 128):
            b = (TM // 128) * i + ii
            Ls = lhs_par([w1_u[c, pl.ds(640, TR // 2), :] for c in range(4)])
            xw = jnp.concatenate([_bf(x_u[c, pl.ds(64 * b, 64), :]) for c in range(4)], 1)
            raw = jax.lax.dot_general(jnp.concatenate(Ls, 1), xw, NT, preferred_element_type=F32)
            t = 0.5 * raw
            hs = t + t * jnp.tanh(t)
            full = jnp.concatenate([hs, jnp.zeros((128 - TR, 128), F32)], 0).T
            h_b[i][10, pl.ds(128 * ii, 128), :] = full.astype(BF)
            push_dl(full, state['t'] + TR + TDL2, 8)
            for tok, dt in rows8(raw, 8):
                toks.append((tok, TR * ii + dt))
            state['t'] += TR
        state['t'] -= TR * (TM // 128)
        return toks, TR * (TM // 128)

    pending = []

    def flush():
        while pending:
            pending.pop()(64)

    accs = {}

    def m2(i, g):
        cj = [divmod(f, 11) for f in range(4 * g, 4 * g + 4)]
        hq = [[lhs(h_u[i][oq(j, 11), pl.ds(8 * q, 8), :], 16 * q) for _, j in cj] for q in range(H // 8)]
        fin = []
        for c in sorted(set(c for c, _ in cj)):
            ks = [k for k in range(4) if cj[k][0] == c]
            j0 = cj[ks[0]][1]
            hs = jnp.concatenate([_bf(jnp.concatenate([hq_[k] for hq_ in hq], 0)) for k in ks], 1)
            o = jnp.dot(hs, _bf(w2_u[c, pl.ds(64 * j0, 64 * len(ks)), :]), preferred_element_type=F32)
            acc = o if j0 == 0 else o + accs.pop((i, c))
            if j0 + len(ks) < 11:
                accs[i, c] = acc
            else:
                bb_v[c, pl.ds(i * TM, TM), :] = acc * og_v[pl.ds(i * TM, TM), :]
                fin.append(c)
        return rows8(acc, 8), TM, fin

    def out_copy(i, c):
        return pltpu.make_async_copy(o_v.at[c, pl.ds(128 * i, 128)],
                                     o_hbm.at[0, pl.ds(128 * i, 128), pl.ds(128 * c, 128)], s_o.at[0])

    def combine(i, c, tok):
        av = []
        for n in range(8):
            for hf in range(2):
                a = a_v[c, pl.ds(8 * hf * AP + 8 * i + n, 8, stride=AP), :]
                av.append(a if tok is None else gate(a, tok))
        b = bb_v[c, pl.ds(128 * i, 128), :]
        o = g_v[oq(i, 16)] * jnp.concatenate(av, 0) + b
        o_v[c, pl.ds(128 * i, 128), :] = o.astype(BF)
        out_copy(i, c).start()

    VQ, MQ = [], []
    for b in range(XC * TM // 16):
        VQ.append((('gate', b), P(gate_pk, b), CG, [('xall', 0)]))

    def pre1(r0):
        for n2 in (2 * r0, 2 * r0 + 1):
            for gam in range(8):
                deps = [('rest', 0)] + ([(('d1', 2 * (r0 - 2)), 0)] if r0 >= 2 else [])
                VQ.append((('pre1', n2, gam), P(p1_pre, n2, gam), 58 * RATE / RATE1, deps))

    def mid(name, dep, fn, r0):
        for n2 in (2 * r0, 2 * r0 + 1):
            for q in range(4):
                VQ.append(((name, n2, q), P(fn, n2, q), CMID, [((dep, n2), L_MID)]))
    for r0 in range(10):
        if r0 < 8:
            pre1(r0)
        if r0 >= 2:
            mid('mid1', 'd1', p1_mid, r0 - 2)
    for r0 in range(10):
        if r0 < 8:
            for n2 in (2 * r0, 2 * r0 + 1):
                MQ.append((('d1', n2), P(p1_d, n2), [(('pre1', n2, 7), L_PRE)]))
        if r0 >= 2:
            for n2 in (2 * r0 - 4, 2 * r0 - 3):
                MQ.append((('s1', n2), P(p1_s, n2), [(('mid1', n2, 3), L_LHS)]))
    late_gates = list(range(XC * TM // 16, S // 16))
    kp = [0]

    def add2(items, extra=()):
        for it in items:
            kp[0] += 1
            if it[0] == 'v':
                VQ.append((('p2', kp[0]), it[1], it[2], list(extra) + [(('s1', 15), L_POST)]))
            else:
                MQ.append(('flip', it[1], [(('p2', kp[0] - 1), L_PRE)]))
    a0, b0 = p2_items(0)
    add2(a0)
    for g in range(1, 4):
        add2(p2_items(g)[0])
    add2(b0, [('flip', 250)])
    for g in range(4, 32):
        for b in late_gates[2 * (g - 4):2 * (g - 4) + 2]:
            VQ.append((('gate', b), P(gate_pk, b), 40, [('rest', 0)]))
        add2(p2_items(g)[0])
    last2 = [(VQ[-1][0], 100)]
    for r0 in range(9):
        if r0 < 8:
            for n2 in (2 * r0, 2 * r0 + 1):
                for q in range(4):
                    VQ.append((('pre3', n2, q), P(p3_pre, n2, q), C3, last2))
        if r0 >= 1:
            mid('mid3', 's3', p3_mid, r0 - 1)
    for r0 in range(9):
        if r0 < 8:
            for n2 in (2 * r0, 2 * r0 + 1):
                MQ.append((('s3', n2), P(p3_s, n2), [(('pre3', n2, 3), L_PRE)]))
        if r0 >= 1:
            MQ.append((('d3', r0 - 1), P(p3_d, r0 - 1), [(('mid3', 2 * r0 - 1, 3), L_LHS)]))
    for i in range(NCH):
        for c in range(4):
            for ii in range(TM // 128):
                VQ.append((('cmb', i, c, ii), P(combine, (TM // 128) * i + ii, c), CCOST,
                           [(('d3', 7), L_POST + 256), (('m2', i, c), 0)]))

    pieces = [('m1', 0, i, (0, 1, 2, 3), (0,)) for i in range(2)]
    pieces += [('m1', 1, i, js, (0,)) for i in range(4) for js in ((0, 1, 2, 3), (4, 5, 6, 7)) if i >= 2 or js[0] == 4]
    for i in range(4):
        pieces += [('m1', 2, i, (0, 1), (1, 2)), ('m1', 2, i, (2, 3), (1, 2)), ('m1', 2, i, (4, 5, 6, 7), (1,))]
    ks = []
    for i in range(4):
        ks += [('m1', 3, i, (0, 1, 2, 3), (3,)), ('m1', 3, i, (4, 5), (2, 3)), ('m1', 3, i, (6, 7), (2, 3))]
    full = [('m1', 3, i, (j,), (0, 1, 2, 3)) for i in range(XC) for j in range(10) if i >= KA or j >= KB]
    last = [('m1', 3, i, (10,), (0, 1, 2, 3)) for i in range(XC)]
    while ks or full or last:
        pieces += ks[:1] + full[:2] + ks[1:2] + full[2:3] + last[:1] + full[3:4]
        ks, last, full = ks[2:], last[1:], full[4:]
    wwait = len(pieces)
    pieces += [('m1', 3, i, (j,), (0, 1, 2, 3)) for i in range(XC, NCH) for j in range(10)]
    m2s = [('m2', i, g) for i in range(NCH) for g in range(11)]
    for k, i in enumerate(range(XC, NCH)):
        m2s.insert(MTPOS + 3 * k, ('m1', 3, i, (10,), (0, 1, 2, 3)))
    pieces += m2s

    when = {}

    def ok(deps, now):
        return all(d in when and when[d] + dl <= now for d, dl in deps)

    def issue(toks, cost):
        for tok, dt in toks:
            now = state['t'] + dt
            if VQ and now >= state['nxt'] and ok(VQ[0][3], now):
                name, fn, ops, _ = VQ.pop(0)
                state['now'] = now
                fn(tok)
                when[name] = now
                state['nxt'] = max(state['nxt'], now - 8) + ops / RATE
        state['t'] += cost

    def try_mxu():
        t0 = state['t']
        while MQ and ok(MQ[0][2], state['t']) and state['t'] - t0 < MBURST:
            name, fn, _ = MQ.pop(0)
            when[name] = state['t']
            issue(*fn())

    wv_done = -1
    for n, pc in enumerate(pieces):
        if pc[0] == 'm1' and pc[1] > wv_done:
            wv_done = pc[1]
            wait(wv_done)
            new_mask()
            flush()
            if wv_done == NWAVE - 1:
                when['xall'] = state['t']
        if n == wwait:
            wait(NWAVE)
            new_mask()
            flush()
            when['rest'] = state['t']
        try_mxu()
        if pc[0] == 'm1' and pc[3] == (10,):
            issue(*mt(pc[2]))
        elif pc[0] == 'm1':
            issue(*m1(pc[2], pc[3], pc[4], len(pc[3]) == 1 and n + 1 == wwait))
        else:
            toks, cost, fin = m2(pc[1], pc[2])
            issue(toks, cost)
            for c in fin:
                when['m2', pc[1], c] = state['t']
    assert not MQ
    for it in VQ:
        assert it[0][0] == 'cmb', it[0]
        it[1](None)
    for i in range(16):
        for c in range(4):
            out_copy(i, c).wait()


@jax.jit
def pallas_gated_mix__spectral_gfnet__dense_activation_silu__prompt_kernel(A_x, A_w_r, A_w_i, B_x, B_w1, B_w2, gate_w):
    consts = jnp.asarray(_consts(), dtype=BF)
    zero = jnp.zeros((1,), jnp.int32)
    hbm = pl.BlockSpec(memory_space=pltpu.HBM)
    dma = pltpu.SemaphoreType.DMA
    return pl.pallas_call(
        _kernel,
        in_specs=[hbm] * 8,
        out_specs=hbm,
        out_shape=jax.ShapeDtypeStruct((1, S, D), BF),
        scratch_shapes=[
            pltpu.VMEM((4, S, 128), BF),
            pltpu.VMEM((4, F, 128), BF),
            pltpu.VMEM((4, FP, 128), BF),
            pltpu.VMEM((16, 256, 128), BF),
            pltpu.VMEM((16, 256, 128), BF),
            pltpu.VMEM((2, 1, S), BF),
            pltpu.VMEM((NCONST, 128, 128), BF),
            pltpu.VMEM((16, 256, 128), F32),
            pltpu.VMEM((16, 256, 128), F32),
            pltpu.VMEM((16, 256, 128), BF),
            pltpu.VMEM((16, 256, 128), BF),
            pltpu.VMEM((4, 16 * AP, 128), F32),
            pltpu.VMEM((4, S, 128), F32),
            pltpu.VMEM((16, 128, 128), F32),
            pltpu.VMEM((S, 128), F32),
            pltpu.VMEM((4, S, 128), BF),
            pltpu.VMEM((KA, KB, TM, 128), F32),
            pltpu.SMEM((1,), jnp.int32),
            pltpu.VMEM((4, 128), BF),
            pltpu.VMEM((4, 16, 128), F32),
            dma((NWAVE + 1,)), dma((1,)),
        ] + [pltpu.VMEM((11, TM, 128), BF) for _ in range(NCH)]
        + [pltpu.VMEM((4, 128, 128), BF) for _ in range(3 * NB)],
        compiler_params=pltpu.CompilerParams(vmem_limit_bytes=100 << 20),
    )(zero, A_x, A_w_r.T, A_w_i.T, B_w1.T, B_w2, gate_w.reshape(4, 128), consts)
```

```python
import functools
import numpy as np
import jax
import jax.numpy as jnp
import jax.experimental.pallas as pl
import jax.experimental.pallas.tpu as pltpu

S, D, F = 2048, 512, 1376
FP = 1408
ODD = ((1, 7), (5, 3))
BF = jnp.bfloat16
F32 = jnp.float32
U32 = jnp.uint32
C8 = float(np.sqrt(0.5))
NT = (((1,), (1,)), ((), ()))


def _kd_of_row(rho):
    t, i = divmod(rho, 64)
    return 4 * i + 2 * t if t < 2 else 8 * (i % 32) + ODD[t - 2][i // 32]


@functools.lru_cache(maxsize=None)
def _consts():
    l = np.arange(128)
    A = np.zeros((4, 128, 128))
    for t in range(4):
        for i in range(64):
            rho = 64 * t + i
            kd = _kd_of_row(rho)
            if t < 2:
                ang = 2 * np.pi * ((l * kd) % 512) / 512
                A[t, i] = np.cos(ang)
                A[t, 64 + i] = -np.sin(ang)
                if rho == 0:
                    A[t, 64] = np.where(l % 2 == 0, 1.0, -1.0)
            else:
                f = t - 2
                lp = np.arange(64)
                k, cj = (kd, 1.0) if kd % 8 == 1 + 4 * f else (512 - kd, -1.0)
                ang = 2 * np.pi * ((lp * k) % 512) / 512
                c, s = np.cos(ang), -np.sin(ang)
                sg = 1.0 if f == 0 else -1.0
                A[t, i, :64] = c
                A[t, i, 64:] = -s * sg
                A[t, 64 + i, :64] = cj * s
                A[t, 64 + i, 64:] = cj * c * sg
    Ai = np.zeros((4, 128, 128))
    for t in range(4):
        sc = np.full(128, 2.0 / (S * D))
        if t == 0:
            sc[0] = sc[64] = 1.0 / (S * D)
        M = A[t] * sc[:, None]
        Ai[t] = M if t % 2 == 0 else np.concatenate([M[64:], M[:64]], 0)
    Ms = np.zeros((16, 2, 128, 128))
    n1 = np.arange(64)[:, None]
    k1 = np.arange(64)[None, :]
    for e in range(2):
        for n2 in range(16):
            ang = 2 * np.pi * (((16 * n1 + n2) * (e + 2 * k1)) % 2048) / 2048
            c, s = np.cos(ang), -np.sin(ang)
            re_cols = 2 * np.arange(64) + e
            im_cols = (2 * np.arange(64) + 1 + e) % 128
            M = np.zeros((128, 128))
            rr = slice(0, 64) if e == 0 else slice(64, 128)
            ir = slice(64, 128) if e == 0 else slice(0, 64)
            M[rr, re_cols] = c
            M[ir, re_cols] = -s
            M[rr, im_cols] = s
            M[ir, im_cols] = c
            Ms[n2, e] = M
    J = np.zeros((1, 128, 128))
    J[0, l, (128 - l) % 128] = 1.0
    allc = np.concatenate([A, Ai, J, Ms.reshape(32, 128, 128)], 0)
    return allc.astype(np.float32)


CA, CAI, CJ, CM = 0, 4, 8, 9
NCONST = 41


def _add(a, b):
    (x, sx), (y, sy) = a, b
    if sx == sy:
        return (x + y, sx)
    return (x - y, 1) if sx > 0 else (y - x, 1)


def _neg(a):
    return (a[0], -a[1])


def _sub(a, b):
    return _add(a, _neg(b))


def _scale(a, c):
    return (a[0] * (c * a[1]), 1)


def _cadd(a, b):
    return (_add(a[0], b[0]), _add(a[1], b[1]))


def _csub(a, b):
    return (_sub(a[0], b[0]), _sub(a[1], b[1]))


def _mul_mi(a, sgn):
    re, im = a
    return (im, _neg(re)) if sgn > 0 else (_neg(im), re)


def _twiddle(a, j, sgn):
    j = j % 16
    if j % 4 == 0:
        for _ in range(j // 4):
            a = _mul_mi(a, sgn)
        return a
    re, im = a
    if j % 2 == 0:
        if sgn > 0:
            r = _scale(_add(re, im), C8)
            i = _scale(_sub(im, re), C8)
        else:
            r = _scale(_sub(re, im), C8)
            i = _scale(_add(im, re), C8)
        a = (r, i)
        for _ in range(j // 4):
            a = _mul_mi(a, sgn)
        return a
    c = float(np.cos(2 * np.pi * j / 16))
    s = float(-sgn * np.sin(2 * np.pi * j / 16))
    r = _sub(_scale(re, c), _scale(im, s))
    i = _add(_scale(re, s), _scale(im, c))
    return (r, i)


def _dft4(v, sgn):
    a, b, c, d = v
    t0, t1 = _cadd(a, c), _csub(a, c)
    t2, t3 = _cadd(b, d), _mul_mi(_csub(b, d), sgn)
    return [_cadd(t0, t2), _cadd(t1, t3), _csub(t0, t2), _csub(t1, t3)]


def _force(a):
    return a[0] if a[1] > 0 else -a[0]


def _lo_f32(w):
    return pltpu.bitcast(w << 16, F32)


def _hi_f32(w):
    return pltpu.bitcast(w & jnp.uint32(0xFFFF0000), F32)


def _bf(u):
    return pltpu.bitcast(u, BF)


def _lane(shape):
    return jax.lax.broadcasted_iota(jnp.int32, shape, 1)


TM = 256
NCH = S // TM
H = TM // 2
TR = F - 1280
AP = 136
NB = 16
KA, KB = 4, 8
XC = 6
NWAVE = 4
RATE = 1.8
RATE1 = 1.15
C3 = 24
CMID = 24
CG = 110
CCOST = 110
L_PRE = 350
L_LHS = 250
L_MID = 150
L_POST = 450
DLAT = 260
XDL = 100
PDL = 300
GDL = 400
TDL2 = 500
DLQ2 = 48
MBURST = 256
MTPOS = 30


def _kernel(z_hbm, x_hbm, wr_hbm, wi_hbm, w1_hbm, w2_hbm, gw_hbm, c_hbm, o_hbm,
            xb, w1b, w2b, wr_b, wi_b, wl_v, c_b, xr_v, xi_v, yr_b, yi_b, a_v, bb_v, g_v, og_v, o_v, p_v,
            z_ref, gw_ref, gw_f, sems, s_o, *bufs):
    P = functools.partial
    h_b, t_b, z_b, v_b = bufs[:NCH], bufs[NCH:NCH + NB], bufs[NCH + NB:NCH + 2 * NB], bufs[NCH + 2 * NB:]
    x_u, w1_u, w2_u, wr_u, wi_u, c_u, yr_u, yi_u = [
        r.bitcast(U32) for r in (xb, w1b, w2b, wr_b, wi_b, c_b, yr_b, yi_b)]
    h_u, t_u, z_u, v_u = [[r.bitcast(U32) for r in rs] for rs in (h_b, t_b, z_b, v_b)]
    groups = []

    def xrows(r0, r1, cs):
        return [(x_hbm.at[0, pl.ds(r0, r1 - r0), pl.ds(128 * c, 128)], xb.at[c, pl.ds(r0, r1 - r0)]) for c in cs]

    def w1rows(r0, r1, cs):
        return [(w1_hbm.at[pl.ds(r0, r1 - r0), pl.ds(128 * c, 128)], w1b.at[c, pl.ds(r0, r1 - r0)]) for c in cs]

    A4 = range(4)
    groups.append(xrows(0, 2 * TM, [0]) + w1rows(0, 512, [0]))
    groups.append(xrows(2 * TM, 4 * TM, [0]) + w1rows(512, 1024, [0]))
    groups.append(xrows(0, 4 * TM, [1]) + w1rows(0, 1024, [1]) + xrows(0, 4 * TM, [2]) + w1rows(0, 512, [2]))
    groups.append(w1rows(512, 1024, [2]) + xrows(0, 4 * TM, [3]) + w1rows(0, 1024, [3])
                  + w1rows(1024, F, A4) + xrows(4 * TM, XC * TM, A4))
    groups[0].append((z_hbm, z_ref))
    groups[-1].append((gw_hbm, gw_ref))
    rest = xrows(XC * TM, S, A4) + [(c_hbm, c_b)]
    rest += [(w2_hbm.at[:, pl.ds(128 * c, 128)], w2b.at[c, pl.ds(0, F)]) for c in range(4)]
    for k in range(16):
        rest.append((wr_hbm.at[pl.ds(0, 256), pl.ds(128 * k, 128)], wr_b.at[k]))
        rest.append((wi_hbm.at[pl.ds(0, 256), pl.ds(128 * k, 128)], wi_b.at[k]))
    rest.append((wr_hbm.at[pl.ds(256, 1), :], wl_v.at[0]))
    rest.append((wi_hbm.at[pl.ds(256, 1), :], wl_v.at[1]))
    groups.append(rest)
    copies = [[pltpu.make_async_copy(s_, d_, sems.at[gi]) for s_, d_ in g] for gi, g in enumerate(groups)]
    for g in copies:
        for cp in g:
            cp.start()

    def wait(gi):
        for cp in copies[gi]:
            cp.wait()
        if gi == NWAVE - 1:
            for c in range(4):
                gw_f[c] = jnp.broadcast_to(gw_ref[c:c + 1, :].astype(F32), (16, 128))
        if gi == NWAVE:
            for c in range(4):
                w2b[c, pl.ds(F, FP - F), :] = jnp.zeros((FP - F, 128), BF)

    fmask_box = {}
    dlq = []

    def gate(v, tok):
        if v.dtype != tok.dtype:
            tok = pltpu.bitcast(tok, v.dtype)
        return jnp.where(fmask_box['m'], tok, v)

    def new_mask():
        dlq.clear()
        z = z_ref[0]
        fmask_box.clear()
        fmask_box['z'] = z
        fmask_box['m'] = jnp.full((8, 128), z, jnp.int32) != 0

    def oq(k, n):
        if (k, n) not in fmask_box:
            fmask_box[k, n] = jnp.clip(k + fmask_box['z'], 0, n - 1)
        return fmask_box[k, n]

    def gatec(v, tok):
        out = list(v)
        for i in (0, 1):
            (r, sr), (im, si) = v[i]
            out[i] = ((gate(r, tok), sr), (gate(im, tok), si))
        return out

    def cmat(i):
        return _bf(c_u[i])

    def rows8(a, step):
        return [(a[8 * q:8 * q + 8, 0:128], step * q) for q in range(a.shape[0] // 8)]

    state = dict(t=0, nxt=0)

    def push_dl(a, t0, step):
        for v, dt in rows8(a, step):
            dlq.append((v, t0 + dt))

    def lhs(u, dt):
        tok = None
        dlq.sort(key=lambda e: e[1])
        for _ in range(2 if len(dlq) > DLQ2 else 1):
            if dlq and dlq[0][1] <= state['t'] + dt:
                v = pltpu.bitcast(dlq.pop(0)[0], U32)
                tok = v if tok is None else tok | v
        return u if tok is None else gate(u, tok)

    def lhs_par(ops):
        n = ops[0].shape[0] // 8
        g = [[lhs(u[8 * q:8 * q + 8], 16 * q) for u in ops] for q in range(n)]
        return [_bf(jnp.concatenate([g[q][k] for q in range(n)], 0)) for k in range(len(ops))]

    T1s = {}
    Zs = {}

    def p1_pre(n2, gam, tok):
        unp = _hi_f32 if n2 % 2 else _lo_f32
        lo = _lane((8, 128)) < 64
        r0 = n2 // 2 + 64 * gam
        a = [unp(gate(x_u[c, pl.ds(r0, 8, stride=8), :], tok)) for c in range(4)]
        b = [unp(x_u[c, pl.ds(r0 + 512, 8, stride=8), :]) for c in range(4)]
        for e in range(2):
            U = [a[c] + b[c] if e == 0 else a[c] - b[c] for c in range(4)]
            p0, p1_, m0, m1 = U[0] + U[2], U[1] + U[3], U[0] - U[2], U[1] - U[3]
            Pv = jnp.where(lo, m0, (m0 + m1) * (-C8))
            Qn = pltpu.roll(jnp.where(lo, m1, (m1 - m0) * C8), 64, 1)
            for t, val in enumerate([p0 + p1_, p0 - p1_, Pv - Qn, Pv + Qn]):
                if gam % 2 == 0:
                    T1s[n2, t, e] = val
                else:
                    pair = jnp.concatenate([T1s.pop((n2, t, e)), val], 0)
                    t_b[n2][t, pl.ds(64 * e + 8 * (gam - 1), 16), :] = pair.astype(BF)
                if t == 2:
                    dlq.append((val, state['now'] + PDL))

    def p1_d(n2):
        As = lhs_par([c_u[CA + t] for t in range(4)])
        for t in range(4):
            Z = jax.lax.dot_general(As[t], _bf(t_u[n2][oq(t, 4)]), NT, preferred_element_type=F32)
            z_b[n2][t] = Z.astype(BF)
        return rows8(Z, 8), 128

    def p1_mid(n2, t, tok):
        lo = _lane((32, 128)) < 64
        z = z_u[n2][oq(t, 4)]
        ZR = z[:32]
        RI = pltpu.roll(jnp.concatenate([gate(z[32 + 8 * q:40 + 8 * q], tok) for q in range(4)], 0), 64, 1)
        Zs[n2, 0, t] = jnp.where(lo, ZR, RI)
        Zs[n2, 1, t] = jnp.where(lo, RI, ZR)
        push_dl(Zs[n2, 0, t], state['now'] + PDL, 4)

    def p1_s(n2):
        T0, T1 = [jnp.concatenate([Zs.pop((n2, e, t)) for t in range(4)], 0) for e in range(2)]
        even = (_lane((128, 128)) % 2) == 0
        xi = []
        Ls = lhs_par([T0[:64], T1[:64], T0[64:], T1[64:]])
        for hf in range(2):
            O0 = jnp.dot(Ls[2 * hf], cmat(CM + 2 * n2), preferred_element_type=F32)
            O1 = jnp.dot(Ls[2 * hf + 1], cmat(CM + 2 * n2 + 1), preferred_element_type=F32)
            xr_v[n2, 128 * hf:128 * hf + 128, :] = jnp.where(even, O0, O1)
            xi.append(pltpu.roll(jnp.where(even, O1, O0), 127, 1))
            xi_v[n2, 128 * hf:128 * hf + 128, :] = xi[-1]
        for q in range(16):
            for hf in range(2):
                dlq.append((xi[hf][8 * q:8 * q + 8], state['t'] + DLAT + XDL + 8 * q))
        return rows8(O1, 8), 128

    def p2_items(grp):
        row = pl.ds(8 * grp, 8)
        kd0 = _kd_of_row(8 * grp)
        wrow = pl.ds(kd0 // 2, 8, stride=(_kd_of_row(8 * grp + 1) - kd0) // 2)
        unp = _hi_f32 if kd0 % 2 else _lo_f32
        y = [[None] * 4 for _ in range(4)]
        z = [[None] * 4 for _ in range(4)]
        X = [None] * 16
        Y = [None] * 16
        st = {}

        def f1(b, tok):
            v = [((xr_v[oq(4 * a + b, 16), row, :], 1), (xi_v[oq(4 * a + b, 16), row, :], 1)) for a in range(4)]
            o = _dft4(gatec(v, tok), +1)
            for kap in range(4):
                y[kap][b] = _twiddle(o[kap], b * kap, +1)

        def mid_a(kap, tok):
            o = _dft4(gatec(y[kap], tok), +1)
            for io in range(4):
                k = kap + 4 * io
                wr = unp(wr_u[k, wrow, :])
                wi = unp(wi_u[k, wrow, :])
                X[k] = o[io]
                (xr, sr), (xi, si) = o[io]
                Y[k] = (_sub((xr * wr, sr), (xi * wi, si)), _add((xr * wi, sr), (xi * wr, si)))

        def mid_b(kap):
            o2 = _dft4([Y[kap + 4 * io] for io in range(4)], -1)
            for b2 in range(4):
                z[b2][kap] = _twiddle(o2[b2], kap * b2, -1)

        def mid(kap, tok):
            mid_a(kap, tok)
            mid_b(kap)

        def i2(b2, tok):
            o = _dft4(gatec(z[b2], tok), -1)
            for io in range(4):
                yr_b[b2 + 4 * io, row, :] = _force(o[io][0]).astype(BF)
                yi_b[b2 + 4 * io, row, :] = _force(o[io][1]).astype(BF)

        def sp_stack(k, tok):
            sub = jax.lax.broadcasted_iota(jnp.int32, (8, 128), 0)
            w0r = unp(wr_u[k, wrow, :])[0:1]
            w0i = unp(wi_u[k, wrow, :])[0:1]
            wlr = wl_v[0, :, 128 * k:128 * k + 128].astype(F32)
            wli = wl_v[1, :, 128 * k:128 * k + 128].astype(F32)
            pr = gate(_force(X[k][0]), tok)[0:1]
            pi = _force(X[k][1])[0:1]
            blk = jnp.zeros((8, 128), F32)
            for jj, r in enumerate([pr, pi, w0r, w0i, wlr, wli]):
                blk = jnp.where(sub == jj, jnp.broadcast_to(r, (8, 128)), blk)
            st[k] = blk

        def sp_flip():
            full = jnp.concatenate([st[k] for k in range(16)], 0)
            fl = []
            for hf in range(2):
                part = full[64 * hf:64 * hf + 64]
                hi_ = part.astype(BF)
                lo_ = (part - hi_.astype(F32)).astype(BF)
                fh = jnp.dot(hi_, cmat(CJ), preferred_element_type=F32)
                fl.append(jnp.dot(lo_, cmat(CJ), preferred_element_type=F32) + fh)
            fl = jnp.concatenate(fl, 0)
            st['fl'] = fl
            return rows8(fl, 4), 64

        def sp_fix(k, tok):
            sub = jax.lax.broadcasted_iota(jnp.int32, (8, 128), 0)
            fl = st['fl']
            fa = fl[8 * (15 - k):8 * (15 - k) + 8]
            fb = fl[8 * ((16 - k) % 16):8 * ((16 - k) % 16) + 8]
            f = gate(jnp.where(_lane((8, 128)) == 0, fb, fa), tok)
            o = st[k]
            pr, pi, w0r, w0i, wlr, wli = [o[jj:jj + 1] for jj in range(6)]
            fpr, fpi, f0r, f0i, flr, fli = [f[jj:jj + 1] for jj in range(6)]
            s0r, s0i = w0r + f0r, w0i - f0i
            slr, sli = wlr + flr, wli - fli
            Ar, Ai_ = (s0r + slr) * 0.25, (s0i + sli) * 0.25
            Br, Bi = (s0r - slr) * 0.25, (s0i - sli) * 0.25
            yr0 = pr * Ar - pi * Ai_ + fpr * Br + fpi * Bi
            yi0 = pr * Ai_ + pi * Ar + fpr * Bi - fpi * Br
            yr = jnp.where(sub == 0, jnp.broadcast_to(yr0, (8, 128)), _force(Y[k][0]))
            yi = jnp.where(sub == 0, jnp.broadcast_to(yi0, (8, 128)), _force(Y[k][1]))
            Y[k] = ((yr, 1), (yi, 1))
            dlq.append((yr, state['t'] + 400))
            dlq.append((yi, state['t'] + 400))
            if k >= 12:
                mid_b(k - 12)

        first = [('v', P(f1, b), 30) for b in range(4)]
        last = [('v', P(i2, b), 28) for b in range(4)]
        if grp != 0:
            return first + [('v', P(mid, k), 78) for k in range(4)] + last, []
        a = (first + [('v', P(mid_a, k), 52) for k in range(4)] + [('v', P(sp_stack, k), 24) for k in range(16)]
             + [('m', sp_flip, 64)])
        b = [('v', P(sp_fix, k), 50 + (26 if k >= 12 else 0)) for k in range(16)] + last
        return a, b

    B3 = {}
    V3 = {}

    def p3_pre(n2, q, tok):
        even = (_lane((32, 128)) % 2) == 0
        Ru = yr_u[oq(n2, 16), pl.ds(32 * q, 32), :]
        Iu = yi_u[oq(n2, 16), pl.ds(32 * q, 32), :]
        Ou = pltpu.roll(jnp.concatenate([gate(Iu[8 * i:8 * i + 8], tok) for i in range(4)], 0), 1, 1)
        B3[n2, 0, q] = jnp.where(even, Ru, Ou)
        B3[n2, 1, q] = jnp.where(even, Ou, Ru)
        push_dl(B3[n2, 0, q], state['now'] + PDL, 4)

    def p3_s(n2):
        V = []
        Ms_ = lhs_par([c_u[CM + 2 * n2 + e] for e in range(2)])
        for e in range(2):
            B = _bf(jnp.concatenate([B3.pop((n2, e, q)) for q in range(4)], 0))
            V.append(jax.lax.dot_general(Ms_[e], B, NT, preferred_element_type=F32))
        V0, V1 = V
        V0r, V0i = V0[:64], V0[64:]
        V1i, V1r = V1[:64], V1[64:]
        VR = jnp.concatenate([V0r + V1r, V0r - V1r], 0)
        VI = jnp.concatenate([V0i + V1i, V0i - V1i], 0)
        for hf in range(2):
            v_b[n2][hf] = VR[:, 128 * hf:128 * hf + 128].astype(BF)
            v_b[n2][2 + hf] = VI[:, 128 * hf:128 * hf + 128].astype(BF)
        return rows8(V[1], 8), 128

    def p3_mid(n2, q, tok):
        hf, o = q // 2, 32 * (q % 2)
        lo = _lane((32, 128)) < 64
        r = v_u[n2][oq(hf, 4), pl.ds(o, 32), :]
        im = v_u[n2][oq(2 + hf, 4), pl.ds(o, 32), :]
        ri = pltpu.roll(jnp.concatenate([gate(im[8 * i:8 * i + 8], tok) for i in range(4)], 0), 64, 1)
        V3[n2, 2 * hf, q % 2] = jnp.where(lo, r, ri)
        V3[n2, 2 * hf + 1, q % 2] = jnp.where(lo, ri, r)
        push_dl(V3[n2, 2 * hf, q % 2], state['now'] + PDL, 4)

    def p3_d(r0):
        Gl = lhs_par([jnp.concatenate([V3.pop((n2, t, k)) for n2 in (2 * r0, 2 * r0 + 1) for k in range(2)], 0)
                      for t in range(4)])
        o = [jnp.dot(Gl[t], cmat(CAI + t), preferred_element_type=F32) for t in range(4)]
        v0, v2, T1, T3 = o
        lo = _lane((256, 128)) < 64
        Pp = T1 + T3
        Qp = pltpu.roll(T1 - T3, 64, 1)
        m0 = jnp.where(lo, Pp, (Qp - Pp) * C8)
        m1n = jnp.where(lo, Qp, (Pp + Qp) * C8)
        p0, p1_ = v0 + v2, v0 - v2
        y = [p0 + m0, p1_ - m1n, p0 - m0, p1_ + m1n]
        for s_ in range(2):
            for c in range(4):
                a_v[c, pl.ds(AP * (2 * r0 + s_), 128), :] = y[c][128 * s_:128 * s_ + 128]
        push_dl(m0, state['t'] + DLAT + 16, 8)
        push_dl(m1n, state['t'] + DLAT + 16, 8)
        return rows8(v0, 8), 256

    h_done = set()
    when = {}

    def m1(i, js, cs, defer):
        r2 = i * H
        xs = [[lhs(x_u[c, pl.ds(r2 + 8 * q, 8), :], 16 * q) for c in cs] for q in range(H // 8)]
        xc = jnp.concatenate([_bf(jnp.concatenate([xq[k] for xq in xs], 0)) for k in range(len(cs))], 1)
        w1 = jnp.concatenate([_bf(w1_u[c, pl.ds(64 * js[0], 64 * len(js)), :]) for c in cs], 1)
        raw = jax.lax.dot_general(xc, w1, NT, preferred_element_type=F32)

        def post(lat):
            for k, j in enumerate(js):
                r = raw[:, 128 * k:128 * k + 128]
                if cs[0] > 0:
                    r = r + p_v[i, j]
                if cs[-1] < 3:
                    p_v[i, j] = r
                    continue
                t = 0.5 * r
                th = jnp.tanh(t)
                t0 = state['t'] + lat + TM * k
                hs = t + t * th
                h_b[i][j] = hs.astype(BF)
                h_done.add((i, j))
                for q in range(TM // 16):
                    dlq.append((hs[16 * q + 8:16 * q + 16], t0 + 16 + 16 * q))
        if defer:
            pending.append(post)
        else:
            post(DLAT)
        return rows8(raw, 8), TM

    def gate_pk(b, tok):
        s_ = None
        for c in range(4):
            xv = _bf(gate(x_u[c, pl.ds(8 * b, 8), :], tok)).astype(F32) * gw_f[oq(c, 4)]
            s_ = xv if s_ is None else s_ + xv
        lg = jnp.broadcast_to(jnp.sum(s_, axis=1, keepdims=True), (16, 128))
        tg = 0.5 * jnp.tanh(0.5 * lg)
        g_v[b // 8, pl.ds(16 * (b % 8), 16), :] = 0.5 + tg
        og_v[pl.ds(16 * b, 16), :] = 0.5 - tg
        push_dl(tg, state['now'] + GDL, 0)

    def mt(i):
        toks = []
        for ii in range(TM // 128):
            b = (TM // 128) * i + ii
            Ls = lhs_par([w1_u[c, pl.ds(640, TR // 2), :] for c in range(4)])
            xw = jnp.concatenate([_bf(x_u[c, pl.ds(64 * b, 64), :]) for c in range(4)], 1)
            raw = jax.lax.dot_general(jnp.concatenate(Ls, 1), xw, NT, preferred_element_type=F32)
            t = 0.5 * raw
            hs = t + t * jnp.tanh(t)
            full = jnp.concatenate([hs, jnp.zeros((128 - TR, 128), F32)], 0).T
            h_b[i][10, pl.ds(128 * ii, 128), :] = full.astype(BF)
            push_dl(full, state['t'] + TR + TDL2, 8)
            for tok, dt in rows8(raw, 8):
                toks.append((tok, TR * ii + dt))
            state['t'] += TR
        state['t'] -= TR * (TM // 128)
        h_done.add((i, 10))
        return toks, TR * (TM // 128)

    pending = []

    def flush():
        while pending:
            pending.pop()(64)

    accs = {}

    def m2(i, g):
        assert all((i, j) in h_done for j in range(11))
        assert all(('gate', b) in when for b in range(i * TM // 16, (i + 1) * TM // 16))
        cj = [divmod(f, 11) for f in range(4 * g, 4 * g + 4)]
        hq = [[lhs(h_u[i][oq(j, 11), pl.ds(8 * q, 8), :], 16 * q) for _, j in cj] for q in range(H // 8)]
        fin = []
        for c in sorted(set(c for c, _ in cj)):
            ks = [k for k in range(4) if cj[k][0] == c]
            j0 = cj[ks[0]][1]
            hs = jnp.concatenate([_bf(jnp.concatenate([hq_[k] for hq_ in hq], 0)) for k in ks], 1)
            o = jnp.dot(hs, _bf(w2_u[c, pl.ds(64 * j0, 64 * len(ks)), :]), preferred_element_type=F32)
            acc = o if j0 == 0 else o + accs.pop((i, c))
            if j0 + len(ks) < 11:
                accs[i, c] = acc
            else:
                bb_v[c, pl.ds(i * TM, TM), :] = acc * og_v[pl.ds(i * TM, TM), :]
                fin.append(c)
        return rows8(acc, 8), TM, fin

    def out_copy(i, c):
        return pltpu.make_async_copy(o_v.at[c, pl.ds(128 * i, 128)],
                                     o_hbm.at[0, pl.ds(128 * i, 128), pl.ds(128 * c, 128)], s_o.at[0])

    def combine(i, c, tok):
        av = []
        for n in range(8):
            for hf in range(2):
                a = a_v[c, pl.ds(8 * hf * AP + 8 * i + n, 8, stride=AP), :]
                av.append(a if tok is None else gate(a, tok))
        b = bb_v[c, pl.ds(128 * i, 128), :]
        o = g_v[oq(i, 16)] * jnp.concatenate(av, 0) + b
        o_v[c, pl.ds(128 * i, 128), :] = o.astype(BF)
        out_copy(i, c).start()

    VQ, MQ = [], []
    for b in range(XC * TM // 16):
        VQ.append((('gate', b), P(gate_pk, b), CG, [('xall', 0)]))

    def pre1(r0):
        for n2 in (2 * r0, 2 * r0 + 1):
            for gam in range(8):
                deps = [('rest', 0)] + ([(('d1', 2 * (r0 - 2)), 0)] if r0 >= 2 else [])
                VQ.append((('pre1', n2, gam), P(p1_pre, n2, gam), 58 * RATE / RATE1, deps))

    def mid(name, dep, fn, r0):
        for n2 in (2 * r0, 2 * r0 + 1):
            for q in range(4):
                VQ.append(((name, n2, q), P(fn, n2, q), CMID, [((dep, n2), L_MID)]))
    for r0 in range(10):
        if r0 < 8:
            pre1(r0)
        if r0 >= 2:
            mid('mid1', 'd1', p1_mid, r0 - 2)
    for r0 in range(10):
        if r0 < 8:
            for n2 in (2 * r0, 2 * r0 + 1):
                MQ.append((('d1', n2), P(p1_d, n2), [(('pre1', n2, 7), L_PRE)]))
        if r0 >= 2:
            for n2 in (2 * r0 - 4, 2 * r0 - 3):
                MQ.append((('s1', n2), P(p1_s, n2), [(('mid1', n2, 3), L_LHS)]))
    late_gates = list(range(XC * TM // 16, S // 16))
    kp = [0]

    def add2(items, extra=()):
        for it in items:
            kp[0] += 1
            if it[0] == 'v':
                VQ.append((('p2', kp[0]), it[1], it[2], list(extra) + [(('s1', 15), L_POST)]))
            else:
                MQ.append(('flip', it[1], [(('p2', kp[0] - 1), L_PRE)]))
    a0, b0 = p2_items(0)
    add2(a0)
    for g in range(1, 4):
        add2(p2_items(g)[0])
    add2(b0, [('flip', 250)])
    for g in range(4, 32):
        for b in late_gates[2 * (g - 4):2 * (g - 4) + 2]:
            VQ.append((('gate', b), P(gate_pk, b), 40, [('rest', 0)]))
        add2(p2_items(g)[0])
    last2 = [(VQ[-1][0], 100)]
    for r0 in range(9):
        if r0 < 8:
            for n2 in (2 * r0, 2 * r0 + 1):
                for q in range(4):
                    VQ.append((('pre3', n2, q), P(p3_pre, n2, q), C3, last2))
        if r0 >= 1:
            mid('mid3', 's3', p3_mid, r0 - 1)
    for r0 in range(9):
        if r0 < 8:
            for n2 in (2 * r0, 2 * r0 + 1):
                MQ.append((('s3', n2), P(p3_s, n2), [(('pre3', n2, 3), L_PRE)]))
        if r0 >= 1:
            MQ.append((('d3', r0 - 1), P(p3_d, r0 - 1), [(('mid3', 2 * r0 - 1, 3), L_LHS)]))
    for i in range(NCH):
        for c in range(4):
            for ii in range(TM // 128):
                VQ.append((('cmb', i, c, ii), P(combine, (TM // 128) * i + ii, c), CCOST,
                           [(('d3', 7), L_POST + 256), (('m2', i, c), 0)]))

    pieces = [('m1', 0, i, (0, 1, 2, 3), (0,)) for i in range(2)]
    pieces += [('m1', 1, i, js, (0,)) for i in range(4) for js in ((0, 1, 2, 3), (4, 5, 6, 7)) if i >= 2 or js[0] == 4]
    for i in range(4):
        pieces += [('m1', 2, i, (0, 1), (1, 2)), ('m1', 2, i, (2, 3), (1, 2)), ('m1', 2, i, (4, 5, 6, 7), (1,))]
    ks = []
    for i in range(4):
        ks += [('m1', 3, i, (0, 1, 2, 3), (3,)), ('m1', 3, i, (4, 5), (2, 3)), ('m1', 3, i, (6, 7), (2, 3))]
    full = [('m1', 3, i, (j,), (0, 1, 2, 3)) for i in range(XC) for j in range(10) if i >= KA or j >= KB]
    last = [('m1', 3, i, (10,), (0, 1, 2, 3)) for i in range(XC)]
    while ks or full or last:
        pieces += ks[:1] + full[:2] + ks[1:2] + full[2:3] + last[:1] + full[3:4]
        ks, last, full = ks[2:], last[1:], full[4:]
    wwait = len(pieces)
    pieces += [('m1', 3, i, (j,), (0, 1, 2, 3)) for i in range(XC, NCH) for j in range(10)]
    m2s = [('m2', i, g) for i in range(NCH) for g in range(11)]
    for k, i in enumerate(range(XC, NCH)):
        m2s.insert(MTPOS + 3 * k, ('m1', 3, i, (10,), (0, 1, 2, 3)))
    pieces += m2s

    def ok(deps, now):
        return all(d in when and when[d] + dl <= now for d, dl in deps)

    def issue(toks, cost):
        for tok, dt in toks:
            now = state['t'] + dt
            if VQ and now >= state['nxt'] and ok(VQ[0][3], now):
                name, fn, ops, _ = VQ.pop(0)
                state['now'] = now
                fn(tok)
                when[name] = now
                state['nxt'] = max(state['nxt'], now - 8) + ops / RATE
        state['t'] += cost

    def try_mxu():
        t0 = state['t']
        while MQ and ok(MQ[0][2], state['t']) and state['t'] - t0 < MBURST:
            name, fn, _ = MQ.pop(0)
            when[name] = state['t']
            issue(*fn())

    wv_done = -1
    for n, pc in enumerate(pieces):
        if pc[0] == 'm1' and pc[1] > wv_done:
            wv_done = pc[1]
            wait(wv_done)
            new_mask()
            flush()
            if wv_done == NWAVE - 1:
                when['xall'] = state['t']
        if n == wwait:
            wait(NWAVE)
            new_mask()
            flush()
            when['rest'] = state['t']
        try_mxu()
        if pc[0] == 'm1' and pc[3] == (10,):
            issue(*mt(pc[2]))
        elif pc[0] == 'm1':
            issue(*m1(pc[2], pc[3], pc[4], len(pc[3]) == 1 and n + 1 == wwait))
        else:
            toks, cost, fin = m2(pc[1], pc[2])
            issue(toks, cost)
            for c in fin:
                when['m2', pc[1], c] = state['t']
    assert not MQ
    for it in VQ:
        assert it[0][0] == 'cmb', it[0]
        it[1](None)
    for i in range(16):
        for c in range(4):
            out_copy(i, c).wait()


@jax.jit
def pallas_gated_mix__spectral_gfnet__dense_activation_silu__prompt_kernel(A_x, A_w_r, A_w_i, B_x, B_w1, B_w2, gate_w):
    consts = jnp.asarray(_consts(), dtype=BF)
    zero = jnp.zeros((1,), jnp.int32)
    hbm = pl.BlockSpec(memory_space=pltpu.HBM)
    dma = pltpu.SemaphoreType.DMA
    return pl.pallas_call(
        _kernel,
        in_specs=[hbm] * 8,
        out_specs=hbm,
        out_shape=jax.ShapeDtypeStruct((1, S, D), BF),
        scratch_shapes=[
            pltpu.VMEM((4, S, 128), BF),
            pltpu.VMEM((4, F, 128), BF),
            pltpu.VMEM((4, FP, 128), BF),
            pltpu.VMEM((16, 256, 128), BF),
            pltpu.VMEM((16, 256, 128), BF),
            pltpu.VMEM((2, 1, S), BF),
            pltpu.VMEM((NCONST, 128, 128), BF),
            pltpu.VMEM((16, 256, 128), F32),
            pltpu.VMEM((16, 256, 128), F32),
            pltpu.VMEM((16, 256, 128), BF),
            pltpu.VMEM((16, 256, 128), BF),
            pltpu.VMEM((4, 16 * AP, 128), F32),
            pltpu.VMEM((4, S, 128), F32),
            pltpu.VMEM((16, 128, 128), F32),
            pltpu.VMEM((S, 128), F32),
            pltpu.VMEM((4, S, 128), BF),
            pltpu.VMEM((KA, KB, TM, 128), F32),
            pltpu.SMEM((1,), jnp.int32),
            pltpu.VMEM((4, 128), BF),
            pltpu.VMEM((4, 16, 128), F32),
            dma((NWAVE + 1,)), dma((1,)),
        ] + [pltpu.VMEM((11, TM, 128), BF) for _ in range(NCH)]
        + [pltpu.VMEM((4, 128, 128), BF) for _ in range(3 * NB)],
        compiler_params=pltpu.CompilerParams(vmem_limit_bytes=100 << 20),
    )(zero, A_x, A_w_r.T, A_w_i.T, B_w1.T, B_w2, gate_w.reshape(4, 128), consts)
```

```python
import functools
import numpy as np
import jax
import jax.numpy as jnp
import jax.experimental.pallas as pl
import jax.experimental.pallas.tpu as pltpu

S, D, F = 2048, 512, 1376
FP = 1408
ODD = ((1, 7), (5, 3))
BF = jnp.bfloat16
F32 = jnp.float32
U32 = jnp.uint32
C8 = float(np.sqrt(0.5))
NT = (((1,), (1,)), ((), ()))


def _kd_of_row(rho):
    t, i = divmod(rho, 64)
    return 4 * i + 2 * t if t < 2 else 8 * (i % 32) + ODD[t - 2][i // 32]


@functools.lru_cache(maxsize=None)
def _consts():
    l = np.arange(128)
    A = np.zeros((4, 128, 128))
    for t in range(4):
        for i in range(64):
            rho = 64 * t + i
            kd = _kd_of_row(rho)
            if t < 2:
                ang = 2 * np.pi * ((l * kd) % 512) / 512
                A[t, i] = np.cos(ang)
                A[t, 64 + i] = -np.sin(ang)
                if rho == 0:
                    A[t, 64] = np.where(l % 2 == 0, 1.0, -1.0)
            else:
                f = t - 2
                lp = np.arange(64)
                k, cj = (kd, 1.0) if kd % 8 == 1 + 4 * f else (512 - kd, -1.0)
                ang = 2 * np.pi * ((lp * k) % 512) / 512
                c, s = np.cos(ang), -np.sin(ang)
                sg = 1.0 if f == 0 else -1.0
                A[t, i, :64] = c
                A[t, i, 64:] = -s * sg
                A[t, 64 + i, :64] = cj * s
                A[t, 64 + i, 64:] = cj * c * sg
    Ai = np.zeros((4, 128, 128))
    for t in range(4):
        sc = np.full(128, 2.0 / (S * D))
        if t == 0:
            sc[0] = sc[64] = 1.0 / (S * D)
        M = A[t] * sc[:, None]
        Ai[t] = M if t % 2 == 0 else np.concatenate([M[64:], M[:64]], 0)
    Ms = np.zeros((16, 2, 128, 128))
    n1 = np.arange(64)[:, None]
    k1 = np.arange(64)[None, :]
    for e in range(2):
        for n2 in range(16):
            ang = 2 * np.pi * (((16 * n1 + n2) * (e + 2 * k1)) % 2048) / 2048
            c, s = np.cos(ang), -np.sin(ang)
            re_cols = 2 * np.arange(64) + e
            im_cols = (2 * np.arange(64) + 1 + e) % 128
            M = np.zeros((128, 128))
            rr = slice(0, 64) if e == 0 else slice(64, 128)
            ir = slice(64, 128) if e == 0 else slice(0, 64)
            M[rr, re_cols] = c
            M[ir, re_cols] = -s
            M[rr, im_cols] = s
            M[ir, im_cols] = c
            Ms[n2, e] = M
    J = np.zeros((1, 128, 128))
    J[0, l, (128 - l) % 128] = 1.0
    allc = np.concatenate([A, Ai, J, Ms.reshape(32, 128, 128)], 0)
    return allc.astype(np.float32)


CA, CAI, CJ, CM = 0, 4, 8, 9
NCONST = 41


def _add(a, b):
    (x, sx), (y, sy) = a, b
    if sx == sy:
        return (x + y, sx)
    return (x - y, 1) if sx > 0 else (y - x, 1)


def _neg(a):
    return (a[0], -a[1])


def _sub(a, b):
    return _add(a, _neg(b))


def _scale(a, c):
    return (a[0] * (c * a[1]), 1)


def _cadd(a, b):
    return (_add(a[0], b[0]), _add(a[1], b[1]))


def _csub(a, b):
    return (_sub(a[0], b[0]), _sub(a[1], b[1]))


def _mul_mi(a, sgn):
    re, im = a
    return (im, _neg(re)) if sgn > 0 else (_neg(im), re)


def _twiddle(a, j, sgn):
    j = j % 16
    if j % 4 == 0:
        for _ in range(j // 4):
            a = _mul_mi(a, sgn)
        return a
    re, im = a
    if j % 2 == 0:
        if sgn > 0:
            r = _scale(_add(re, im), C8)
            i = _scale(_sub(im, re), C8)
        else:
            r = _scale(_sub(re, im), C8)
            i = _scale(_add(im, re), C8)
        a = (r, i)
        for _ in range(j // 4):
            a = _mul_mi(a, sgn)
        return a
    c = float(np.cos(2 * np.pi * j / 16))
    s = float(-sgn * np.sin(2 * np.pi * j / 16))
    r = _sub(_scale(re, c), _scale(im, s))
    i = _add(_scale(re, s), _scale(im, c))
    return (r, i)


def _dft4(v, sgn):
    a, b, c, d = v
    t0, t1 = _cadd(a, c), _csub(a, c)
    t2, t3 = _cadd(b, d), _mul_mi(_csub(b, d), sgn)
    return [_cadd(t0, t2), _cadd(t1, t3), _csub(t0, t2), _csub(t1, t3)]


def _force(a):
    return a[0] if a[1] > 0 else -a[0]


def _lo_f32(w):
    return pltpu.bitcast(w << 16, F32)


def _hi_f32(w):
    return pltpu.bitcast(w & jnp.uint32(0xFFFF0000), F32)


def _bf(u):
    return pltpu.bitcast(u, BF)


def _lane(shape):
    return jax.lax.broadcasted_iota(jnp.int32, shape, 1)


TM = 256
NCH = S // TM
H = TM // 2
TR = F - 1280
AP = 136
NB = 16
KA, KB = 4, 8
XC = 6
NWAVE = 4
RATE = 1.8
RATE1 = 1.15
C3 = 24
CMID = 24
CG = 110
CCOST = 110
L_PRE = 350
L_LHS = 250
L_MID = 150
L_POST = 450
DLAT = 260
XDL = 100
PDL = 300
GDL = 400
TDL2 = 500
DLQ2 = 48
MBURST = 256
MTPOS = 30


def _kernel(z_hbm, x_hbm, wr_hbm, wi_hbm, w1_hbm, w2_hbm, gw_hbm, c_hbm, o_hbm,
            w2b, wr_b, wi_b, wl_v, c_b, xr_v, xi_v, yr_b, yi_b, a_v, bb_v, g_v, og_v, o_v, p_v,
            z_ref, gw_ref, gw_f, sems, s_o, *bufs):
    P = functools.partial
    bufs = list(bufs)
    h_b, t_b, z_b, v_b, x_b, w1_b = [[bufs.pop(0) for _ in range(n)] for n in (NCH, NB, NB, NB, 16, 12)]
    w2_u, wr_u, wi_u, c_u, yr_u, yi_u = [r.bitcast(U32) for r in (w2b, wr_b, wi_b, c_b, yr_b, yi_b)]
    h_u, t_u, z_u, v_u, x_v, w1_v = [[r.bitcast(U32) for r in rs] for rs in (h_b, t_b, z_b, v_b, x_b, w1_b)]

    def x_u(c, r, n, stride=1):
        return x_v[4 * (r // 256) + c][pl.ds(r % 256, n, stride=stride), :]

    def w1_u(c, r, n):
        return w1_v[4 * (r // 256) + c][pl.ds(r % 256, n), :]

    groups = []

    def xrows(r0, r1, cs):
        return [(x_hbm.at[0, pl.ds(r, 512), pl.ds(128 * c, 128)], x_b[4 * (r // 512) + c])
                for c in cs for r in range(r0, r1, 512)]

    def w1rows(r0, r1, cs):
        return [(w1_hbm.at[pl.ds(r, min(512, F - r)), pl.ds(128 * c, 128)], w1_b[4 * (r // 512) + c])
                for c in cs for r in range(r0, r1, 512)]

    A4 = range(4)
    groups.append(xrows(0, 2 * TM, [0]) + w1rows(0, 512, [0]))
    groups.append(xrows(2 * TM, 4 * TM, [0]) + w1rows(512, 1024, [0]))
    groups.append(xrows(0, 4 * TM, [1]) + w1rows(0, 1024, [1]) + xrows(0, 4 * TM, [2]) + w1rows(0, 512, [2]))
    groups.append(w1rows(512, 1024, [2]) + xrows(0, 4 * TM, [3]) + w1rows(0, 1024, [3])
                  + w1rows(1024, F, A4) + xrows(4 * TM, XC * TM, A4))
    groups[0].append((z_hbm, z_ref))
    groups[-1].append((gw_hbm, gw_ref))
    rest = xrows(XC * TM, S, A4) + [(c_hbm, c_b)]
    rest += [(w2_hbm.at[:, pl.ds(128 * c, 128)], w2b.at[c, pl.ds(0, F)]) for c in range(4)]
    for k in range(16):
        rest.append((wr_hbm.at[pl.ds(0, 256), pl.ds(128 * k, 128)], wr_b.at[k]))
        rest.append((wi_hbm.at[pl.ds(0, 256), pl.ds(128 * k, 128)], wi_b.at[k]))
    rest.append((wr_hbm.at[pl.ds(256, 1), :], wl_v.at[0]))
    rest.append((wi_hbm.at[pl.ds(256, 1), :], wl_v.at[1]))
    groups.append(rest)
    copies = [[pltpu.make_async_copy(s_, d_, sems.at[gi]) for s_, d_ in g] for gi, g in enumerate(groups)]
    for g in copies:
        for cp in g:
            cp.start()

    def wait(gi):
        for cp in copies[gi]:
            cp.wait()
        if gi == NWAVE - 1:
            for c in range(4):
                gw_f[c] = jnp.broadcast_to(gw_ref[c:c + 1, :].astype(F32), (16, 128))
        if gi == NWAVE:
            for c in range(4):
                w2b[c, pl.ds(F, FP - F), :] = jnp.zeros((FP - F, 128), BF)

    fmask_box = {}
    dlq = []

    def gate(v, tok):
        if v.dtype != tok.dtype:
            tok = pltpu.bitcast(tok, v.dtype)
        return jnp.where(fmask_box['m'], tok, v)

    def new_mask():
        dlq.clear()
        z = z_ref[0]
        fmask_box.clear()
        fmask_box['z'] = z
        fmask_box['m'] = jnp.full((8, 128), z, jnp.int32) != 0

    def oq(k, n):
        if (k, n) not in fmask_box:
            fmask_box[k, n] = jnp.clip(k + fmask_box['z'], 0, n - 1)
        return fmask_box[k, n]

    def gatec(v, tok):
        out = list(v)
        for i in (0, 1):
            (r, sr), (im, si) = v[i]
            out[i] = ((gate(r, tok), sr), (gate(im, tok), si))
        return out

    def cmat(i):
        return _bf(c_u[i])

    def rows8(a, step):
        return [(a[8 * q:8 * q + 8, 0:128], step * q) for q in range(a.shape[0] // 8)]

    state = dict(t=0, nxt=0)

    def push_dl(a, t0, step):
        for v, dt in rows8(a, step):
            dlq.append((v, t0 + dt))

    def lhs(u, dt):
        tok = None
        dlq.sort(key=lambda e: e[1])
        for _ in range(2 if len(dlq) > DLQ2 else 1):
            if dlq and dlq[0][1] <= state['t'] + dt:
                v = pltpu.bitcast(dlq.pop(0)[0], U32)
                tok = v if tok is None else tok | v
        return u if tok is None else gate(u, tok)

    def lhs_par(ops):
        n = ops[0].shape[0] // 8
        g = [[lhs(u[8 * q:8 * q + 8], 16 * q) for u in ops] for q in range(n)]
        return [_bf(jnp.concatenate([g[q][k] for q in range(n)], 0)) for k in range(len(ops))]

    T1s = {}
    Zs = {}

    def p1_pre(n2, gam, tok):
        unp = _hi_f32 if n2 % 2 else _lo_f32
        lo = _lane((8, 128)) < 64
        r0 = n2 // 2 + 64 * gam
        a = [unp(gate(x_u(c, r0, 8, 8), tok)) for c in range(4)]
        b = [unp(x_u(c, r0 + 512, 8, 8)) for c in range(4)]
        for e in range(2):
            U = [a[c] + b[c] if e == 0 else a[c] - b[c] for c in range(4)]
            p0, p1_, m0, m1 = U[0] + U[2], U[1] + U[3], U[0] - U[2], U[1] - U[3]
            Pv = jnp.where(lo, m0, (m0 + m1) * (-C8))
            Qn = pltpu.roll(jnp.where(lo, m1, (m1 - m0) * C8), 64, 1)
            for t, val in enumerate([p0 + p1_, p0 - p1_, Pv - Qn, Pv + Qn]):
                if gam % 2 == 0:
                    T1s[n2, t, e] = val
                else:
                    pair = jnp.concatenate([T1s.pop((n2, t, e)), val], 0)
                    t_b[n2][t, pl.ds(64 * e + 8 * (gam - 1), 16), :] = pair.astype(BF)
                if t == 2:
                    dlq.append((val, state['now'] + PDL))

    def p1_d(n2):
        As = lhs_par([c_u[CA + t] for t in range(4)])
        for t in range(4):
            Z = jax.lax.dot_general(As[t], _bf(t_u[n2][oq(t, 4)]), NT, preferred_element_type=F32)
            z_b[n2][t] = Z.astype(BF)
        return rows8(Z, 8), 128

    def p1_mid(n2, t, tok):
        lo = _lane((32, 128)) < 64
        z = z_u[n2][oq(t, 4)]
        ZR = z[:32]
        RI = pltpu.roll(jnp.concatenate([gate(z[32 + 8 * q:40 + 8 * q], tok) for q in range(4)], 0), 64, 1)
        Zs[n2, 0, t] = jnp.where(lo, ZR, RI)
        Zs[n2, 1, t] = jnp.where(lo, RI, ZR)
        push_dl(Zs[n2, 0, t], state['now'] + PDL, 4)

    def p1_s(n2):
        T0, T1 = [jnp.concatenate([Zs.pop((n2, e, t)) for t in range(4)], 0) for e in range(2)]
        even = (_lane((128, 128)) % 2) == 0
        xi = []
        Ls = lhs_par([T0[:64], T1[:64], T0[64:], T1[64:]])
        for hf in range(2):
            O0 = jnp.dot(Ls[2 * hf], cmat(CM + 2 * n2), preferred_element_type=F32)
            O1 = jnp.dot(Ls[2 * hf + 1], cmat(CM + 2 * n2 + 1), preferred_element_type=F32)
            xr_v[n2, 128 * hf:128 * hf + 128, :] = jnp.where(even, O0, O1)
            xi.append(pltpu.roll(jnp.where(even, O1, O0), 127, 1))
            xi_v[n2, 128 * hf:128 * hf + 128, :] = xi[-1]
        for q in range(16):
            for hf in range(2):
                dlq.append((xi[hf][8 * q:8 * q + 8], state['t'] + DLAT + XDL + 8 * q))
        return rows8(O1, 8), 128

    def p2_items(grp):
        row = pl.ds(8 * grp, 8)
        kd0 = _kd_of_row(8 * grp)
        wrow = pl.ds(kd0 // 2, 8, stride=(_kd_of_row(8 * grp + 1) - kd0) // 2)
        unp = _hi_f32 if kd0 % 2 else _lo_f32
        y = [[None] * 4 for _ in range(4)]
        z = [[None] * 4 for _ in range(4)]
        X = [None] * 16
        Y = [None] * 16
        st = {}

        def f1(b, tok):
            v = [((xr_v[oq(4 * a + b, 16), row, :], 1), (xi_v[oq(4 * a + b, 16), row, :], 1)) for a in range(4)]
            o = _dft4(gatec(v, tok), +1)
            for kap in range(4):
                y[kap][b] = _twiddle(o[kap], b * kap, +1)

        def mid_a(kap, tok):
            o = _dft4(gatec(y[kap], tok), +1)
            for io in range(4):
                k = kap + 4 * io
                wr = unp(wr_u[k, wrow, :])
                wi = unp(wi_u[k, wrow, :])
                X[k] = o[io]
                (xr, sr), (xi, si) = o[io]
                Y[k] = (_sub((xr * wr, sr), (xi * wi, si)), _add((xr * wi, sr), (xi * wr, si)))

        def mid_b(kap):
            o2 = _dft4([Y[kap + 4 * io] for io in range(4)], -1)
            for b2 in range(4):
                z[b2][kap] = _twiddle(o2[b2], kap * b2, -1)

        def mid(kap, tok):
            mid_a(kap, tok)
            mid_b(kap)

        def i2(b2, tok):
            o = _dft4(gatec(z[b2], tok), -1)
            for io in range(4):
                yr_b[b2 + 4 * io, row, :] = _force(o[io][0]).astype(BF)
                yi_b[b2 + 4 * io, row, :] = _force(o[io][1]).astype(BF)

        def sp_stack(k, tok):
            sub = jax.lax.broadcasted_iota(jnp.int32, (8, 128), 0)
            w0r = unp(wr_u[k, wrow, :])[0:1]
            w0i = unp(wi_u[k, wrow, :])[0:1]
            wlr = wl_v[0, :, 128 * k:128 * k + 128].astype(F32)
            wli = wl_v[1, :, 128 * k:128 * k + 128].astype(F32)
            pr = gate(_force(X[k][0]), tok)[0:1]
            pi = _force(X[k][1])[0:1]
            blk = jnp.zeros((8, 128), F32)
            for jj, r in enumerate([pr, pi, w0r, w0i, wlr, wli]):
                blk = jnp.where(sub == jj, jnp.broadcast_to(r, (8, 128)), blk)
            st[k] = blk

        def sp_flip():
            full = jnp.concatenate([st[k] for k in range(16)], 0)
            fl = []
            for hf in range(2):
                part = full[64 * hf:64 * hf + 64]
                hi_ = part.astype(BF)
                lo_ = (part - hi_.astype(F32)).astype(BF)
                fh = jnp.dot(hi_, cmat(CJ), preferred_element_type=F32)
                fl.append(jnp.dot(lo_, cmat(CJ), preferred_element_type=F32) + fh)
            fl = jnp.concatenate(fl, 0)
            st['fl'] = fl
            return rows8(fl, 4), 64

        def sp_fix(k, tok):
            sub = jax.lax.broadcasted_iota(jnp.int32, (8, 128), 0)
            fl = st['fl']
            fa = fl[8 * (15 - k):8 * (15 - k) + 8]
            fb = fl[8 * ((16 - k) % 16):8 * ((16 - k) % 16) + 8]
            f = gate(jnp.where(_lane((8, 128)) == 0, fb, fa), tok)
            o = st[k]
            pr, pi, w0r, w0i, wlr, wli = [o[jj:jj + 1] for jj in range(6)]
            fpr, fpi, f0r, f0i, flr, fli = [f[jj:jj + 1] for jj in range(6)]
            s0r, s0i = w0r + f0r, w0i - f0i
            slr, sli = wlr + flr, wli - fli
            Ar, Ai_ = (s0r + slr) * 0.25, (s0i + sli) * 0.25
            Br, Bi = (s0r - slr) * 0.25, (s0i - sli) * 0.25
            yr0 = pr * Ar - pi * Ai_ + fpr * Br + fpi * Bi
            yi0 = pr * Ai_ + pi * Ar + fpr * Bi - fpi * Br
            yr = jnp.where(sub == 0, jnp.broadcast_to(yr0, (8, 128)), _force(Y[k][0]))
            yi = jnp.where(sub == 0, jnp.broadcast_to(yi0, (8, 128)), _force(Y[k][1]))
            Y[k] = ((yr, 1), (yi, 1))
            dlq.append((yr, state['t'] + 400))
            dlq.append((yi, state['t'] + 400))
            if k >= 12:
                mid_b(k - 12)

        first = [('v', P(f1, b), 30) for b in range(4)]
        last = [('v', P(i2, b), 28) for b in range(4)]
        if grp != 0:
            return first + [('v', P(mid, k), 78) for k in range(4)] + last, []
        a = (first + [('v', P(mid_a, k), 52) for k in range(4)] + [('v', P(sp_stack, k), 24) for k in range(16)]
             + [('m', sp_flip, 64)])
        b = [('v', P(sp_fix, k), 50 + (26 if k >= 12 else 0)) for k in range(16)] + last
        return a, b

    B3 = {}
    V3 = {}

    def p3_pre(n2, q, tok):
        even = (_lane((32, 128)) % 2) == 0
        Ru = yr_u[oq(n2, 16), pl.ds(32 * q, 32), :]
        Iu = yi_u[oq(n2, 16), pl.ds(32 * q, 32), :]
        Ou = pltpu.roll(jnp.concatenate([gate(Iu[8 * i:8 * i + 8], tok) for i in range(4)], 0), 1, 1)
        B3[n2, 0, q] = jnp.where(even, Ru, Ou)
        B3[n2, 1, q] = jnp.where(even, Ou, Ru)
        push_dl(B3[n2, 0, q], state['now'] + PDL, 4)

    def p3_s(n2):
        V = []
        Ms_ = lhs_par([c_u[CM + 2 * n2 + e] for e in range(2)])
        for e in range(2):
            B = _bf(jnp.concatenate([B3.pop((n2, e, q)) for q in range(4)], 0))
            V.append(jax.lax.dot_general(Ms_[e], B, NT, preferred_element_type=F32))
        V0, V1 = V
        V0r, V0i = V0[:64], V0[64:]
        V1i, V1r = V1[:64], V1[64:]
        VR = jnp.concatenate([V0r + V1r, V0r - V1r], 0)
        VI = jnp.concatenate([V0i + V1i, V0i - V1i], 0)
        for hf in range(2):
            v_b[n2][hf] = VR[:, 128 * hf:128 * hf + 128].astype(BF)
            v_b[n2][2 + hf] = VI[:, 128 * hf:128 * hf + 128].astype(BF)
        return rows8(V[1], 8), 128

    def p3_mid(n2, q, tok):
        hf, o = q // 2, 32 * (q % 2)
        lo = _lane((32, 128)) < 64
        r = v_u[n2][oq(hf, 4), pl.ds(o, 32), :]
        im = v_u[n2][oq(2 + hf, 4), pl.ds(o, 32), :]
        ri = pltpu.roll(jnp.concatenate([gate(im[8 * i:8 * i + 8], tok) for i in range(4)], 0), 64, 1)
        V3[n2, 2 * hf, q % 2] = jnp.where(lo, r, ri)
        V3[n2, 2 * hf + 1, q % 2] = jnp.where(lo, ri, r)
        push_dl(V3[n2, 2 * hf, q % 2], state['now'] + PDL, 4)

    def p3_d(r0):
        Gl = lhs_par([jnp.concatenate([V3.pop((n2, t, k)) for n2 in (2 * r0, 2 * r0 + 1) for k in range(2)], 0)
                      for t in range(4)])
        o = [jnp.dot(Gl[t], cmat(CAI + t), preferred_element_type=F32) for t in range(4)]
        v0, v2, T1, T3 = o
        lo = _lane((256, 128)) < 64
        Pp = T1 + T3
        Qp = pltpu.roll(T1 - T3, 64, 1)
        m0 = jnp.where(lo, Pp, (Qp - Pp) * C8)
        m1n = jnp.where(lo, Qp, (Pp + Qp) * C8)
        p0, p1_ = v0 + v2, v0 - v2
        y = [p0 + m0, p1_ - m1n, p0 - m0, p1_ + m1n]
        for s_ in range(2):
            for c in range(4):
                a_v[c, pl.ds(AP * (2 * r0 + s_), 128), :] = y[c][128 * s_:128 * s_ + 128]
        push_dl(m0, state['t'] + DLAT + 16, 8)
        push_dl(m1n, state['t'] + DLAT + 16, 8)
        return rows8(v0, 8), 256

    h_done = set()
    when = {}

    def m1(i, js, cs, defer):
        r2 = i * H
        xs = [[lhs(x_u(c, r2 + 8 * q, 8), 16 * q) for c in cs] for q in range(H // 8)]
        xc = jnp.concatenate([_bf(jnp.concatenate([xq[k] for xq in xs], 0)) for k in range(len(cs))], 1)
        w1 = jnp.concatenate([_bf(w1_u(c, 64 * js[0], 64 * len(js))) for c in cs], 1)
        raw = jax.lax.dot_general(xc, w1, NT, preferred_element_type=F32)

        def post(lat):
            for k, j in enumerate(js):
                r = raw[:, 128 * k:128 * k + 128]
                if cs[0] > 0:
                    r = r + p_v[i, j]
                if cs[-1] < 3:
                    p_v[i, j] = r
                    continue
                t = 0.5 * r
                th = jnp.tanh(t)
                t0 = state['t'] + lat + TM * k
                hs = t + t * th
                h_b[i][j] = hs.astype(BF)
                h_done.add((i, j))
                for q in range(TM // 16):
                    dlq.append((hs[16 * q + 8:16 * q + 16], t0 + 16 + 16 * q))
        if defer:
            pending.append(post)
        else:
            post(DLAT)
        return rows8(raw, 8), TM

    def gate_pk(b, tok):
        s_ = None
        for c in range(4):
            xv = _bf(gate(x_u(c, 8 * b, 8), tok)).astype(F32) * gw_f[oq(c, 4)]
            s_ = xv if s_ is None else s_ + xv
        lg = jnp.broadcast_to(jnp.sum(s_, axis=1, keepdims=True), (16, 128))
        tg = 0.5 * jnp.tanh(0.5 * lg)
        g_v[b // 8, pl.ds(16 * (b % 8), 16), :] = 0.5 + tg
        og_v[pl.ds(16 * b, 16), :] = 0.5 - tg
        push_dl(tg, state['now'] + GDL, 0)

    def mt(i):
        toks = []
        for ii in range(TM // 128):
            b = (TM // 128) * i + ii
            Ls = lhs_par([w1_u(c, 640, TR // 2) for c in range(4)])
            xw = jnp.concatenate([_bf(x_u(c, 64 * b, 64)) for c in range(4)], 1)
            raw = jax.lax.dot_general(jnp.concatenate(Ls, 1), xw, NT, preferred_element_type=F32)
            t = 0.5 * raw
            hs = t + t * jnp.tanh(t)
            full = jnp.concatenate([hs, jnp.zeros((128 - TR, 128), F32)], 0).T
            h_b[i][10, pl.ds(128 * ii, 128), :] = full.astype(BF)
            push_dl(full, state['t'] + TR + TDL2, 8)
            for tok, dt in rows8(raw, 8):
                toks.append((tok, TR * ii + dt))
            state['t'] += TR
        state['t'] -= TR * (TM // 128)
        h_done.add((i, 10))
        return toks, TR * (TM // 128)

    pending = []

    def flush():
        while pending:
            pending.pop()(64)

    accs = {}

    def m2(i, g):
        assert all((i, j) in h_done for j in range(11))
        assert all(('gate', b) in when for b in range(i * TM // 16, (i + 1) * TM // 16))
        cj = [divmod(f, 11) for f in range(4 * g, 4 * g + 4)]
        hq = [[lhs(h_u[i][oq(j, 11), pl.ds(8 * q, 8), :], 16 * q) for _, j in cj] for q in range(H // 8)]
        fin = []
        for c in sorted(set(c for c, _ in cj)):
            ks = [k for k in range(4) if cj[k][0] == c]
            j0 = cj[ks[0]][1]
            hs = jnp.concatenate([_bf(jnp.concatenate([hq_[k] for hq_ in hq], 0)) for k in ks], 1)
            o = jnp.dot(hs, _bf(w2_u[c, pl.ds(64 * j0, 64 * len(ks)), :]), preferred_element_type=F32)
            acc = o if j0 == 0 else o + accs.pop((i, c))
            if j0 + len(ks) < 11:
                accs[i, c] = acc
            else:
                bb_v[c, pl.ds(i * TM, TM), :] = acc * og_v[pl.ds(i * TM, TM), :]
                fin.append(c)
        return rows8(acc, 8), TM, fin

    def out_copy(i, c):
        return pltpu.make_async_copy(o_v.at[c, pl.ds(128 * i, 128)],
                                     o_hbm.at[0, pl.ds(128 * i, 128), pl.ds(128 * c, 128)], s_o.at[0])

    def combine(i, c, tok):
        av = []
        for n in range(8):
            for hf in range(2):
                a = a_v[c, pl.ds(8 * hf * AP + 8 * i + n, 8, stride=AP), :]
                av.append(a if tok is None else gate(a, tok))
        b = bb_v[c, pl.ds(128 * i, 128), :]
        o = g_v[oq(i, 16)] * jnp.concatenate(av, 0) + b
        o_v[c, pl.ds(128 * i, 128), :] = o.astype(BF)
        out_copy(i, c).start()

    VQ, MQ = [], []
    for b in range(XC * TM // 16):
        VQ.append((('gate', b), P(gate_pk, b), CG, [('xall', 0)]))

    def pre1(r0):
        for n2 in (2 * r0, 2 * r0 + 1):
            for gam in range(8):
                deps = [('rest', 0)] + ([(('d1', 2 * (r0 - 2)), 0)] if r0 >= 2 else [])
                VQ.append((('pre1', n2, gam), P(p1_pre, n2, gam), 58 * RATE / RATE1, deps))

    def mid(name, dep, fn, r0):
        for n2 in (2 * r0, 2 * r0 + 1):
            for q in range(4):
                VQ.append(((name, n2, q), P(fn, n2, q), CMID, [((dep, n2), L_MID)]))
    for r0 in range(10):
        if r0 < 8:
            pre1(r0)
        if r0 >= 2:
            mid('mid1', 'd1', p1_mid, r0 - 2)
    for r0 in range(10):
        if r0 < 8:
            for n2 in (2 * r0, 2 * r0 + 1):
                MQ.append((('d1', n2), P(p1_d, n2), [(('pre1', n2, 7), L_PRE)]))
        if r0 >= 2:
            for n2 in (2 * r0 - 4, 2 * r0 - 3):
                MQ.append((('s1', n2), P(p1_s, n2), [(('mid1', n2, 3), L_LHS)]))
    late_gates = list(range(XC * TM // 16, S // 16))
    kp = [0]

    def add2(items, extra=()):
        for it in items:
            kp[0] += 1
            if it[0] == 'v':
                VQ.append((('p2', kp[0]), it[1], it[2], list(extra) + [(('s1', 15), L_POST)]))
            else:
                MQ.append(('flip', it[1], [(('p2', kp[0] - 1), L_PRE)]))
    a0, b0 = p2_items(0)
    add2(a0)
    for g in range(1, 4):
        add2(p2_items(g)[0])
    add2(b0, [('flip', 250)])
    for g in range(4, 32):
        for b in late_gates[2 * (g - 4):2 * (g - 4) + 2]:
            VQ.append((('gate', b), P(gate_pk, b), 40, [('rest', 0)]))
        add2(p2_items(g)[0])
    last2 = [(VQ[-1][0], 100)]
    for r0 in range(9):
        if r0 < 8:
            for n2 in (2 * r0, 2 * r0 + 1):
                for q in range(4):
                    VQ.append((('pre3', n2, q), P(p3_pre, n2, q), C3, last2))
        if r0 >= 1:
            mid('mid3', 's3', p3_mid, r0 - 1)
    for r0 in range(9):
        if r0 < 8:
            for n2 in (2 * r0, 2 * r0 + 1):
                MQ.append((('s3', n2), P(p3_s, n2), [(('pre3', n2, 3), L_PRE)]))
        if r0 >= 1:
            MQ.append((('d3', r0 - 1), P(p3_d, r0 - 1), [(('mid3', 2 * r0 - 1, 3), L_LHS)]))
    for i in range(NCH):
        for c in range(4):
            for ii in range(TM // 128):
                VQ.append((('cmb', i, c, ii), P(combine, (TM // 128) * i + ii, c), CCOST,
                           [(('d3', 7), L_POST + 256), (('m2', i, c), 0)]))

    pieces = [('m1', 0, i, (0, 1, 2, 3), (0,)) for i in range(2)]
    pieces += [('m1', 1, i, js, (0,)) for i in range(4) for js in ((0, 1, 2, 3), (4, 5, 6, 7)) if i >= 2 or js[0] == 4]
    for i in range(4):
        pieces += [('m1', 2, i, (0, 1), (1, 2)), ('m1', 2, i, (2, 3), (1, 2)), ('m1', 2, i, (4, 5, 6, 7), (1,))]
    ks = []
    for i in range(4):
        ks += [('m1', 3, i, (0, 1, 2, 3), (3,)), ('m1', 3, i, (4, 5), (2, 3)), ('m1', 3, i, (6, 7), (2, 3))]
    full = [('m1', 3, i, (j,), (0, 1, 2, 3)) for i in range(XC) for j in range(10) if i >= KA or j >= KB]
    last = [('m1', 3, i, (10,), (0, 1, 2, 3)) for i in range(XC)]
    while ks or full or last:
        pieces += ks[:1] + full[:2] + ks[1:2] + full[2:3] + last[:1] + full[3:4]
        ks, last, full = ks[2:], last[1:], full[4:]
    wwait = len(pieces)
    pieces += [('m1', 3, i, (j,), (0, 1, 2, 3)) for i in range(XC, NCH) for j in range(10)]
    m2s = [('m2', i, g) for i in range(NCH) for g in range(11)]
    for k, i in enumerate(range(XC, NCH)):
        m2s.insert(MTPOS + 3 * k, ('m1', 3, i, (10,), (0, 1, 2, 3)))
    pieces += m2s

    def ok(deps, now):
        return all(d in when and when[d] + dl <= now for d, dl in deps)

    def issue(toks, cost):
        for tok, dt in toks:
            now = state['t'] + dt
            if VQ and now >= state['nxt'] and ok(VQ[0][3], now):
                name, fn, ops, _ = VQ.pop(0)
                state['now'] = now
                fn(tok)
                when[name] = now
                state['nxt'] = max(state['nxt'], now - 8) + ops / RATE
        state['t'] += cost

    def try_mxu():
        t0 = state['t']
        while MQ and ok(MQ[0][2], state['t']) and state['t'] - t0 < MBURST:
            name, fn, _ = MQ.pop(0)
            when[name] = state['t']
            issue(*fn())

    wv_done = -1
    for n, pc in enumerate(pieces):
        if pc[0] == 'm1' and pc[1] > wv_done:
            wv_done = pc[1]
            wait(wv_done)
            new_mask()
            flush()
            if wv_done == NWAVE - 1:
                when['xall'] = state['t']
        if n == wwait:
            wait(NWAVE)
            new_mask()
            flush()
            when['rest'] = state['t']
        try_mxu()
        if pc[0] == 'm1' and pc[3] == (10,):
            issue(*mt(pc[2]))
        elif pc[0] == 'm1':
            issue(*m1(pc[2], pc[3], pc[4], len(pc[3]) == 1 and n + 1 == wwait))
        else:
            toks, cost, fin = m2(pc[1], pc[2])
            issue(toks, cost)
            for c in fin:
                when['m2', pc[1], c] = state['t']
    assert not MQ
    for it in VQ:
        assert it[0][0] == 'cmb', it[0]
        it[1](None)
    for i in range(16):
        for c in range(4):
            out_copy(i, c).wait()


@jax.jit
def pallas_gated_mix__spectral_gfnet__dense_activation_silu__prompt_kernel(A_x, A_w_r, A_w_i, B_x, B_w1, B_w2, gate_w):
    consts = jnp.asarray(_consts(), dtype=BF)
    zero = jnp.zeros((1,), jnp.int32)
    hbm = pl.BlockSpec(memory_space=pltpu.HBM)
    dma = pltpu.SemaphoreType.DMA
    return pl.pallas_call(
        _kernel,
        in_specs=[hbm] * 8,
        out_specs=hbm,
        out_shape=jax.ShapeDtypeStruct((1, S, D), BF),
        scratch_shapes=[
            pltpu.VMEM((4, FP, 128), BF),
            pltpu.VMEM((16, 256, 128), BF),
            pltpu.VMEM((16, 256, 128), BF),
            pltpu.VMEM((2, 1, S), BF),
            pltpu.VMEM((NCONST, 128, 128), BF),
            pltpu.VMEM((16, 256, 128), F32),
            pltpu.VMEM((16, 256, 128), F32),
            pltpu.VMEM((16, 256, 128), BF),
            pltpu.VMEM((16, 256, 128), BF),
            pltpu.VMEM((4, 16 * AP, 128), F32),
            pltpu.VMEM((4, S, 128), F32),
            pltpu.VMEM((16, 128, 128), F32),
            pltpu.VMEM((S, 128), F32),
            pltpu.VMEM((4, S, 128), BF),
            pltpu.VMEM((KA, KB, TM, 128), F32),
            pltpu.SMEM((1,), jnp.int32),
            pltpu.VMEM((4, 128), BF),
            pltpu.VMEM((4, 16, 128), F32),
            dma((NWAVE + 1,)), dma((1,)),
        ] + [pltpu.VMEM((11, TM, 128), BF) for _ in range(NCH)]
        + [pltpu.VMEM((4, 128, 128), BF) for _ in range(3 * NB)]
        + [pltpu.VMEM((512, 128), BF) for _ in range(16 + 8)]
        + [pltpu.VMEM((F - 1024, 128), BF) for _ in range(4)],
        compiler_params=pltpu.CompilerParams(vmem_limit_bytes=100 << 20),
    )(zero, A_x, A_w_r.T, A_w_i.T, B_w1.T, B_w2, gate_w.reshape(4, 128), consts)
```

```python
import functools
import numpy as np
import jax
import jax.numpy as jnp
import jax.experimental.pallas as pl
import jax.experimental.pallas.tpu as pltpu

S, D, F = 2048, 512, 1376
FP = 1408
ODD = ((1, 7), (5, 3))
BF = jnp.bfloat16
F32 = jnp.float32
U32 = jnp.uint32
C8 = float(np.sqrt(0.5))
NT = (((1,), (1,)), ((), ()))


def _kd_of_row(rho):
    t, i = divmod(rho, 64)
    return 4 * i + 2 * t if t < 2 else 8 * (i % 32) + ODD[t - 2][i // 32]


@functools.lru_cache(maxsize=None)
def _consts():
    l = np.arange(128)
    A = np.zeros((4, 128, 128))
    for t in range(4):
        for i in range(64):
            rho = 64 * t + i
            kd = _kd_of_row(rho)
            if t < 2:
                ang = 2 * np.pi * ((l * kd) % 512) / 512
                A[t, i] = np.cos(ang)
                A[t, 64 + i] = -np.sin(ang)
                if rho == 0:
                    A[t, 64] = np.where(l % 2 == 0, 1.0, -1.0)
            else:
                f = t - 2
                lp = np.arange(64)
                k, cj = (kd, 1.0) if kd % 8 == 1 + 4 * f else (512 - kd, -1.0)
                ang = 2 * np.pi * ((lp * k) % 512) / 512
                c, s = np.cos(ang), -np.sin(ang)
                sg = 1.0 if f == 0 else -1.0
                A[t, i, :64] = c
                A[t, i, 64:] = -s * sg
                A[t, 64 + i, :64] = cj * s
                A[t, 64 + i, 64:] = cj * c * sg
    Ai = np.zeros((4, 128, 128))
    for t in range(4):
        sc = np.full(128, 2.0 / (S * D))
        if t == 0:
            sc[0] = sc[64] = 1.0 / (S * D)
        M = A[t] * sc[:, None]
        Ai[t] = M if t % 2 == 0 else np.concatenate([M[64:], M[:64]], 0)
    Ms = np.zeros((16, 2, 128, 128))
    n1 = np.arange(64)[:, None]
    k1 = np.arange(64)[None, :]
    for e in range(2):
        for n2 in range(16):
            ang = 2 * np.pi * (((16 * n1 + n2) * (e + 2 * k1)) % 2048) / 2048
            c, s = np.cos(ang), -np.sin(ang)
            re_cols = 2 * np.arange(64) + e
            im_cols = (2 * np.arange(64) + 1 + e) % 128
            M = np.zeros((128, 128))
            rr = slice(0, 64) if e == 0 else slice(64, 128)
            ir = slice(64, 128) if e == 0 else slice(0, 64)
            M[rr, re_cols] = c
            M[ir, re_cols] = -s
            M[rr, im_cols] = s
            M[ir, im_cols] = c
            Ms[n2, e] = M
    J = np.zeros((1, 128, 128))
    J[0, l, (128 - l) % 128] = 1.0
    allc = np.concatenate([A, Ai, J, Ms.reshape(32, 128, 128)], 0)
    return allc.astype(np.float32)


CA, CAI, CJ, CM = 0, 4, 8, 9
NCONST = 41


def _add(a, b):
    (x, sx), (y, sy) = a, b
    if sx == sy:
        return (x + y, sx)
    return (x - y, 1) if sx > 0 else (y - x, 1)


def _neg(a):
    return (a[0], -a[1])


def _sub(a, b):
    return _add(a, _neg(b))


def _scale(a, c):
    return (a[0] * (c * a[1]), 1)


def _cadd(a, b):
    return (_add(a[0], b[0]), _add(a[1], b[1]))


def _csub(a, b):
    return (_sub(a[0], b[0]), _sub(a[1], b[1]))


def _mul_mi(a, sgn):
    re, im = a
    return (im, _neg(re)) if sgn > 0 else (_neg(im), re)


def _twiddle(a, j, sgn):
    j = j % 16
    if j % 4 == 0:
        for _ in range(j // 4):
            a = _mul_mi(a, sgn)
        return a
    re, im = a
    if j % 2 == 0:
        if sgn > 0:
            r = _scale(_add(re, im), C8)
            i = _scale(_sub(im, re), C8)
        else:
            r = _scale(_sub(re, im), C8)
            i = _scale(_add(im, re), C8)
        a = (r, i)
        for _ in range(j // 4):
            a = _mul_mi(a, sgn)
        return a
    c = float(np.cos(2 * np.pi * j / 16))
    s = float(-sgn * np.sin(2 * np.pi * j / 16))
    r = _sub(_scale(re, c), _scale(im, s))
    i = _add(_scale(re, s), _scale(im, c))
    return (r, i)


def _dft4(v, sgn):
    a, b, c, d = v
    t0, t1 = _cadd(a, c), _csub(a, c)
    t2, t3 = _cadd(b, d), _mul_mi(_csub(b, d), sgn)
    return [_cadd(t0, t2), _cadd(t1, t3), _csub(t0, t2), _csub(t1, t3)]


def _force(a):
    return a[0] if a[1] > 0 else -a[0]


def _lo_f32(w):
    return pltpu.bitcast(w << 16, F32)


def _hi_f32(w):
    return pltpu.bitcast(w & jnp.uint32(0xFFFF0000), F32)


def _bf(u):
    return pltpu.bitcast(u, BF)


def _lane(shape):
    return jax.lax.broadcasted_iota(jnp.int32, shape, 1)


TM = 256
NCH = S // TM
H = TM // 2
TR = F - 1280
AP = 136
NB = 16
KA, KB = 4, 8
XC = 6
NWAVE = 4
RATE = 1.8
RATE1 = 1.15
C3 = 20
CMID = 20
CG = 120
CCOST = 130
L_PRE = 350
L_LHS = 300
L_MID = 180
L_POST = 450
DLAT = 260
XDL = 140
PDL = 340
GDL = 400
TDL2 = 500
DLQ2 = 64
MBURST = 256
MTPOS = 26


def _kernel(z_hbm, x_hbm, wr_hbm, wi_hbm, w1_hbm, w2_hbm, gw_hbm, c_hbm, o_hbm,
            w2b, wr_b, wi_b, wl_v, c_b, xr_v, xi_v, yr_b, yi_b, a_v, bb_v, g_v, og_v, o_v, p_v,
            z_ref, gw_ref, gw_f, sems, s_o, *bufs):
    P = functools.partial
    bufs = list(bufs)
    h_b, t_b, z_b, v_b, x_b, w1_b = [[bufs.pop(0) for _ in range(n)] for n in (NCH, NB, NB, NB, 16, 12)]
    w2_u, wr_u, wi_u, c_u, yr_u, yi_u = [r.bitcast(U32) for r in (w2b, wr_b, wi_b, c_b, yr_b, yi_b)]
    h_u, t_u, z_u, v_u, x_v, w1_v = [[r.bitcast(U32) for r in rs] for rs in (h_b, t_b, z_b, v_b, x_b, w1_b)]

    def x_u(c, r, n, stride=1):
        return x_v[4 * (r // 256) + c][pl.ds(r % 256, n, stride=stride), :]

    def w1_u(c, r, n):
        return w1_v[4 * (r // 256) + c][pl.ds(r % 256, n), :]

    groups = []

    def xrows(r0, r1, cs):
        return [(x_hbm.at[0, pl.ds(r, 512), pl.ds(128 * c, 128)], x_b[4 * (r // 512) + c])
                for c in cs for r in range(r0, r1, 512)]

    def w1rows(r0, r1, cs):
        return [(w1_hbm.at[pl.ds(r, min(512, F - r)), pl.ds(128 * c, 128)], w1_b[4 * (r // 512) + c])
                for c in cs for r in range(r0, r1, 512)]

    A4 = range(4)
    groups.append(xrows(0, 2 * TM, [0]) + w1rows(0, 512, [0]))
    groups.append(xrows(2 * TM, 4 * TM, [0]) + w1rows(512, 1024, [0]))
    groups.append(xrows(0, 4 * TM, [1]) + w1rows(0, 1024, [1]) + xrows(0, 4 * TM, [2]) + w1rows(0, 512, [2]))
    groups.append(w1rows(512, 1024, [2]) + xrows(0, 4 * TM, [3]) + w1rows(0, 1024, [3])
                  + w1rows(1024, F, A4) + xrows(4 * TM, XC * TM, A4))
    groups[0].append((z_hbm, z_ref))
    groups[-1].append((gw_hbm, gw_ref))
    rest = xrows(XC * TM, S, A4) + [(c_hbm, c_b)]
    rest += [(w2_hbm.at[:, pl.ds(128 * c, 128)], w2b.at[c, pl.ds(0, F)]) for c in range(4)]
    for k in range(16):
        rest.append((wr_hbm.at[pl.ds(0, 256), pl.ds(128 * k, 128)], wr_b.at[k]))
        rest.append((wi_hbm.at[pl.ds(0, 256), pl.ds(128 * k, 128)], wi_b.at[k]))
    rest.append((wr_hbm.at[pl.ds(256, 1), :], wl_v.at[0]))
    rest.append((wi_hbm.at[pl.ds(256, 1), :], wl_v.at[1]))
    groups.append(rest)
    copies = [[pltpu.make_async_copy(s_, d_, sems.at[gi]) for s_, d_ in g] for gi, g in enumerate(groups)]
    for g in copies:
        for cp in g:
            cp.start()

    def wait(gi):
        for cp in copies[gi]:
            cp.wait()
        if gi == NWAVE - 1:
            for c in range(4):
                gw_f[c] = jnp.broadcast_to(gw_ref[c:c + 1, :].astype(F32), (16, 128))
        if gi == NWAVE:
            for c in range(4):
                w2b[c, pl.ds(F, FP - F), :] = jnp.zeros((FP - F, 128), BF)

    fmask_box = {}
    dlq = []

    def gate(v, tok):
        if v.dtype != tok.dtype:
            tok = pltpu.bitcast(tok, v.dtype)
        return jnp.where(fmask_box['m'], tok, v)

    def new_mask():
        dlq.clear()
        z = z_ref[0]
        fmask_box.clear()
        fmask_box['z'] = z
        fmask_box['m'] = jnp.full((8, 128), z, jnp.int32) != 0

    def oq(k, n):
        if (k, n) not in fmask_box:
            fmask_box[k, n] = jnp.clip(k + fmask_box['z'], 0, n - 1)
        return fmask_box[k, n]

    def gatec(v, tok):
        out = list(v)
        for i in (0, 1):
            (r, sr), (im, si) = v[i]
            out[i] = ((gate(r, tok), sr), (gate(im, tok), si))
        return out

    def cmat(i):
        return _bf(c_u[i])

    def rows8(a, step):
        return [(a[8 * q:8 * q + 8, 0:128], step * q) for q in range(a.shape[0] // 8)]

    state = dict(t=0, nxt=0)

    def push_dl(a, t0, step):
        for v, dt in rows8(a, step):
            dlq.append((v, t0 + dt))

    def lhs(u, dt):
        tok = None
        dlq.sort(key=lambda e: e[1])
        for _ in range(2 if len(dlq) > DLQ2 else 1):
            if dlq and dlq[0][1] <= state['t'] + dt:
                v = pltpu.bitcast(dlq.pop(0)[0], U32)
                tok = v if tok is None else tok | v
        return u if tok is None else gate(u, tok)

    def lhs_par(ops):
        n = ops[0].shape[0] // 8
        g = [[lhs(u[8 * q:8 * q + 8], 16 * q) for u in ops] for q in range(n)]
        return [_bf(jnp.concatenate([g[q][k] for q in range(n)], 0)) for k in range(len(ops))]

    T1s = {}
    Zs = {}

    def p1_pre(n2, gam, tok):
        unp = _hi_f32 if n2 % 2 else _lo_f32
        lo = _lane((8, 128)) < 64
        r0 = n2 // 2 + 64 * gam
        a = [unp(gate(x_u(c, r0, 8, 8), tok)) for c in range(4)]
        b = [unp(x_u(c, r0 + 512, 8, 8)) for c in range(4)]
        for e in range(2):
            U = [a[c] + b[c] if e == 0 else a[c] - b[c] for c in range(4)]
            p0, p1_, m0, m1 = U[0] + U[2], U[1] + U[3], U[0] - U[2], U[1] - U[3]
            Pv = jnp.where(lo, m0, (m0 + m1) * (-C8))
            Qn = pltpu.roll(jnp.where(lo, m1, (m1 - m0) * C8), 64, 1)
            for t, val in enumerate([p0 + p1_, p0 - p1_, Pv - Qn, Pv + Qn]):
                if gam % 2 == 0:
                    T1s[n2, t, e] = val
                else:
                    pair = jnp.concatenate([T1s.pop((n2, t, e)), val], 0)
                    t_b[n2][t, pl.ds(64 * e + 8 * (gam - 1), 16), :] = pair.astype(BF)
                if t == 2:
                    dlq.append((val, state['now'] + PDL))

    def p1_d(n2):
        As = lhs_par([c_u[CA + t] for t in range(4)])
        for t in range(4):
            Z = jax.lax.dot_general(As[t], _bf(t_u[n2][oq(t, 4)]), NT, preferred_element_type=F32)
            z_b[n2][t] = Z.astype(BF)
        return rows8(Z, 8), 128

    def p1_mid(n2, t, tok):
        lo = _lane((32, 128)) < 64
        z = z_u[n2][oq(t, 4)]
        ZR = z[:32]
        RI = pltpu.roll(jnp.concatenate([gate(z[32 + 8 * q:40 + 8 * q], tok) for q in range(4)], 0), 64, 1)
        Zs[n2, 0, t] = jnp.where(lo, ZR, RI)
        Zs[n2, 1, t] = jnp.where(lo, RI, ZR)
        push_dl(Zs[n2, 0, t], state['now'] + PDL, 4)

    def p1_s(n2):
        T0, T1 = [jnp.concatenate([Zs.pop((n2, e, t)) for t in range(4)], 0) for e in range(2)]
        even = (_lane((128, 128)) % 2) == 0
        xi = []
        Ls = lhs_par([T0[:64], T1[:64], T0[64:], T1[64:]])
        for hf in range(2):
            O0 = jnp.dot(Ls[2 * hf], cmat(CM + 2 * n2), preferred_element_type=F32)
            O1 = jnp.dot(Ls[2 * hf + 1], cmat(CM + 2 * n2 + 1), preferred_element_type=F32)
            xr_v[n2, 128 * hf:128 * hf + 128, :] = jnp.where(even, O0, O1)
            xi.append(pltpu.roll(jnp.where(even, O1, O0), 127, 1))
            xi_v[n2, 128 * hf:128 * hf + 128, :] = xi[-1]
        for q in range(16):
            for hf in range(2):
                dlq.append((xi[hf][8 * q:8 * q + 8], state['t'] + DLAT + XDL + 8 * q))
        return rows8(O1, 8), 128

    def p2_items(grp):
        row = pl.ds(8 * grp, 8)
        kd0 = _kd_of_row(8 * grp)
        wrow = pl.ds(kd0 // 2, 8, stride=(_kd_of_row(8 * grp + 1) - kd0) // 2)
        unp = _hi_f32 if kd0 % 2 else _lo_f32
        y = [[None] * 4 for _ in range(4)]
        z = [[None] * 4 for _ in range(4)]
        X = [None] * 16
        Y = [None] * 16
        st = {}

        def f1(b, tok):
            v = [((xr_v[oq(4 * a + b, 16), row, :], 1), (xi_v[oq(4 * a + b, 16), row, :], 1)) for a in range(4)]
            o = _dft4(gatec(v, tok), +1)
            for kap in range(4):
                y[kap][b] = _twiddle(o[kap], b * kap, +1)

        def mid_a(kap, tok):
            o = _dft4(gatec(y[kap], tok), +1)
            for io in range(4):
                k = kap + 4 * io
                wr = unp(wr_u[k, wrow, :])
                wi = unp(wi_u[k, wrow, :])
                X[k] = o[io]
                (xr, sr), (xi, si) = o[io]
                Y[k] = (_sub((xr * wr, sr), (xi * wi, si)), _add((xr * wi, sr), (xi * wr, si)))

        def mid_b(kap):
            o2 = _dft4([Y[kap + 4 * io] for io in range(4)], -1)
            for b2 in range(4):
                z[b2][kap] = _twiddle(o2[b2], kap * b2, -1)

        def mid(kap, tok):
            mid_a(kap, tok)
            mid_b(kap)

        def i2(b2, tok):
            o = _dft4(gatec(z[b2], tok), -1)
            for io in range(4):
                yr_b[b2 + 4 * io, row, :] = _force(o[io][0]).astype(BF)
                yi_b[b2 + 4 * io, row, :] = _force(o[io][1]).astype(BF)

        def sp_stack(k, tok):
            sub = jax.lax.broadcasted_iota(jnp.int32, (8, 128), 0)
            w0r = unp(wr_u[k, wrow, :])[0:1]
            w0i = unp(wi_u[k, wrow, :])[0:1]
            wlr = wl_v[0, :, 128 * k:128 * k + 128].astype(F32)
            wli = wl_v[1, :, 128 * k:128 * k + 128].astype(F32)
            pr = gate(_force(X[k][0]), tok)[0:1]
            pi = _force(X[k][1])[0:1]
            blk = jnp.zeros((8, 128), F32)
            for jj, r in enumerate([pr, pi, w0r, w0i, wlr, wli]):
                blk = jnp.where(sub == jj, jnp.broadcast_to(r, (8, 128)), blk)
            st[k] = blk

        def sp_flip():
            full = jnp.concatenate([st[k] for k in range(16)], 0)
            fl = []
            for hf in range(2):
                part = full[64 * hf:64 * hf + 64]
                hi_ = part.astype(BF)
                lo_ = (part - hi_.astype(F32)).astype(BF)
                fh = jnp.dot(hi_, cmat(CJ), preferred_element_type=F32)
                fl.append(jnp.dot(lo_, cmat(CJ), preferred_element_type=F32) + fh)
            fl = jnp.concatenate(fl, 0)
            st['fl'] = fl
            return rows8(fl, 4), 64

        def sp_fix(k, tok):
            sub = jax.lax.broadcasted_iota(jnp.int32, (8, 128), 0)
            fl = st['fl']
            fa = fl[8 * (15 - k):8 * (15 - k) + 8]
            fb = fl[8 * ((16 - k) % 16):8 * ((16 - k) % 16) + 8]
            f = gate(jnp.where(_lane((8, 128)) == 0, fb, fa), tok)
            o = st[k]
            pr, pi, w0r, w0i, wlr, wli = [o[jj:jj + 1] for jj in range(6)]
            fpr, fpi, f0r, f0i, flr, fli = [f[jj:jj + 1] for jj in range(6)]
            s0r, s0i = w0r + f0r, w0i - f0i
            slr, sli = wlr + flr, wli - fli
            Ar, Ai_ = (s0r + slr) * 0.25, (s0i + sli) * 0.25
            Br, Bi = (s0r - slr) * 0.25, (s0i - sli) * 0.25
            yr0 = pr * Ar - pi * Ai_ + fpr * Br + fpi * Bi
            yi0 = pr * Ai_ + pi * Ar + fpr * Bi - fpi * Br
            yr = jnp.where(sub == 0, jnp.broadcast_to(yr0, (8, 128)), _force(Y[k][0]))
            yi = jnp.where(sub == 0, jnp.broadcast_to(yi0, (8, 128)), _force(Y[k][1]))
            Y[k] = ((yr, 1), (yi, 1))
            dlq.append((yr, state['t'] + 400))
            dlq.append((yi, state['t'] + 400))
            if k >= 12:
                mid_b(k - 12)

        first = [('v', P(f1, b), 30) for b in range(4)]
        last = [('v', P(i2, b), 28) for b in range(4)]
        if grp != 0:
            return first + [('v', P(mid, k), 78) for k in range(4)] + last, []
        a = (first + [('v', P(mid_a, k), 52) for k in range(4)] + [('v', P(sp_stack, k), 24) for k in range(16)]
             + [('m', sp_flip, 64)])
        b = [('v', P(sp_fix, k), 50 + (26 if k >= 12 else 0)) for k in range(16)] + last
        return a, b

    B3 = {}
    V3 = {}

    def p3_pre(n2, q, tok):
        even = (_lane((32, 128)) % 2) == 0
        Ru = yr_u[oq(n2, 16), pl.ds(32 * q, 32), :]
        Iu = yi_u[oq(n2, 16), pl.ds(32 * q, 32), :]
        Ou = pltpu.roll(jnp.concatenate([gate(Iu[8 * i:8 * i + 8], tok) for i in range(4)], 0), 1, 1)
        B3[n2, 0, q] = jnp.where(even, Ru, Ou)
        B3[n2, 1, q] = jnp.where(even, Ou, Ru)
        push_dl(B3[n2, 0, q], state['now'] + PDL, 4)

    def p3_s(n2):
        V = []
        Ms_ = lhs_par([c_u[CM + 2 * n2 + e] for e in range(2)])
        for e in range(2):
            B = _bf(jnp.concatenate([B3.pop((n2, e, q)) for q in range(4)], 0))
            V.append(jax.lax.dot_general(Ms_[e], B, NT, preferred_element_type=F32))
        V0, V1 = V
        V0r, V0i = V0[:64], V0[64:]
        V1i, V1r = V1[:64], V1[64:]
        VR = jnp.concatenate([V0r + V1r, V0r - V1r], 0)
        VI = jnp.concatenate([V0i + V1i, V0i - V1i], 0)
        for hf in range(2):
            v_b[n2][hf] = VR[:, 128 * hf:128 * hf + 128].astype(BF)
            v_b[n2][2 + hf] = VI[:, 128 * hf:128 * hf + 128].astype(BF)
        return rows8(V[1], 8), 128

    def p3_mid(n2, q, tok):
        hf, o = q // 2, 32 * (q % 2)
        lo = _lane((32, 128)) < 64
        r = v_u[n2][oq(hf, 4), pl.ds(o, 32), :]
        im = v_u[n2][oq(2 + hf, 4), pl.ds(o, 32), :]
        ri = pltpu.roll(jnp.concatenate([gate(im[8 * i:8 * i + 8], tok) for i in range(4)], 0), 64, 1)
        V3[n2, 2 * hf, q % 2] = jnp.where(lo, r, ri)
        V3[n2, 2 * hf + 1, q % 2] = jnp.where(lo, ri, r)
        push_dl(V3[n2, 2 * hf, q % 2], state['now'] + PDL, 4)

    def p3_d(r0):
        Gl = lhs_par([jnp.concatenate([V3.pop((n2, t, k)) for n2 in (2 * r0, 2 * r0 + 1) for k in range(2)], 0)
                      for t in range(4)])
        o = [jnp.dot(Gl[t], cmat(CAI + t), preferred_element_type=F32) for t in range(4)]
        v0, v2, T1, T3 = o
        lo = _lane((256, 128)) < 64
        Pp = T1 + T3
        Qp = pltpu.roll(T1 - T3, 64, 1)
        m0 = jnp.where(lo, Pp, (Qp - Pp) * C8)
        m1n = jnp.where(lo, Qp, (Pp + Qp) * C8)
        p0, p1_ = v0 + v2, v0 - v2
        y = [p0 + m0, p1_ - m1n, p0 - m0, p1_ + m1n]
        for s_ in range(2):
            for c in range(4):
                a_v[c, pl.ds(AP * (2 * r0 + s_), 128), :] = y[c][128 * s_:128 * s_ + 128]
        push_dl(m0, state['t'] + DLAT + 16, 8)
        push_dl(m1n, state['t'] + DLAT + 16, 8)
        return rows8(v0, 8), 256

    h_done = set()
    when = {}

    def m1(i, js, cs, defer):
        r2 = i * H
        xs = [[lhs(x_u(c, r2 + 8 * q, 8), 16 * q) for c in cs] for q in range(H // 8)]
        xc = jnp.concatenate([_bf(jnp.concatenate([xq[k] for xq in xs], 0)) for k in range(len(cs))], 1)
        w1 = jnp.concatenate([_bf(w1_u(c, 64 * js[0], 64 * len(js))) for c in cs], 1)
        raw = jax.lax.dot_general(xc, w1, NT, preferred_element_type=F32)

        def post(lat):
            for k, j in enumerate(js):
                r = raw[:, 128 * k:128 * k + 128]
                if cs[0] > 0:
                    r = r + p_v[i, j]
                if cs[-1] < 3:
                    p_v[i, j] = r
                    continue
                t = 0.5 * r
                th = jnp.tanh(t)
                t0 = state['t'] + lat + TM * k
                hs = t + t * th
                h_b[i][j] = hs.astype(BF)
                h_done.add((i, j))
                for q in range(TM // 16):
                    dlq.append((hs[16 * q + 8:16 * q + 16], t0 + 16 + 16 * q))
        if defer:
            pending.append(post)
        else:
            post(DLAT)
        return rows8(raw, 8), TM

    def gate_pk(b, tok):
        s_ = None
        for c in range(4):
            xv = _bf(gate(x_u(c, 8 * b, 8), tok)).astype(F32) * gw_f[oq(c, 4)]
            s_ = xv if s_ is None else s_ + xv
        lg = jnp.broadcast_to(jnp.sum(s_, axis=1, keepdims=True), (16, 128))
        tg = 0.5 * jnp.tanh(0.5 * lg)
        g_v[b // 8, pl.ds(16 * (b % 8), 16), :] = 0.5 + tg
        og_v[pl.ds(16 * b, 16), :] = 0.5 - tg
        push_dl(tg, state['now'] + GDL, 0)

    def mt(i):
        toks = []
        for ii in range(TM // 128):
            b = (TM // 128) * i + ii
            Ls = lhs_par([w1_u(c, 640, TR // 2) for c in range(4)])
            xw = jnp.concatenate([_bf(x_u(c, 64 * b, 64)) for c in range(4)], 1)
            raw = jax.lax.dot_general(jnp.concatenate(Ls, 1), xw, NT, preferred_element_type=F32)
            t = 0.5 * raw
            hs = t + t * jnp.tanh(t)
            full = jnp.concatenate([hs, jnp.zeros((128 - TR, 128), F32)], 0).T
            h_b[i][10, pl.ds(128 * ii, 128), :] = full.astype(BF)
            push_dl(full, state['t'] + TR + TDL2, 8)
            for tok, dt in rows8(raw, 8):
                toks.append((tok, TR * ii + dt))
            state['t'] += TR
        state['t'] -= TR * (TM // 128)
        h_done.add((i, 10))
        return toks, TR * (TM // 128)

    pending = []

    def flush():
        while pending:
            pending.pop()(64)

    accs = {}

    def m2(i, g):
        assert all((i, j) in h_done for j in range(11))
        assert all(('gate', b) in when for b in range(i * TM // 16, (i + 1) * TM // 16))
        cj = [divmod(f, 11) for f in range(4 * g, 4 * g + 4)]
        hq = [[lhs(h_u[i][oq(j, 11), pl.ds(8 * q, 8), :], 16 * q) for _, j in cj] for q in range(H // 8)]
        fin = []
        for c in sorted(set(c for c, _ in cj)):
            ks = [k for k in range(4) if cj[k][0] == c]
            j0 = cj[ks[0]][1]
            hs = jnp.concatenate([_bf(jnp.concatenate([hq_[k] for hq_ in hq], 0)) for k in ks], 1)
            o = jnp.dot(hs, _bf(w2_u[c, pl.ds(64 * j0, 64 * len(ks)), :]), preferred_element_type=F32)
            acc = o if j0 == 0 else o + accs.pop((i, c))
            if j0 + len(ks) < 11:
                accs[i, c] = acc
            else:
                bb_v[c, pl.ds(i * TM, TM), :] = acc * og_v[pl.ds(i * TM, TM), :]
                fin.append(c)
        return rows8(acc, 8), TM, fin

    def out_copy(i, c):
        return pltpu.make_async_copy(o_v.at[c, pl.ds(128 * i, 128)],
                                     o_hbm.at[0, pl.ds(128 * i, 128), pl.ds(128 * c, 128)], s_o.at[0])

    def combine(i, c, tok):
        av = []
        for n in range(8):
            for hf in range(2):
                a = a_v[c, pl.ds(8 * hf * AP + 8 * i + n, 8, stride=AP), :]
                av.append(a if tok is None else gate(a, tok))
        b = bb_v[c, pl.ds(128 * i, 128), :]
        o = g_v[oq(i, 16)] * jnp.concatenate(av, 0) + b
        o_v[c, pl.ds(128 * i, 128), :] = o.astype(BF)
        out_copy(i, c).start()

    VQ, MQ = [], []
    for b in range(XC * TM // 16):
        VQ.append((('gate', b), P(gate_pk, b), CG, [('xall', 0)]))

    def pre1(r0):
        for n2 in (2 * r0, 2 * r0 + 1):
            for gam in range(8):
                deps = [('rest', 0)] + ([(('d1', 2 * (r0 - 2)), 0)] if r0 >= 2 else [])
                VQ.append((('pre1', n2, gam), P(p1_pre, n2, gam), 58 * RATE / RATE1, deps))

    def mid(name, dep, fn, r0):
        for n2 in (2 * r0, 2 * r0 + 1):
            for q in range(4):
                VQ.append(((name, n2, q), P(fn, n2, q), CMID, [((dep, n2), L_MID)]))
    for r0 in range(10):
        if r0 < 8:
            pre1(r0)
        if r0 >= 2:
            mid('mid1', 'd1', p1_mid, r0 - 2)
    for r0 in range(10):
        if r0 < 8:
            for n2 in (2 * r0, 2 * r0 + 1):
                MQ.append((('d1', n2), P(p1_d, n2), [(('pre1', n2, 7), L_PRE)]))
        if r0 >= 2:
            for n2 in (2 * r0 - 4, 2 * r0 - 3):
                MQ.append((('s1', n2), P(p1_s, n2), [(('mid1', n2, 3), L_LHS)]))
    late_gates = list(range(XC * TM // 16, S // 16))
    kp = [0]

    def add2(items, extra=()):
        for it in items:
            kp[0] += 1
            if it[0] == 'v':
                VQ.append((('p2', kp[0]), it[1], it[2], list(extra) + [(('s1', 15), L_POST)]))
            else:
                MQ.append(('flip', it[1], [(('p2', kp[0] - 1), L_PRE)]))
    a0, b0 = p2_items(0)
    add2(a0)
    for g in range(1, 4):
        add2(p2_items(g)[0])
    add2(b0, [('flip', 250)])
    for g in range(4, 32):
        for b in late_gates[2 * (g - 4):2 * (g - 4) + 2]:
            VQ.append((('gate', b), P(gate_pk, b), 40, [('rest', 0)]))
        add2(p2_items(g)[0])
    last2 = [(VQ[-1][0], 100)]
    for r0 in range(9):
        if r0 < 8:
            for n2 in (2 * r0, 2 * r0 + 1):
                for q in range(4):
                    VQ.append((('pre3', n2, q), P(p3_pre, n2, q), C3, last2))
        if r0 >= 1:
            mid('mid3', 's3', p3_mid, r0 - 1)
    for r0 in range(9):
        if r0 < 8:
            for n2 in (2 * r0, 2 * r0 + 1):
                MQ.append((('s3', n2), P(p3_s, n2), [(('pre3', n2, 3), L_PRE)]))
        if r0 >= 1:
            MQ.append((('d3', r0 - 1), P(p3_d, r0 - 1), [(('mid3', 2 * r0 - 1, 3), L_LHS)]))
    for i in range(NCH):
        for c in range(4):
            for ii in range(TM // 128):
                VQ.append((('cmb', i, c, ii), P(combine, (TM // 128) * i + ii, c), CCOST,
                           [(('d3', 7), L_POST + 256), (('m2', i, c), 0)]))

    pieces = [('m1', 0, i, (0, 1, 2, 3), (0,)) for i in range(2)]
    pieces += [('m1', 1, i, js, (0,)) for i in range(4) for js in ((0, 1, 2, 3), (4, 5, 6, 7)) if i >= 2 or js[0] == 4]
    for i in range(4):
        pieces += [('m1', 2, i, (0, 1), (1, 2)), ('m1', 2, i, (2, 3), (1, 2)), ('m1', 2, i, (4, 5, 6, 7), (1,))]
    ks = []
    for i in range(4):
        ks += [('m1', 3, i, (0, 1, 2, 3), (3,)), ('m1', 3, i, (4, 5), (2, 3)), ('m1', 3, i, (6, 7), (2, 3))]
    full = [('m1', 3, i, (j,), (0, 1, 2, 3)) for i in range(XC) for j in range(10) if i >= KA or j >= KB]
    last = [('m1', 3, i, (10,), (0, 1, 2, 3)) for i in range(XC)]
    while ks or full or last:
        pieces += ks[:1] + full[:2] + ks[1:2] + full[2:3] + last[:1] + full[3:4]
        ks, last, full = ks[2:], last[1:], full[4:]
    wwait = len(pieces)
    pieces += [('m1', 3, i, (j,), (0, 1, 2, 3)) for i in range(XC, NCH) for j in range(10)]
    m2s = [('m2', i, g) for i in range(NCH) for g in range(11)]
    for k, i in enumerate(range(XC, NCH)):
        m2s.insert(MTPOS + 3 * k, ('m1', 3, i, (10,), (0, 1, 2, 3)))
    pieces += m2s

    def ok(deps, now):
        return all(d in when and when[d] + dl <= now for d, dl in deps)

    def issue(toks, cost):
        for tok, dt in toks:
            now = state['t'] + dt
            if VQ and now >= state['nxt'] and ok(VQ[0][3], now):
                name, fn, ops, _ = VQ.pop(0)
                state['now'] = now
                fn(tok)
                when[name] = now
                state['nxt'] = max(state['nxt'], now - 8) + ops / RATE
        state['t'] += cost

    def try_mxu():
        t0 = state['t']
        while MQ and ok(MQ[0][2], state['t']) and state['t'] - t0 < MBURST:
            name, fn, _ = MQ.pop(0)
            when[name] = state['t']
            issue(*fn())

    wv_done = -1
    for n, pc in enumerate(pieces):
        if pc[0] == 'm1' and pc[1] > wv_done:
            wv_done = pc[1]
            wait(wv_done)
            new_mask()
            flush()
            if wv_done == NWAVE - 1:
                when['xall'] = state['t']
        if n == wwait:
            wait(NWAVE)
            new_mask()
            flush()
            when['rest'] = state['t']
        try_mxu()
        if pc[0] == 'm1' and pc[3] == (10,):
            issue(*mt(pc[2]))
        elif pc[0] == 'm1':
            issue(*m1(pc[2], pc[3], pc[4], len(pc[3]) == 1 and n + 1 == wwait))
        else:
            toks, cost, fin = m2(pc[1], pc[2])
            issue(toks, cost)
            for c in fin:
                when['m2', pc[1], c] = state['t']
    assert not MQ
    for it in VQ:
        assert it[0][0] == 'cmb', it[0]
        it[1](None)
    for i in range(16):
        for c in range(4):
            out_copy(i, c).wait()


@jax.jit
def pallas_gated_mix__spectral_gfnet__dense_activation_silu__prompt_kernel(A_x, A_w_r, A_w_i, B_x, B_w1, B_w2, gate_w):
    consts = jnp.asarray(_consts(), dtype=BF)
    zero = jnp.zeros((1,), jnp.int32)
    hbm = pl.BlockSpec(memory_space=pltpu.HBM)
    dma = pltpu.SemaphoreType.DMA
    return pl.pallas_call(
        _kernel,
        in_specs=[hbm] * 8,
        out_specs=hbm,
        out_shape=jax.ShapeDtypeStruct((1, S, D), BF),
        scratch_shapes=[
            pltpu.VMEM((4, FP, 128), BF),
            pltpu.VMEM((16, 256, 128), BF),
            pltpu.VMEM((16, 256, 128), BF),
            pltpu.VMEM((2, 1, S), BF),
            pltpu.VMEM((NCONST, 128, 128), BF),
            pltpu.VMEM((16, 256, 128), F32),
            pltpu.VMEM((16, 256, 128), F32),
            pltpu.VMEM((16, 256, 128), BF),
            pltpu.VMEM((16, 256, 128), BF),
            pltpu.VMEM((4, 16 * AP, 128), F32),
            pltpu.VMEM((4, S, 128), F32),
            pltpu.VMEM((16, 128, 128), F32),
            pltpu.VMEM((S, 128), F32),
            pltpu.VMEM((4, S, 128), BF),
            pltpu.VMEM((KA, KB, TM, 128), F32),
            pltpu.SMEM((1,), jnp.int32),
            pltpu.VMEM((4, 128), BF),
            pltpu.VMEM((4, 16, 128), F32),
            dma((NWAVE + 1,)), dma((1,)),
        ] + [pltpu.VMEM((11, TM, 128), BF) for _ in range(NCH)]
        + [pltpu.VMEM((4, 128, 128), BF) for _ in range(3 * NB)]
        + [pltpu.VMEM((512, 128), BF) for _ in range(16 + 8)]
        + [pltpu.VMEM((F - 1024, 128), BF) for _ in range(4)],
        compiler_params=pltpu.CompilerParams(vmem_limit_bytes=100 << 20),
    )(zero, A_x, A_w_r.T, A_w_i.T, B_w1.T, B_w2, gate_w.reshape(4, 128), consts)
```
